```python
import jax
import jax.numpy as jnp

def _softmax(x, axis=-1):
    return jax.nn.softmax(x, axis=axis)

def _gelu(x):
    return jax.nn.gelu(x, approximate=True)

def _silu(x):
    return jax.nn.silu(x)

def _sigmoid(x):
    return jax.nn.sigmoid(x)

def _layernorm(x, axis=-1, eps=1e-05):
    m = jnp.mean(x, axis=axis, keepdims=True)
    v = jnp.var(x, axis=axis, keepdims=True)
    return (x - m) / jnp.sqrt(v + eps)

def _scatter_add(tgt, idx, src, axis=0):
    return tgt.at[idx].add(src)

def _segment_sum(src, seg, n):
    return jax.ops.segment_sum(src, seg, n)

class _Rng:

    def __init__(self, key):
        self._k = key

    def _next(self):
        self._k, sub = jax.random.split(self._k)
        return sub

    def normal(self, shape):
        return jax.random.normal(self._next(), shape, dtype=jnp.bfloat16)

    def randint(self, lo, hi, shape):
        return jax.random.randint(self._next(), shape, lo, hi, dtype=jnp.int32)

    def uniform(self, shape, lo=0.0, hi=1.0):
        return jax.random.uniform(self._next(), shape, jnp.bfloat16, lo, hi)

    def permutation(self, n):
        return jax.random.permutation(self._next(), n)
kernel_name = 'interleave_layers__memory_aug_infini_attn__moe_arch_mod__prompt'

def setup_inputs():
    _rng = _Rng(jax.random.key(int.from_bytes(__import__("os").urandom(4), "little")))
    _w = lambda a: (lambda t: t.astype(jnp.bfloat16) if jnp.issubdtype(t.dtype, jnp.floating) else t)(jnp.asarray(a))

    def _A_setup():
        B, S, D, H = (1, 2048, 1024, 32)
        N = 4
        L = max(1, S // N)
        sc = D ** (-0.5)
        return {'x': _w((lambda *s: _rng.normal(s) * 0.05)(B, N * L, D)), 'wq': _w((lambda *s: _rng.normal(s) * 0.05)(D, D) * sc), 'wk': _w((lambda *s: _rng.normal(s) * 0.05)(D, D) * sc), 'wv': _w((lambda *s: _rng.normal(s) * 0.05)(D, D) * sc), 'wo': _w((lambda *s: _rng.normal(s) * 0.05)(D, D) * sc), 'beta': _w((lambda *s: _rng.normal(s) * 0.05)(H))}
    _A_in = _A_setup()

    def _B_setup():
        B, S, D, F, C = (1, 2048, 1024, 3584, 2)
        return {'x': _w((lambda *s: _rng.normal(s) * 0.05)(B, S, D)), 'w_r': _w((lambda *s: _rng.normal(s) * 0.05)(D)), 'w_gate': _w((lambda *s: _rng.normal(s) * 0.05)(D, F)), 'w_up': _w((lambda *s: _rng.normal(s) * 0.05)(D, F)), 'w_down': _w((lambda *s: _rng.normal(s) * 0.05)(F, D))}
    _B_in = _B_setup()
    return {'A_x': _A_in['x'], 'A_wq': _A_in['wq'], 'A_wk': _A_in['wk'], 'A_wv': _A_in['wv'], 'A_wo': _A_in['wo'], 'A_beta': _A_in['beta'], 'B_x': _B_in['x'], 'B_w_r': _B_in['w_r'], 'B_w_gate': _B_in['w_gate'], 'B_w_up': _B_in['w_up'], 'B_w_down': _B_in['w_down']}

def reference(A_x, A_wq, A_wk, A_wv, A_wo, A_beta, B_x, B_w_r, B_w_gate, B_w_up, B_w_down):

    def _A_ref(x, wq, wk, wv, wo, beta):
        B, S, D = x.shape
        H = 32
        Dh = D // H
        N = 4
        L = S // N
        q = (lambda x, *d: x.transpose(*d))((x @ wq).reshape(B, S, H, Dh), 0, 2, 1, 3).reshape(B, H, N, L, Dh)
        k = (lambda x, *d: x.transpose(*d))((x @ wk).reshape(B, S, H, Dh), 0, 2, 1, 3).reshape(B, H, N, L, Dh)
        v = (lambda x, *d: x.transpose(*d))((x @ wv).reshape(B, S, H, Dh), 0, 2, 1, 3).reshape(B, H, N, L, Dh)
        phi = lambda t: jnp.where(t > 0, t + 1.0, jnp.exp(t))
        scale = Dh ** (-0.5)
        ar = jnp.arange(L)
        mask = (lambda x, dt: x.astype(dt))(ar[:, None] < ar[None, :], x.dtype) * -1000000000.0
        g = _sigmoid(beta).reshape(1, H, 1, 1)
        M = jnp.einsum('bhd,bhe->bhde', q[:, :, 0, 0, :] * 0.0, q[:, :, 0, 0, :] * 0.0)
        z = q[:, :, 0, 0, :] * 0.0
        outs = []
        for s in range(N):
            qs, ks, vs = (q[:, :, s].copy(), k[:, :, s].copy(), v[:, :, s].copy())
            logits = jnp.einsum('bhqd,bhkd->bhqk', qs, ks) * scale + mask
            p = _softmax(logits, axis=-1)
            a_dot = jnp.einsum('bhqk,bhkd->bhqd', p, vs)
            pq = phi(qs)
            num = jnp.einsum('bhld,bhde->bhle', pq, M)
            den = jnp.einsum('bhld,bhd->bhl', pq, z)[..., None] + 1e-06
            a_mem = num / den
            o = g * a_mem + (1.0 - g) * a_dot
            outs.append(o)
            pk = phi(ks)
            M = M + jnp.einsum('bhld,bhle->bhde', pk, vs)
            z = z + jnp.einsum('bhld->bhd', pk)
        o = (lambda x, *d: x.transpose(*d))(jnp.stack(outs, 2).reshape(B, H, S, Dh), 0, 2, 1, 3).reshape(B, S, D)
        return o @ wo

    def _B_ref(x, w_r, w_gate, w_up, w_down):
        B, S, D = x.shape
        C = 2
        r = x @ w_r
        idx = jnp.argsort(-r, axis=-1)[:, :C]
        idx_e = jnp.repeat(idx.reshape(B, C, 1), D, axis=2)
        x_sel = jnp.take_along_axis(x, idx_e, axis=1)
        g = _silu(x_sel @ w_gate)
        u = x_sel @ w_up
        y = g * u @ w_down
        r_sel = _sigmoid(jnp.take_along_axis(r, idx, axis=1))
        y = y * r_sel.reshape(B, C, 1)
        b_off = (jnp.arange(B) * S).reshape(B, 1)
        flat_idx = (idx + b_off).reshape(B * C)
        zero = (x * 0.0).reshape(B * S, D)
        upd = _scatter_add(zero, flat_idx, y.reshape(B * C, D), axis=0)
        return x + upd.reshape(B, S, D)
    x = A_x
    x = x + _A_ref(_layernorm(x, axis=-1), A_wq, A_wk, A_wv, A_wo, A_beta)
    x = x + _B_ref(_layernorm(x, axis=-1), B_w_r, B_w_gate, B_w_up, B_w_down)
    x = x + _A_ref(_layernorm(x, axis=-1), A_wq, A_wk, A_wv, A_wo, A_beta)
    x = x + _B_ref(_layernorm(x, axis=-1), B_w_r, B_w_gate, B_w_up, B_w_down)
    return x
```

```python
import jax
import jax.numpy as jnp
import jax.experimental.pallas as pl
import jax.experimental.pallas.tpu as pltpu

F32 = jnp.float32
BF16 = jnp.bfloat16

S = 2048
D = 1024
H = 32
DH = 32
NSEG = 4
L = S // NSEG
NG = 8
FF = 3584
FCH = 512
NFC = FF // FCH
LOG2E = 1.4426950408889634
QSCALE = (DH ** -0.5) * LOG2E
NEG = -1000000000.0 * LOG2E
EPS_LN = 1.0013580322265625e-05
NT = (((1,), (1,)), ((), ()))


def _rb(t):
    return t.astype(BF16).astype(F32)


def _ln_f32(x):
    mu = jnp.sum(x, axis=1, keepdims=True) * (1.0 / D)
    xc = x - mu
    var = jnp.sum(xc * xc, axis=1, keepdims=True) * (1.0 / D)
    sd = _rb(jnp.sqrt(_rb(_rb(var) + EPS_LN)))
    return (x - _rb(mu)) * (1.0 / sd)


def _phi(t):
    return jnp.where(t > 0, t + 1.0, jnp.exp(t))


def _kernel(x_hbm, wq_hbm, wk_hbm, wv_hbm, wo_hbm, beta_ref, wr_ref, wg_hbm, wu_hbm, wd_hbm,
            out_hbm,
            R, T, XN, W, WO, WG, WU, WD, OB, MST, RC, GT, WR, CM,
            K0, Q0, PQ0, PK0, VT0, K1, Q1, PQ1, PK1, VT1,
            sx, sw, sm, so):
    bufs = ((K0, Q0, PQ0, PK0, VT0), (K1, Q1, PQ1, PK1, VT1))

    def x_copy(s):
        return pltpu.make_async_copy(x_hbm.at[0, pl.ds(s * L, L), :], R.at[pl.ds(s * L, L), :], sx.at[s])

    def w_copy(g, j):
        src = (wq_hbm, wk_hbm, wv_hbm)[j]
        return pltpu.make_async_copy(src.at[:, pl.ds(g * 128, 128)],
                                     W.at[g, :, pl.ds(j * 128, 128)], sw.at[g, j])

    misc = (pltpu.make_async_copy(wo_hbm, WO, sm.at[0]),
            pltpu.make_async_copy(wg_hbm, WG, sm.at[1]),
            pltpu.make_async_copy(wu_hbm, WU, sm.at[2]),
            pltpu.make_async_copy(wd_hbm, WD, sm.at[3]))

    def out_copy(s):
        return pltpu.make_async_copy(R.at[pl.ds(s * L, L), :], out_hbm.at[0, pl.ds(s * L, L), :], so.at[s])

    x_copy(0).start()
    for g in range(NG):
        for j in range(3):
            w_copy(g, j).start()
    x_copy(1).start()
    misc[0].start()
    x_copy(2).start()
    x_copy(3).start()
    misc[1].start()
    misc[2].start()
    misc[3].start()

    gsig = jax.nn.sigmoid(beta_ref[...].astype(F32).reshape(1, H))
    eye = (jax.lax.broadcasted_iota(jnp.int32, (H, H), 0)
           == jax.lax.broadcasted_iota(jnp.int32, (H, H), 1))
    gcol = jnp.sum(jnp.where(eye, jnp.broadcast_to(gsig, (H, H)), 0.0), axis=1, keepdims=True)
    gfull = jnp.broadcast_to(gcol, (H, 128))
    for g in range(NG):
        GT[g, 0:4, :] = gfull[4 * g:4 * g + 4, :]
        GT[g, 4:8, :] = 1.0 - gfull[4 * g:4 * g + 4, :]
    WR[...] = wr_ref[...].astype(F32).reshape(1, D)
    kk = jax.lax.broadcasted_iota(jnp.int32, (128, 128), 0)
    qq = jax.lax.broadcasted_iota(jnp.int32, (128, 128), 1)
    CM[...] = jnp.where(qq < kk, NEG, 0.0).astype(F32)
    VT0[128:144, :] = jnp.ones((16, L), BF16)
    VT1[128:144, :] = jnp.ones((16, L), BF16)

    def ln1(row0, n):
        x = R[pl.ds(row0, n), :].astype(F32)
        XN[pl.ds(row0, n), :] = _ln_f32(x).astype(BF16)

    def proj(seg, g, buf):
        Kb, Qm, PQ, PK, VT = buf
        row0 = pl.multiple_of(seg * L, L)
        acc = jnp.dot(XN[pl.ds(row0, L), :], W[g], preferred_element_type=F32)
        q = acc[:, 0:128]
        k = acc[:, 128:256]
        v = acc[:, 256:384]
        Kb[...] = k.astype(BF16)
        qs = q * QSCALE
        lh = jax.lax.broadcasted_iota(jnp.int32, (L, 128), 1) // DH
        for h in range(4):
            Qm[h] = jnp.where(lh == h, qs, 0.0).astype(BF16)
        PQ[...] = _phi(q).astype(BF16)
        PK[...] = _phi(k).astype(BF16)
        VT[0:128, :] = v.astype(BF16).T

    def attn(seg, g, buf):
        Kb, Qm, PQ, PK, VT = buf
        st = jnp.where(seg > 0, MST[g], 0.0)
        rd = jax.lax.dot_general(st.astype(BF16), PQ[...], NT, preferred_element_type=F32)
        upd = jnp.dot(VT[...], PK[...], preferred_element_type=F32)
        rr = jax.lax.broadcasted_iota(jnp.int32, (144, 128), 0)
        cc = jax.lax.broadcasted_iota(jnp.int32, (144, 128), 1) // DH
        keep = jnp.where(rr < 128, rr // DH, rr - 128) == cc
        MST[g] = st + jnp.where(keep, upd, 0.0)
        gt = GT[g]
        for qb in range(4):
            nk = 128 * (qb + 1)
            q0 = 128 * qb
            parts = []
            for h in range(4):
                s = jax.lax.dot_general(Kb[0:nk, :], Qm[h, q0:q0 + 128, :], NT,
                                        preferred_element_type=F32)
                sd = s[q0:nk, :] + CM[...]
                if qb > 0:
                    s = jnp.concatenate([s[0:q0, :], sd], axis=0)
                else:
                    s = sd
                m = jnp.max(s, axis=0, keepdims=True)
                p = jnp.exp2(s - m)
                l = jnp.sum(p, axis=0, keepdims=True)
                pv = jnp.dot(VT[32 * h:32 * h + 32, 0:nk], p.astype(BF16),
                             preferred_element_type=F32)
                den = rd[128 + h:129 + h, q0:nk] + 1e-06
                o = (rd[32 * h:32 * h + 32, q0:nk] * (gt[h:h + 1, :] / den)
                     + pv * (gt[4 + h:5 + h, :] / l))
                parts.append(o)
            ot = jnp.concatenate(parts, axis=0)
            OB[g, q0:nk, :] = ot.astype(BF16).T

    def ophase(seg):
        for c in range(4):
            row0 = pl.multiple_of(seg * L + c * 128, 128)
            o = jnp.concatenate([OB[g, c * 128:(c + 1) * 128, :] for g in range(NG)], axis=1)
            a = jnp.dot(o, WO[...], preferred_element_type=F32)
            x1b = (R[pl.ds(row0, 128), :].astype(F32) + _rb(a)).astype(BF16)
            T[pl.ds(row0, 128), :] = x1b
            x1 = x1b.astype(F32)
            y = _rb(_ln_f32(x1))
            RC[pl.ds(row0, 128), :] = _rb(jnp.sum(y * WR[...], axis=1, keepdims=True))
            R[pl.ds(row0, 128), :] = (x1 + y).astype(BF16)

    def ffn_patch(layer):
        r = RC[...]
        idx = jax.lax.broadcasted_iota(jnp.int32, (S, 1), 0)
        m1 = jnp.max(r, axis=0, keepdims=True)
        i1 = jnp.min(jnp.where(r == m1, idx, S - 1))
        r2 = jnp.where(idx == i1, -jnp.inf, r)
        m2 = jnp.max(r2, axis=0, keepdims=True)
        i2 = jnp.min(jnp.where((r2 == m2) & (idx != i1), idx, S - 1))
        b1 = pl.multiple_of((jnp.clip(i1, 0, S - 1) // 16) * 16, 16)
        b2 = pl.multiple_of((jnp.clip(i2, 0, S - 1) // 16) * 16, 16)
        x1 = jnp.concatenate([T[pl.ds(b1, 16), :], T[pl.ds(b2, 16), :]], axis=0).astype(F32)
        yb = _ln_f32(x1).astype(BF16)
        rsel = jnp.concatenate([RC[pl.ds(b1, 16), :], RC[pl.ds(b2, 16), :]], axis=0)

        def fbody(c, acc):
            c0 = pl.multiple_of(c * FCH, FCH)
            gt = _rb(jnp.dot(yb, WG[:, pl.ds(c0, FCH)], preferred_element_type=F32))
            up = _rb(jnp.dot(yb, WU[:, pl.ds(c0, FCH)], preferred_element_type=F32))
            hm = (_rb(gt * _rb(jax.nn.sigmoid(gt))) * up).astype(BF16)
            return acc + jnp.dot(hm, WD[pl.ds(c0, FCH), :], preferred_element_type=F32)

        yv = jax.lax.fori_loop(0, NFC, fbody, jnp.zeros((32, D), F32))
        yv = _rb(_rb(yv) * _rb(jax.nn.sigmoid(rsel)))
        i16 = jax.lax.broadcasted_iota(jnp.int32, (16, 1), 0)
        rows = jnp.concatenate([i16 + b1, i16 + b2], axis=0)
        upd = jnp.where((rows == i1) | (rows == i2), yv, 0.0)
        x2b = (x1 + _rb(yb.astype(F32) + upd)).astype(BF16)
        xnb = _ln_f32(x2b.astype(F32)).astype(BF16)

        @pl.when(layer == 1)
        def _():
            for s in range(NSEG):
                out_copy(s).wait()

        R[pl.ds(b1, 16), :] = x2b[0:16]
        R[pl.ds(b2, 16), :] = x2b[16:32]
        XN[pl.ds(b1, 16), :] = xnb[0:16]
        XN[pl.ds(b2, 16), :] = xnb[16:32]

        @pl.when(layer == 1)
        def _():
            c1 = pltpu.make_async_copy(R.at[pl.ds(b1, 16), :], out_hbm.at[0, pl.ds(b1, 16), :], so.at[0])
            c1.start()

            @pl.when(b2 != b1)
            def _():
                c2 = pltpu.make_async_copy(R.at[pl.ds(b2, 16), :], out_hbm.at[0, pl.ds(b2, 16), :], so.at[1])
                c2.start()
                c2.wait()

            c1.wait()

    x_copy(0).wait()
    ln1(0, L)
    for j in range(3):
        w_copy(0, j).wait()

    def layer_body(layer, carry):
        proj(0, 0, bufs[0])

        def seg_body(seg, carry2):
            first = jnp.logical_and(layer == 0, seg == 0)
            nxt = (seg + 1) % NSEG

            @pl.when(jnp.logical_and(layer == 0, seg < NSEG - 1))
            def _():
                pltpu.make_async_copy(x_hbm.at[0, pl.ds(0, L), :], R.at[pl.ds(0, L), :], sx.at[nxt]).wait()

            def gp_body(gp, carry3):
                g0 = 2 * gp
                g1 = g0 + 1
                g2 = (g0 + 2) % NG

                @pl.when(first)
                def _():
                    for j in range(3):
                        pltpu.make_async_copy(wq_hbm.at[:, pl.ds(0, 128)], W.at[0, :, pl.ds(0, 128)],
                                              sw.at[g1, j]).wait()

                    @pl.when(gp < NG // 2 - 1)
                    def _():
                        for j in range(3):
                            pltpu.make_async_copy(wq_hbm.at[:, pl.ds(0, 128)], W.at[0, :, pl.ds(0, 128)],
                                                  sw.at[g2, j]).wait()

                attn(seg, g0, bufs[0])
                proj(seg, g1, bufs[1])
                ln1(pl.multiple_of(nxt * L + gp * 128, 128), 128)
                attn(seg, g1, bufs[1])
                proj(jnp.where(gp == NG // 2 - 1, nxt, seg), g2, bufs[0])
                return carry3

            jax.lax.fori_loop(0, NG // 2, gp_body, 0)

            @pl.when(first)
            def _():
                misc[0].wait()

            ophase(seg)

            @pl.when(layer == 1)
            def _():
                row0 = pl.multiple_of(seg * L, L)
                pltpu.make_async_copy(R.at[pl.ds(row0, L), :], out_hbm.at[0, pl.ds(row0, L), :],
                                      so.at[seg]).start()

            return carry2

        jax.lax.fori_loop(0, NSEG, seg_body, 0)

        @pl.when(layer == 0)
        def _():
            misc[1].wait()
            misc[2].wait()
            misc[3].wait()

        ffn_patch(layer)
        return carry

    jax.lax.fori_loop(0, 2, layer_body, 0)


@jax.jit
def pallas_interleave_layers__memory_aug_infini_attn__moe_arch_mod__prompt_kernel(
    A_x: jax.Array,
    A_wq: jax.Array,
    A_wk: jax.Array,
    A_wv: jax.Array,
    A_wo: jax.Array,
    A_beta: jax.Array,
    B_x: jax.Array,
    B_w_r: jax.Array,
    B_w_gate: jax.Array,
    B_w_up: jax.Array,
    B_w_down: jax.Array,
):
    hbm = pl.BlockSpec(memory_space=pl.ANY)
    vmem = pl.BlockSpec(memory_space=pltpu.VMEM)
    qkv_set = [
        pltpu.VMEM((L, 128), BF16),
        pltpu.VMEM((4, L, 128), BF16),
        pltpu.VMEM((L, 128), BF16),
        pltpu.VMEM((L, 128), BF16),
        pltpu.VMEM((144, L), BF16),
    ]
    scratch = [
        pltpu.VMEM((S, D), BF16),
        pltpu.VMEM((S, D), BF16),
        pltpu.VMEM((S, D), BF16),
        pltpu.VMEM((NG, D, 384), BF16),
        pltpu.VMEM((D, D), BF16),
        pltpu.VMEM((D, FF), BF16),
        pltpu.VMEM((D, FF), BF16),
        pltpu.VMEM((FF, D), BF16),
        pltpu.VMEM((NG, L, 128), BF16),
        pltpu.VMEM((NG, 144, 128), F32),
        pltpu.VMEM((S, 1), F32),
        pltpu.VMEM((NG, 8, 128), F32),
        pltpu.VMEM((1, D), F32),
        pltpu.VMEM((128, 128), F32),
    ] + qkv_set + qkv_set + [
        pltpu.SemaphoreType.DMA((NSEG,)),
        pltpu.SemaphoreType.DMA((NG, 3)),
        pltpu.SemaphoreType.DMA((4,)),
        pltpu.SemaphoreType.DMA((NSEG,)),
    ]
    return pl.pallas_call(
        _kernel,
        out_shape=jax.ShapeDtypeStruct((1, S, D), BF16),
        in_specs=[hbm, hbm, hbm, hbm, hbm, vmem, vmem, hbm, hbm, hbm],
        out_specs=hbm,
        scratch_shapes=scratch,
        compiler_params=pltpu.CompilerParams(vmem_limit_bytes=100 * 1024 * 1024),
    )(A_x, A_wq, A_wk, A_wv, A_wo, A_beta, B_w_r, B_w_gate, B_w_up, B_w_down)
```

```python
import jax
import jax.numpy as jnp
import jax.experimental.pallas as pl
import jax.experimental.pallas.tpu as pltpu

F32 = jnp.float32
BF16 = jnp.bfloat16

S = 2048
D = 1024
H = 32
DH = 32
NSEG = 4
L = S // NSEG
NG = 8
FF = 3584
FCH = 512
NFC = FF // FCH
LOG2E = 1.4426950408889634
QSCALE = (DH ** -0.5) * LOG2E
NEG = -1000000000.0 * LOG2E
EPS_LN = 1.0013580322265625e-05
NT = (((1,), (1,)), ((), ()))


def _rb(t):
    return t.astype(BF16).astype(F32)


def _ln_f32(x):
    mu = jnp.sum(x, axis=1, keepdims=True) * (1.0 / D)
    xc = x - mu
    var = jnp.sum(xc * xc, axis=1, keepdims=True) * (1.0 / D)
    sd = _rb(jnp.sqrt(_rb(_rb(var) + EPS_LN)))
    return (x - _rb(mu)) * (1.0 / sd)


def _phi(t):
    return jnp.where(t > 0, t + 1.0, jnp.exp(t))


def _kernel(x_hbm, wq_hbm, wk_hbm, wv_hbm, wo_hbm, beta_ref, wr_ref, wg_hbm, wu_hbm, wd_hbm,
            out_hbm,
            R, T, XN, W, WO, WG, WU, WD, OB, MST, RC, GT, WR, CM,
            K0, Q0, PQ0, PK0, VT0, K1, Q1, PQ1, PK1, VT1,
            sx, sw, sm, so):
    bufs = ((K0, Q0, PQ0, PK0, VT0), (K1, Q1, PQ1, PK1, VT1))

    def x_copy(s):
        return pltpu.make_async_copy(x_hbm.at[0, pl.ds(s * L, L), :], R.at[pl.ds(s * L, L), :], sx.at[s])

    def w_copy(g, j):
        src = (wq_hbm, wk_hbm, wv_hbm)[j]
        return pltpu.make_async_copy(src.at[:, pl.ds(g * 128, 128)],
                                     W.at[g, :, pl.ds(j * 128, 128)], sw.at[g, j])

    misc = (pltpu.make_async_copy(wo_hbm, WO, sm.at[0]),
            pltpu.make_async_copy(wg_hbm, WG, sm.at[1]),
            pltpu.make_async_copy(wu_hbm, WU, sm.at[2]),
            pltpu.make_async_copy(wd_hbm, WD, sm.at[3]))

    def out_copy(s):
        return pltpu.make_async_copy(R.at[pl.ds(s * L, L), :], out_hbm.at[0, pl.ds(s * L, L), :], so.at[s])

    x_copy(0).start()
    for g in range(NG):
        for j in range(3):
            w_copy(g, j).start()
    x_copy(1).start()
    misc[0].start()
    x_copy(2).start()
    x_copy(3).start()
    misc[1].start()
    misc[2].start()
    misc[3].start()

    gsig = jax.nn.sigmoid(beta_ref[...].astype(F32).reshape(1, H))
    eye = (jax.lax.broadcasted_iota(jnp.int32, (H, H), 0)
           == jax.lax.broadcasted_iota(jnp.int32, (H, H), 1))
    gcol = jnp.sum(jnp.where(eye, jnp.broadcast_to(gsig, (H, H)), 0.0), axis=1, keepdims=True)
    gfull = jnp.broadcast_to(gcol, (H, 128))
    for g in range(NG):
        GT[g, 0:4, :] = gfull[4 * g:4 * g + 4, :]
        GT[g, 4:8, :] = 1.0 - gfull[4 * g:4 * g + 4, :]
    WR[...] = wr_ref[...].astype(F32).reshape(1, D)
    kk = jax.lax.broadcasted_iota(jnp.int32, (128, 128), 0)
    qq = jax.lax.broadcasted_iota(jnp.int32, (128, 128), 1)
    CM[...] = jnp.where(qq < kk, NEG, 0.0).astype(F32)
    for c in range(4):
        VT0[c, 128:144, :] = jnp.ones((16, 128), BF16)
        VT1[c, 128:144, :] = jnp.ones((16, 128), BF16)

    def ln1(row0, n):
        x = R[pl.ds(row0, n), :].astype(F32)
        XN[pl.ds(row0, n), :] = _ln_f32(x).astype(BF16)

    def proj_chunk(seg, g, buf, c):
        Kb, Qm, PQ, PK, VT = buf
        row0 = pl.multiple_of(seg * L + c * 128, 128)
        acc = jnp.dot(XN[pl.ds(row0, 128), :], W[g], preferred_element_type=F32)
        q = acc[:, 0:128]
        k = acc[:, 128:256]
        v = acc[:, 256:384]
        qs = q * QSCALE
        lh = jax.lax.broadcasted_iota(jnp.int32, (128, 128), 1) // DH
        for h in range(4):
            Qm[c, h * 128:(h + 1) * 128, :] = jnp.where(lh == h, qs, 0.0).astype(BF16)
        PQ[c * 128:(c + 1) * 128, :] = _phi(q).astype(BF16)
        Kb[c * 128:(c + 1) * 128, :] = k.astype(BF16)
        PK[c * 128:(c + 1) * 128, :] = _phi(k).astype(BF16)
        VT[c, 0:128, :] = v.astype(BF16).T

    def proj(seg, g, buf):
        for c in range(4):
            proj_chunk(seg, g, buf, c)

    def step(seg, g, buf, pseg, pg, pbuf, filler=None):
        Kb, Qm, PQ, PK, VT = buf
        gt = GT[g]

        def qk(qb):
            nk = 128 * (qb + 1)
            q0 = 128 * qb
            s = jax.lax.dot_general(Kb[0:nk, :], Qm[qb], NT, preferred_element_type=F32)
            cm = CM[...]
            sd = s[q0:nk, :] + jnp.concatenate([cm, cm, cm, cm], axis=1)
            if qb > 0:
                s = jnp.concatenate([s[0:q0, :], sd], axis=0)
            else:
                s = sd
            m = jnp.max(s, axis=0, keepdims=True)
            p = jnp.exp2(s - m)
            l = jnp.sum(p, axis=0, keepdims=True)
            return p.astype(BF16), l

        def pv(qb, pl_, rd):
            p, l = pl_
            nk = 128 * (qb + 1)
            q0 = 128 * qb
            parts = []
            for h in range(4):
                vt = jnp.concatenate([VT[c, 32 * h:32 * h + 32, :] for c in range(qb + 1)], axis=1)
                o = jnp.dot(vt, p[:, 128 * h:128 * (h + 1)], preferred_element_type=F32)
                den = rd[128 + h:129 + h, q0:nk] + 1e-06
                parts.append(rd[32 * h:32 * h + 32, q0:nk] * (gt[h:h + 1, :] / den)
                             + o * (gt[4 + h:5 + h, :] / l[:, 128 * h:128 * (h + 1)]))
            ot = jnp.concatenate(parts, axis=0)
            OB[g, q0:nk, :] = ot.astype(BF16).T

        a0 = qk(0)
        a1 = qk(1)
        proj_chunk(pseg, pg, pbuf, 0)
        st = jnp.where(seg > 0, MST[g], 0.0)
        rd = jax.lax.dot_general(st.astype(BF16), PQ[...], NT, preferred_element_type=F32)
        a2 = qk(2)
        pv(0, a0, rd)
        pv(1, a1, rd)
        proj_chunk(pseg, pg, pbuf, 1)
        a3 = qk(3)
        pv(2, a2, rd)
        vall = jnp.concatenate([VT[c] for c in range(4)], axis=1)
        upd = jnp.dot(vall, PK[...], preferred_element_type=F32)
        rr = jax.lax.broadcasted_iota(jnp.int32, (144, 128), 0)
        cc = jax.lax.broadcasted_iota(jnp.int32, (144, 128), 1) // DH
        keep = jnp.where(rr < 128, rr // DH, rr - 128) == cc
        MST[g] = st + jnp.where(keep, upd, 0.0)
        proj_chunk(pseg, pg, pbuf, 2)
        pv(3, a3, rd)
        if filler is not None:
            filler()
        proj_chunk(pseg, pg, pbuf, 3)

    def ophase(seg):
        for c in range(4):
            row0 = pl.multiple_of(seg * L + c * 128, 128)
            o = jnp.concatenate([OB[g, c * 128:(c + 1) * 128, :] for g in range(NG)], axis=1)
            a = jnp.dot(o, WO[...], preferred_element_type=F32)
            x1b = (R[pl.ds(row0, 128), :].astype(F32) + _rb(a)).astype(BF16)
            T[pl.ds(row0, 128), :] = x1b
            x1 = x1b.astype(F32)
            y = _rb(_ln_f32(x1))
            RC[pl.ds(row0, 128), :] = _rb(jnp.sum(y * WR[...], axis=1, keepdims=True))
            R[pl.ds(row0, 128), :] = (x1 + y).astype(BF16)

    def ffn_patch(layer):
        r = RC[...]
        idx = jax.lax.broadcasted_iota(jnp.int32, (S, 1), 0)
        m1 = jnp.max(r, axis=0, keepdims=True)
        i1 = jnp.min(jnp.where(r == m1, idx, S - 1))
        r2 = jnp.where(idx == i1, -jnp.inf, r)
        m2 = jnp.max(r2, axis=0, keepdims=True)
        i2 = jnp.min(jnp.where((r2 == m2) & (idx != i1), idx, S - 1))
        b1 = pl.multiple_of((jnp.clip(i1, 0, S - 1) // 16) * 16, 16)
        b2 = pl.multiple_of((jnp.clip(i2, 0, S - 1) // 16) * 16, 16)
        x1 = jnp.concatenate([T[pl.ds(b1, 16), :], T[pl.ds(b2, 16), :]], axis=0).astype(F32)
        yb = _ln_f32(x1).astype(BF16)
        rsel = jnp.concatenate([RC[pl.ds(b1, 16), :], RC[pl.ds(b2, 16), :]], axis=0)

        def fbody(c, acc):
            c0 = pl.multiple_of(c * FCH, FCH)
            gt = _rb(jnp.dot(yb, WG[:, pl.ds(c0, FCH)], preferred_element_type=F32))
            up = _rb(jnp.dot(yb, WU[:, pl.ds(c0, FCH)], preferred_element_type=F32))
            hm = (_rb(gt * _rb(jax.nn.sigmoid(gt))) * up).astype(BF16)
            return acc + jnp.dot(hm, WD[pl.ds(c0, FCH), :], preferred_element_type=F32)

        yv = jax.lax.fori_loop(0, NFC, fbody, jnp.zeros((32, D), F32))
        yv = _rb(_rb(yv) * _rb(jax.nn.sigmoid(rsel)))
        i16 = jax.lax.broadcasted_iota(jnp.int32, (16, 1), 0)
        rows = jnp.concatenate([i16 + b1, i16 + b2], axis=0)
        upd = jnp.where((rows == i1) | (rows == i2), yv, 0.0)
        x2b = (x1 + _rb(yb.astype(F32) + upd)).astype(BF16)
        xnb = _ln_f32(x2b.astype(F32)).astype(BF16)

        @pl.when(layer == 1)
        def _():
            for s in range(NSEG):
                out_copy(s).wait()

        R[pl.ds(b1, 16), :] = x2b[0:16]
        R[pl.ds(b2, 16), :] = x2b[16:32]
        XN[pl.ds(b1, 16), :] = xnb[0:16]
        XN[pl.ds(b2, 16), :] = xnb[16:32]

        @pl.when(layer == 1)
        def _():
            c1 = pltpu.make_async_copy(R.at[pl.ds(b1, 16), :], out_hbm.at[0, pl.ds(b1, 16), :], so.at[0])
            c1.start()

            @pl.when(b2 != b1)
            def _():
                c2 = pltpu.make_async_copy(R.at[pl.ds(b2, 16), :], out_hbm.at[0, pl.ds(b2, 16), :], so.at[1])
                c2.start()
                c2.wait()

            c1.wait()

    x_copy(0).wait()
    ln1(0, L)
    for j in range(3):
        w_copy(0, j).wait()

    def layer_body(layer, carry):
        proj(0, 0, bufs[0])

        def seg_body(seg, carry2):
            first = jnp.logical_and(layer == 0, seg == 0)
            nxt = (seg + 1) % NSEG

            @pl.when(jnp.logical_and(layer == 0, seg < NSEG - 1))
            def _():
                pltpu.make_async_copy(x_hbm.at[0, pl.ds(0, L), :], R.at[pl.ds(0, L), :], sx.at[nxt]).wait()

            def gp_body(gp, carry3):
                g0 = 2 * gp
                g1 = g0 + 1
                g2 = (g0 + 2) % NG

                @pl.when(first)
                def _():
                    for j in range(3):
                        pltpu.make_async_copy(wq_hbm.at[:, pl.ds(0, 128)], W.at[0, :, pl.ds(0, 128)],
                                              sw.at[g1, j]).wait()

                    @pl.when(gp < NG // 2 - 1)
                    def _():
                        for j in range(3):
                            pltpu.make_async_copy(wq_hbm.at[:, pl.ds(0, 128)], W.at[0, :, pl.ds(0, 128)],
                                                  sw.at[g2, j]).wait()

                step(seg, g0, bufs[0], seg, g1, bufs[1],
                     lambda: ln1(pl.multiple_of(nxt * L + gp * 128, 128), 128))
                step(seg, g1, bufs[1], jnp.where(gp == NG // 2 - 1, nxt, seg), g2, bufs[0])
                return carry3

            jax.lax.fori_loop(0, NG // 2, gp_body, 0)

            @pl.when(first)
            def _():
                misc[0].wait()

            ophase(seg)

            @pl.when(layer == 1)
            def _():
                row0 = pl.multiple_of(seg * L, L)
                pltpu.make_async_copy(R.at[pl.ds(row0, L), :], out_hbm.at[0, pl.ds(row0, L), :],
                                      so.at[seg]).start()

            return carry2

        jax.lax.fori_loop(0, NSEG, seg_body, 0)

        @pl.when(layer == 0)
        def _():
            misc[1].wait()
            misc[2].wait()
            misc[3].wait()

        ffn_patch(layer)
        return carry

    jax.lax.fori_loop(0, 2, layer_body, 0)


@jax.jit
def pallas_interleave_layers__memory_aug_infini_attn__moe_arch_mod__prompt_kernel(
    A_x: jax.Array,
    A_wq: jax.Array,
    A_wk: jax.Array,
    A_wv: jax.Array,
    A_wo: jax.Array,
    A_beta: jax.Array,
    B_x: jax.Array,
    B_w_r: jax.Array,
    B_w_gate: jax.Array,
    B_w_up: jax.Array,
    B_w_down: jax.Array,
):
    hbm = pl.BlockSpec(memory_space=pl.ANY)
    vmem = pl.BlockSpec(memory_space=pltpu.VMEM)
    qkv_set = [
        pltpu.VMEM((L, 128), BF16),
        pltpu.VMEM((4, L, 128), BF16),
        pltpu.VMEM((L, 128), BF16),
        pltpu.VMEM((L, 128), BF16),
        pltpu.VMEM((4, 144, 128), BF16),
    ]
    scratch = [
        pltpu.VMEM((S, D), BF16),
        pltpu.VMEM((S, D), BF16),
        pltpu.VMEM((S, D), BF16),
        pltpu.VMEM((NG, D, 384), BF16),
        pltpu.VMEM((D, D), BF16),
        pltpu.VMEM((D, FF), BF16),
        pltpu.VMEM((D, FF), BF16),
        pltpu.VMEM((FF, D), BF16),
        pltpu.VMEM((NG, L, 128), BF16),
        pltpu.VMEM((NG, 144, 128), F32),
        pltpu.VMEM((S, 1), F32),
        pltpu.VMEM((NG, 8, 128), F32),
        pltpu.VMEM((1, D), F32),
        pltpu.VMEM((128, 128), F32),
    ] + qkv_set + qkv_set + [
        pltpu.SemaphoreType.DMA((NSEG,)),
        pltpu.SemaphoreType.DMA((NG, 3)),
        pltpu.SemaphoreType.DMA((4,)),
        pltpu.SemaphoreType.DMA((NSEG,)),
    ]
    return pl.pallas_call(
        _kernel,
        out_shape=jax.ShapeDtypeStruct((1, S, D), BF16),
        in_specs=[hbm, hbm, hbm, hbm, hbm, vmem, vmem, hbm, hbm, hbm],
        out_specs=hbm,
        scratch_shapes=scratch,
        compiler_params=pltpu.CompilerParams(vmem_limit_bytes=100 * 1024 * 1024),
    )(A_x, A_wq, A_wk, A_wv, A_wo, A_beta, B_w_r, B_w_gate, B_w_up, B_w_down)
```

```python
import functools

import jax
import jax.numpy as jnp
import jax.experimental.pallas as pl
import jax.experimental.pallas.tpu as pltpu

F32 = jnp.float32
BF16 = jnp.bfloat16

S = 2048
D = 1024
H = 32
DH = 32
NSEG = 4
L = S // NSEG
NG = 8
FF = 3584
FCH = 512
NFC = FF // FCH
LOG2E = 1.4426950408889634
QSCALE = (DH ** -0.5) * LOG2E
NEG = -1000000000.0 * LOG2E
EPS_LN = 1.0013580322265625e-05
NT = (((1,), (1,)), ((), ()))
SCHED = ("Q0 Q1 R G0 P G1 P P G2 Q2 P P G3 P P G4 P P G5 Q3 P P G6 P P G7 P P G8 P P G9 F "
         "P P P P P P P U")


def _rb(t):
    return t.astype(BF16).astype(F32)


def _ln_f32(x):
    mu = jnp.sum(x, axis=1, keepdims=True) * (1.0 / D)
    xc = x - mu
    var = jnp.sum(xc * xc, axis=1, keepdims=True) * (1.0 / D)
    sd = _rb(jnp.sqrt(_rb(_rb(var) + EPS_LN)))
    return (x - _rb(mu)) * (1.0 / sd)


def _phi(t):
    return jnp.where(t > 0, t + 1.0, jnp.exp(t))


def _kernel(x_hbm, wq_hbm, wk_hbm, wv_hbm, wo_hbm, beta_ref, wr_ref, wg_hbm, wu_hbm, wd_hbm,
            out_hbm,
            R, T, XN, W, WO, WG, WU, WD, OB, MST, RC, GT, WR, CM,
            K0, Q0, PQ0, PK0, VT0, SA0, SB0, SC0, SD0, RD0, K1, Q1, PQ1, PK1, VT1, SA1, SB1, SC1, SD1, RD1,
            ZS, sx, sw, sm, so):
    bufs = ((K0, Q0, PQ0, PK0, VT0, (SA0, SB0, SC0, SD0), RD0), (K1, Q1, PQ1, PK1, VT1, (SA1, SB1, SC1, SD1), RD1))
    ZS[0] = 0
    XNu = XN.bitcast(jnp.uint32)
    Wu = W.bitcast(jnp.uint32)

    def x_copy(s):
        return pltpu.make_async_copy(x_hbm.at[0, pl.ds(s * L, L), :], R.at[pl.ds(s * L, L), :], sx.at[s])

    def w_copy(g, j):
        src = (wq_hbm, wk_hbm, wv_hbm)[j]
        return pltpu.make_async_copy(src.at[:, pl.ds(g * 128, 128)],
                                     W.at[g, j], sw.at[g, j])

    misc = (pltpu.make_async_copy(wo_hbm, WO, sm.at[0]),
            pltpu.make_async_copy(wg_hbm, WG, sm.at[1]),
            pltpu.make_async_copy(wu_hbm, WU, sm.at[2]),
            pltpu.make_async_copy(wd_hbm, WD, sm.at[3]))

    def out_copy(s):
        return pltpu.make_async_copy(R.at[pl.ds(s * L, L), :], out_hbm.at[0, pl.ds(s * L, L), :], so.at[s])

    x_copy(0).start()
    for g in range(NG):
        for j in range(3):
            w_copy(g, j).start()
    x_copy(1).start()
    misc[0].start()
    x_copy(2).start()
    x_copy(3).start()
    misc[1].start()
    misc[2].start()
    misc[3].start()

    gsig = jax.nn.sigmoid(beta_ref[...].astype(F32).reshape(1, H))
    eye = (jax.lax.broadcasted_iota(jnp.int32, (H, H), 0)
           == jax.lax.broadcasted_iota(jnp.int32, (H, H), 1))
    gcol = jnp.sum(jnp.where(eye, jnp.broadcast_to(gsig, (H, H)), 0.0), axis=1, keepdims=True)
    gfull = jnp.broadcast_to(gcol, (H, 128))
    for g in range(NG):
        GT[g, 0:4, :] = gfull[4 * g:4 * g + 4, :]
        GT[g, 4:8, :] = 1.0 - gfull[4 * g:4 * g + 4, :]
    WR[...] = wr_ref[...].astype(F32).reshape(1, D)
    kk = jax.lax.broadcasted_iota(jnp.int32, (128, 128), 0)
    qq = jax.lax.broadcasted_iota(jnp.int32, (128, 128), 1)
    CM[...] = jnp.where(qq < kk, NEG, 0.0).astype(F32)
    for c in range(4):
        VT0[c, 128:144, :] = jnp.ones((16, 128), BF16)
        VT1[c, 128:144, :] = jnp.ones((16, 128), BF16)

    def ln1(row0, n):
        x = R[pl.ds(row0, n), :].astype(F32)
        y = _ln_f32(x).astype(BF16)
        for k in range(8):
            XN[k, pl.ds(row0, n), :] = y[:, k * 128:(k + 1) * 128]

    def proj_rounds(seg, g, buf):
        Kb, Qm, PQ, PK, VT, SB, RD = buf
        zz = ZS[0]
        part = {}

        def rnd(c, j, half):
            r2 = pl.multiple_of(seg * (L // 2) + c * 64 + zz * j, 64)
            xn = jnp.concatenate([pltpu.bitcast(XNu[k, pl.ds(r2, 64), :], BF16)
                                  for k in range(4 * half, 4 * half + 4)], axis=1)
            w = pltpu.bitcast(Wu[g, j, 256 * half:256 * half + 256, :], BF16)
            t = jnp.dot(xn, w, preferred_element_type=F32)
            if half == 0:
                part[0] = t
                return
            t = part[0] + t
            if j == 0:
                qs = t * QSCALE
                lh = jax.lax.broadcasted_iota(jnp.int32, (128, 128), 1) // DH
                for h in range(4):
                    Qm[c, h * 128:(h + 1) * 128, :] = jnp.where(lh == h, qs, 0.0).astype(BF16)
                PQ[c * 128:(c + 1) * 128, :] = _phi(t).astype(BF16)
            elif j == 1:
                Kb[c * 128:(c + 1) * 128, :] = t.astype(BF16)
                PK[c * 128:(c + 1) * 128, :] = _phi(t).astype(BF16)
            else:
                VT[c, 0:128, :] = t.astype(BF16).T

        return [functools.partial(rnd, c, j, half) for c in range(4) for j in range(3) for half in range(2)]

    def proj(seg, g, buf):
        for f in proj_rounds(seg, g, buf):
            f()

    def step(seg, g, buf, pseg, pg, pbuf, filler=None):
        Kb, Qm, PQ, PK, VT, SB, RD = buf
        gt = GT[g]
        zz = ZS[0]
        P = proj_rounds(pseg, pg, pbuf)
        mx_ = {}
        acc = {}
        fin = {}

        def qk(qb):
            nk = 128 * (qb + 1)
            s = jax.lax.dot_general(Kb[0:nk, :], Qm[qb], NT, preferred_element_type=F32)
            m8 = None
            for c in range(qb + 1):
                blk = s[c * 128:(c + 1) * 128, :]
                if c == qb:
                    cm = CM[...]
                    blk = blk + jnp.concatenate([cm, cm, cm, cm], axis=1)
                SB[qb][c * 128:(c + 1) * 128, :] = blk
                mx = jnp.max(blk.reshape(16, 8, 512), axis=0)
                m8 = mx if m8 is None else jnp.maximum(m8, mx)
            mx_[qb] = jnp.max(m8, axis=0, keepdims=True)

        def pv_tile(qb, h, c):
            m = mx_[qb][:, 128 * h:128 * (h + 1)]
            p = jnp.exp2(SB[qb][pl.ds(pl.multiple_of(zz + c * 128, 128), 128), 128 * h:128 * (h + 1)] - m)
            l8 = p[120:128]
            for r in range(14, -1, -1):
                l8 = l8 + p[8 * r:8 * r + 8]
            o = jnp.dot(VT[c, 32 * h:32 * h + 32, :], p.astype(BF16), preferred_element_type=F32)
            if c > 0:
                o0, l0 = acc[(qb, h)]
                o = o0 + o
                l8 = l0 + l8
            acc[(qb, h)] = (o, l8)
            if c == qb:
                l = jnp.sum(l8, axis=0, keepdims=True)
                num = RD[zz + qb, 32 * h:32 * h + 32, :]
                den = RD[zz + qb, 128:136, :][h:h + 1, :] + 1e-06
                fin[(qb, h)] = (num * (gt[h:h + 1, :] / den) + o * (gt[4 + h:5 + h, :] / l)).astype(BF16)
                if h == 3:
                    ot = jnp.concatenate([fin[(qb, i)] for i in range(4)], axis=0)
                    OB[g, 128 * qb:128 * (qb + 1), :] = ot.T

        tiles = [(qb, h, c) for qb in range(4) for h in range(4) for c in range(qb + 1)]

        def G(i):
            for t in tiles[4 * i:4 * i + 4]:
                pv_tile(*t)

        def rd():
            st = jnp.where(seg > 0, MST[g], 0.0)
            r = jax.lax.dot_general(st.astype(BF16), PQ[...], NT, preferred_element_type=F32)
            for c in range(4):
                RD[c] = r[0:136, c * 128:(c + 1) * 128]

        def upd():
            vall = jnp.concatenate([VT[c] for c in range(4)], axis=1)
            u = jnp.dot(vall, PK[...], preferred_element_type=F32)
            rr = jax.lax.broadcasted_iota(jnp.int32, (144, 128), 0)
            cc = jax.lax.broadcasted_iota(jnp.int32, (144, 128), 1) // DH
            keep = jnp.where(rr < 128, rr // DH, rr - 128) == cc
            st2 = jnp.where(seg > 0, MST[g + zz], 0.0)
            MST[g] = st2 + jnp.where(keep, u, 0.0)

        pi = 0
        for tok in SCHED.split():
            if tok == "P":
                P[pi]()
                pi += 1
            elif tok[0] == "Q":
                qk(int(tok[1]))
            elif tok[0] == "G":
                G(int(tok[1]))
            elif tok == "R":
                rd()
            elif tok == "U":
                upd()
            elif tok == "F":
                if filler is not None:
                    filler()
        assert pi == 24

    def ophase(seg):
        for c in range(4):
            row0 = pl.multiple_of(seg * L + c * 128, 128)
            o = jnp.concatenate([OB[g, c * 128:(c + 1) * 128, :] for g in range(NG)], axis=1)
            a = jnp.dot(o, WO[...], preferred_element_type=F32)
            x1b = (R[pl.ds(row0, 128), :].astype(F32) + _rb(a)).astype(BF16)
            T[pl.ds(row0, 128), :] = x1b
            x1 = x1b.astype(F32)
            y = _rb(_ln_f32(x1))
            RC[pl.ds(row0, 128), :] = _rb(jnp.sum(y * WR[...], axis=1, keepdims=True))
            R[pl.ds(row0, 128), :] = (x1 + y).astype(BF16)

    def ffn_patch(layer):
        r = RC[...]
        idx = jax.lax.broadcasted_iota(jnp.int32, (S, 1), 0)
        m1 = jnp.max(r, axis=0, keepdims=True)
        i1 = jnp.min(jnp.where(r == m1, idx, S - 1))
        r2 = jnp.where(idx == i1, -jnp.inf, r)
        m2 = jnp.max(r2, axis=0, keepdims=True)
        i2 = jnp.min(jnp.where((r2 == m2) & (idx != i1), idx, S - 1))
        b1 = pl.multiple_of((jnp.clip(i1, 0, S - 1) // 16) * 16, 16)
        b2 = pl.multiple_of((jnp.clip(i2, 0, S - 1) // 16) * 16, 16)
        x1 = jnp.concatenate([T[pl.ds(b1, 16), :], T[pl.ds(b2, 16), :]], axis=0).astype(F32)
        yb = _ln_f32(x1).astype(BF16)
        rsel = jnp.concatenate([RC[pl.ds(b1, 16), :], RC[pl.ds(b2, 16), :]], axis=0)

        def fbody(c, acc):
            c0 = pl.multiple_of(c * FCH, FCH)
            gt = _rb(jnp.dot(yb, WG[:, pl.ds(c0, FCH)], preferred_element_type=F32))
            up = _rb(jnp.dot(yb, WU[:, pl.ds(c0, FCH)], preferred_element_type=F32))
            hm = (_rb(gt * _rb(jax.nn.sigmoid(gt))) * up).astype(BF16)
            return acc + jnp.dot(hm, WD[pl.ds(c0, FCH), :], preferred_element_type=F32)

        yv = jax.lax.fori_loop(0, NFC, fbody, jnp.zeros((32, D), F32))
        yv = _rb(_rb(yv) * _rb(jax.nn.sigmoid(rsel)))
        i16 = jax.lax.broadcasted_iota(jnp.int32, (16, 1), 0)
        rows = jnp.concatenate([i16 + b1, i16 + b2], axis=0)
        upd = jnp.where((rows == i1) | (rows == i2), yv, 0.0)
        x2b = (x1 + _rb(yb.astype(F32) + upd)).astype(BF16)
        xnb = _ln_f32(x2b.astype(F32)).astype(BF16)

        @pl.when(layer == 1)
        def _():
            for s in range(NSEG):
                out_copy(s).wait()

        R[pl.ds(b1, 16), :] = x2b[0:16]
        R[pl.ds(b2, 16), :] = x2b[16:32]
        for k in range(8):
            XN[k, pl.ds(b1, 16), :] = xnb[0:16, k * 128:(k + 1) * 128]
            XN[k, pl.ds(b2, 16), :] = xnb[16:32, k * 128:(k + 1) * 128]

        @pl.when(layer == 1)
        def _():
            c1 = pltpu.make_async_copy(R.at[pl.ds(b1, 16), :], out_hbm.at[0, pl.ds(b1, 16), :], so.at[0])
            c1.start()

            @pl.when(b2 != b1)
            def _():
                c2 = pltpu.make_async_copy(R.at[pl.ds(b2, 16), :], out_hbm.at[0, pl.ds(b2, 16), :], so.at[1])
                c2.start()
                c2.wait()

            c1.wait()

    x_copy(0).wait()
    ln1(0, L)
    for j in range(3):
        w_copy(0, j).wait()

    def layer_body(layer, carry):
        proj(0, 0, bufs[0])

        def seg_body(seg, carry2):
            first = jnp.logical_and(layer == 0, seg == 0)
            nxt = (seg + 1) % NSEG

            @pl.when(jnp.logical_and(layer == 0, seg < NSEG - 1))
            def _():
                pltpu.make_async_copy(x_hbm.at[0, pl.ds(0, L), :], R.at[pl.ds(0, L), :], sx.at[nxt]).wait()

            def gp_body(gp, carry3):
                g0 = 2 * gp
                g1 = g0 + 1
                g2 = (g0 + 2) % NG

                @pl.when(first)
                def _():
                    for j in range(3):
                        pltpu.make_async_copy(wq_hbm.at[:, pl.ds(0, 128)], W.at[0, 0],
                                              sw.at[g1, j]).wait()

                    @pl.when(gp < NG // 2 - 1)
                    def _():
                        for j in range(3):
                            pltpu.make_async_copy(wq_hbm.at[:, pl.ds(0, 128)], W.at[0, 0],
                                                  sw.at[g2, j]).wait()

                step(seg, g0, bufs[0], seg, g1, bufs[1],
                     lambda: ln1(pl.multiple_of(nxt * L + gp * 128, 128), 128))
                step(seg, g1, bufs[1], jnp.where(gp == NG // 2 - 1, nxt, seg), g2, bufs[0])
                return carry3

            jax.lax.fori_loop(0, NG // 2, gp_body, 0)

            @pl.when(first)
            def _():
                misc[0].wait()

            ophase(seg)

            @pl.when(layer == 1)
            def _():
                row0 = pl.multiple_of(seg * L, L)
                pltpu.make_async_copy(R.at[pl.ds(row0, L), :], out_hbm.at[0, pl.ds(row0, L), :],
                                      so.at[seg]).start()

            return carry2

        jax.lax.fori_loop(0, NSEG, seg_body, 0)

        @pl.when(layer == 0)
        def _():
            misc[1].wait()
            misc[2].wait()
            misc[3].wait()

        ffn_patch(layer)
        return carry

    jax.lax.fori_loop(0, 2, layer_body, 0)


@jax.jit
def pallas_interleave_layers__memory_aug_infini_attn__moe_arch_mod__prompt_kernel(
    A_x: jax.Array,
    A_wq: jax.Array,
    A_wk: jax.Array,
    A_wv: jax.Array,
    A_wo: jax.Array,
    A_beta: jax.Array,
    B_x: jax.Array,
    B_w_r: jax.Array,
    B_w_gate: jax.Array,
    B_w_up: jax.Array,
    B_w_down: jax.Array,
):
    hbm = pl.BlockSpec(memory_space=pl.ANY)
    vmem = pl.BlockSpec(memory_space=pltpu.VMEM)
    qkv_set = [
        pltpu.VMEM((L, 128), BF16),
        pltpu.VMEM((4, L, 128), BF16),
        pltpu.VMEM((L, 128), BF16),
        pltpu.VMEM((L, 128), BF16),
        pltpu.VMEM((4, 144, 128), BF16),
        pltpu.VMEM((128, L), F32),
        pltpu.VMEM((256, L), F32),
        pltpu.VMEM((384, L), F32),
        pltpu.VMEM((512, L), F32),
        pltpu.VMEM((4, 136, 128), F32),
    ]
    scratch = [
        pltpu.VMEM((S, D), BF16),
        pltpu.VMEM((S, D), BF16),
        pltpu.VMEM((8, S, 128), BF16),
        pltpu.VMEM((NG, 3, D, 128), BF16),
        pltpu.VMEM((D, D), BF16),
        pltpu.VMEM((D, FF), BF16),
        pltpu.VMEM((D, FF), BF16),
        pltpu.VMEM((FF, D), BF16),
        pltpu.VMEM((NG, L, 128), BF16),
        pltpu.VMEM((NG, 144, 128), F32),
        pltpu.VMEM((S, 1), F32),
        pltpu.VMEM((NG, 8, 128), F32),
        pltpu.VMEM((1, D), F32),
        pltpu.VMEM((128, 128), F32),
    ] + qkv_set + qkv_set + [
        pltpu.SMEM((1,), jnp.int32),
        pltpu.SemaphoreType.DMA((NSEG,)),
        pltpu.SemaphoreType.DMA((NG, 3)),
        pltpu.SemaphoreType.DMA((4,)),
        pltpu.SemaphoreType.DMA((NSEG,)),
    ]
    return pl.pallas_call(
        _kernel,
        out_shape=jax.ShapeDtypeStruct((1, S, D), BF16),
        in_specs=[hbm, hbm, hbm, hbm, hbm, vmem, vmem, hbm, hbm, hbm],
        out_specs=hbm,
        scratch_shapes=scratch,
        compiler_params=pltpu.CompilerParams(vmem_limit_bytes=100 * 1024 * 1024),
    )(A_x, A_wq, A_wk, A_wv, A_wo, A_beta, B_w_r, B_w_gate, B_w_up, B_w_down)
```

```python
import jax
import jax.numpy as jnp
import jax.experimental.pallas as pl
import jax.experimental.pallas.tpu as pltpu

F32 = jnp.float32
BF16 = jnp.bfloat16
U32 = jnp.uint32

S = 2048
D = 1024
H = 32
DH = 32
NSEG = 4
L = S // NSEG
NG = 8
FF = 3584
FCH = 512
NFC = FF // FCH
LOG2E = 1.4426950408889634
QSCALE = (DH ** -0.5) * LOG2E
NEG = -1000000000.0 * LOG2E
EPS_LN = 1.0013580322265625e-05
NT = (((1,), (1,)), ((), ()))
PZ = 1024
PD = 1032

SCHED_A = ("Q0 Q1 P P G0 f P P G1 f f P P G2 f Q2 P P G3 f f P P G4 f P P G5 f P P f f f f Q3 G6 P P G7 P P G8 P P G9 "
           "P P P P U | "
           "Q0 Q1 P G0 P P G1 P P G2 Q2 P P G3 P P G4 P P G5 Q3 P P G6 P P G7 P P G8 P P G9 P P P P P U")
SCHED_B = ("O O f Q0 O O f Q1 R O O f G0 O O f G1 O O f G2 Q2 O O f G3 O O f G4 O O f G5 f f f f Q3 "
           "P P t G6 P P t G7 P P t G8 P P t G9 P P t P P P P t P P P P t P P P P t P P U | "
           "Q0 Q1 R G0 P G1 P P G2 Q2 P P G3 P t P G4 P P G5 Q3 P t P G6 P P G7 P t P G8 P P G9 "
           "P t P P P P P P U")
SCHED_T = ("O O f Q0 O O f Q1 R O O f G0 O O f G1 O O f G2 Q2 O O f G3 O O f G4 O O f G5 f f f f Q3 "
           "P P t G6 P P t G7 P P t G8 P P t G9 P P t P P t P P t P P t P P t P P t P P t P P t | "
           "Q0 Q1 R G0 O O G1 O O G2 Q2 O O G3 O O G4 O O G5 Q3 O O G6 O O G7 O O G8 O O t G9 "
           "O O t t O O t t O O t O O t t O O t t O O t O O t "
           "O O t t O O t O O t t O O t O O t t O O t O O t t O O t "
           "O O t t O O t O O t t O O t O O t t O O t O O t t O O t "
           "O O t O O t O O t O O t O O t O O t O O O O "
           "O O t O O O O t O O O O t O O O O O O t t t")


def _rb(t):
    return t.astype(BF16).astype(F32)


def _rinv(var):
    return 1.0 / _rb(jnp.sqrt(_rb(_rb(var) + EPS_LN)))


def _ln_f32(x):
    mu = jnp.sum(x, axis=1, keepdims=True) * (1.0 / D)
    xc = x - mu
    var = jnp.sum(xc * xc, axis=1, keepdims=True) * (1.0 / D)
    return (x - _rb(mu)) * _rinv(var)


def _phi(t):
    return jnp.where(t > 0, t + 1.0, jnp.exp(t))


def _bind(f, *a):
    return lambda: f(*a)


def _kernel(x_hbm, wq_hbm, wk_hbm, wv_hbm, wo_hbm, beta_ref, wr_ref, wg_hbm, wu_hbm, wd_hbm,
            out_hbm,
            R, T, XN, W, WO, WG, WU, WD, OB, MST, GT, WR, CM, PN, RT,
            K0, Q0, PQ0, PK0, VT0, SA0, SB0, SC0, SD0, RD0, K1, Q1, PQ1, PK1, VT1, SA1, SB1, SC1, SD1, RD1,
            ZS, sx, sw, sm, so):
    bufs = ((K0, Q0, PQ0, PK0, VT0, (SA0, SB0, SC0, SD0), RD0), (K1, Q1, PQ1, PK1, VT1, (SA1, SB1, SC1, SD1), RD1))
    ZS[0] = 0
    XNu = XN.bitcast(U32)
    Wu = W.bitcast(U32)
    WOu = WO.bitcast(U32)
    OBu = OB.bitcast(U32)
    Tu = T.bitcast(U32)

    def x_copy(row0, n, s):
        return pltpu.make_async_copy(x_hbm.at[0, pl.ds(row0, n), :], R.at[pl.ds(row0, n), :], sx.at[s])

    def w_copy(g, j):
        src = (wq_hbm, wk_hbm, wv_hbm)[j]
        return pltpu.make_async_copy(src.at[:, pl.ds(pl.multiple_of(g * 128, 128), 128)], W.at[g, j], sw.at[g, j])

    def wo_copy(n):
        return pltpu.make_async_copy(wo_hbm.at[:, pl.ds(n * 128, 128)], WO.at[n], sm.at[n])

    ffn_copies = (pltpu.make_async_copy(wg_hbm, WG, sm.at[8]),
                  pltpu.make_async_copy(wu_hbm, WU, sm.at[9]),
                  pltpu.make_async_copy(wd_hbm, WD, sm.at[10]))

    def out_copy(row0, n, s):
        return pltpu.make_async_copy(R.at[pl.ds(row0, n), :], out_hbm.at[0, pl.ds(row0, n), :], so.at[s])

    x_copy(0, 128, 0).start()
    w_copy(0, 0).start()
    x_copy(128, 128, 1).start()
    w_copy(0, 1).start()
    w_copy(0, 2).start()
    x_copy(256, 128, 2).start()
    x_copy(384, 128, 3).start()
    for g in (1, 2):
        for j in range(3):
            w_copy(g, j).start()
    x_copy(512, 128, 4).start()

    gsig = jax.nn.sigmoid(beta_ref[...].astype(F32).reshape(1, H))
    eye = (jax.lax.broadcasted_iota(jnp.int32, (H, H), 0)
           == jax.lax.broadcasted_iota(jnp.int32, (H, H), 1))
    gcol = jnp.sum(jnp.where(eye, jnp.broadcast_to(gsig, (H, H)), 0.0), axis=1, keepdims=True)
    gfull = jnp.broadcast_to(gcol, (H, 128))
    for g in range(NG):
        GT[g, 0:4, :] = gfull[4 * g:4 * g + 4, :]
        GT[g, 4:8, :] = 1.0 - gfull[4 * g:4 * g + 4, :]
    WR[...] = jnp.broadcast_to(wr_ref[...].astype(F32).reshape(1, D), (8, D))
    kk = jax.lax.broadcasted_iota(jnp.int32, (128, 128), 0)
    qq = jax.lax.broadcasted_iota(jnp.int32, (128, 128), 1)
    CM[...] = jnp.where(qq < kk, NEG, 0.0).astype(F32)
    for c in range(4):
        VT0[c, 128:144, :] = jnp.ones((16, 128), BF16)
        VT1[c, 128:144, :] = jnp.ones((16, 128), BF16)
    RT[...] = jnp.zeros((16, 128), F32)
    PN[PZ:PZ + 8, :] = jnp.zeros((8, 128), F32)

    def ln_units(row0, nrows, router, slab):
        zz = ZS[0]

        def ld(i, k, v):
            if router:
                r2 = pl.multiple_of(row0 // 2 + 16 * i + zz * v, 16)
                return pltpu.bitcast(Tu[k, pl.ds(r2, 16), :], BF16).astype(F32)
            r1 = pl.multiple_of(row0 + 32 * i + zz * v, 32)
            return R[pl.ds(r1, 32), k * 128:(k + 1) * 128].astype(F32)

        def st_put(i, j, val):
            r = pl.multiple_of((slab + j) * 128 + 32 * i + zz, 32)
            PN[pl.ds(r, 32), :] = jnp.broadcast_to(val, (32, 128))

        def st_get(i, j, v):
            return PN[pl.ds(pl.multiple_of((slab + j) * 128 + 32 * i + zz * v, 32), 32), :]

        def mean(i):
            z = PN[pl.ds(pl.multiple_of(PZ + zz, 8), 8), :]
            acc = jnp.concatenate([z, z, z, z], axis=0)
            for k in range(8):
                acc = acc + ld(i, k, 1)
            st_put(i, 0, jnp.sum(acc, axis=1, keepdims=True) * (1.0 / D))

        def var(i):
            mu = st_get(i, 0, 2)
            acc = None
            for k in range(8):
                xc = ld(i, k, 2) - mu
                acc = xc * xc if acc is None else acc + xc * xc
            st_put(i, 0, _rb(mu))
            st_put(i, 1, _rinv(jnp.sum(acc, axis=1, keepdims=True) * (1.0 / D)))

        def norm(i):
            mu = st_get(i, 0, 3)
            ri = st_get(i, 1, 3)
            r2 = pl.multiple_of(row0 // 2 + 16 * i, 16)
            acc = None
            for k in range(8):
                x = ld(i, k, 3)
                y = ((x - mu) * ri).astype(BF16)
                if not router:
                    XNu[k, pl.ds(r2, 16), :] = pltpu.bitcast(y, U32)
                    continue
                y = y.astype(F32)
                wr = WR[:, k * 128:(k + 1) * 128]
                yw = y * jnp.concatenate([wr, wr, wr, wr], axis=0)
                acc = yw if acc is None else acc + yw
                R[pl.ds(pl.multiple_of(row0 + 32 * i, 32), 32), k * 128:(k + 1) * 128] = (x + y).astype(BF16)
            if router:
                r = jnp.broadcast_to(_rb(jnp.sum(acc, axis=1, keepdims=True)), (32, 128))
                tok = row0 + 32 * i
                rrow = pl.multiple_of((tok // 1024) * 8, 8)
                lane = jax.lax.broadcasted_iota(jnp.int32, (8, 128), 1) - (tok % 1024) // 8
                v = RT[pl.ds(rrow, 8), :]
                for j in range(4):
                    v = jnp.where(lane == j, r[8 * j:8 * j + 8], v)
                RT[pl.ds(rrow, 8), :] = v

        n = nrows // 32
        return [_bind(f, i) for f in (mean, var, norm) for i in range(n)]

    def proj_rounds(seg, g, buf):
        Kb, Qm, PQ, PK, VT, SB, RD = buf
        zz = ZS[0]
        part = {}

        def rnd(c, j, half):
            r2 = pl.multiple_of(seg * (L // 2) + c * 64 + zz * j, 64)
            xn = jnp.concatenate([pltpu.bitcast(XNu[k, pl.ds(r2, 64), :], BF16)
                                  for k in range(4 * half, 4 * half + 4)], axis=1)
            w = pltpu.bitcast(Wu[g, j, pl.ds(pl.multiple_of(256 * half + zz * c, 256), 256), :], BF16)
            t = jnp.dot(xn, w, preferred_element_type=F32)
            if half == 0:
                part[0] = t
                return
            t = part[0] + t
            PN[PD:PD + 8, :] = t[120:128]
            if j == 0:
                qs = t * QSCALE
                lh = jax.lax.broadcasted_iota(jnp.int32, (128, 128), 1) // DH
                for h in range(4):
                    Qm[c, h * 128:(h + 1) * 128, :] = jnp.where(lh == h, qs, 0.0).astype(BF16)
                PQ[c * 128:(c + 1) * 128, :] = _phi(t).astype(BF16)
            elif j == 1:
                Kb[c * 128:(c + 1) * 128, :] = t.astype(BF16)
                PK[c * 128:(c + 1) * 128, :] = _phi(t).astype(BF16)
            else:
                VT[c, 0:128, :] = t.astype(BF16).T

        return [_bind(rnd, c, j, half) for c in range(4) for j in range(3) for half in range(2)]

    def out_rounds(seg, off, nrows):
        zz = ZS[0]
        part = {}
        n2 = nrows // 2

        def rnd(n, half):
            o2 = pl.multiple_of(((seg % 2) * L + off) // 2 + zz * (n + 1), 16)
            o = jnp.concatenate([pltpu.bitcast(OBu[k, pl.ds(o2, n2), :], BF16)
                                 for k in range(4 * half, 4 * half + 4)], axis=1)
            w = pltpu.bitcast(WOu[n, pl.ds(pl.multiple_of(256 * half + zz * (seg * L + off), 256), 256), :], BF16)
            t = jnp.dot(o, w, preferred_element_type=F32)
            if half == 0:
                part[0] = t
                return
            r2 = pl.multiple_of((seg * L + off) // 2, 16)
            x = R[pl.ds(pl.multiple_of(seg * L + off, 32), nrows), n * 128:(n + 1) * 128].astype(F32)
            t = part[0] + t
            PN[PD:PD + 8, :] = t[nrows - 8:nrows]
            x1 = (x + _rb(t)).astype(BF16)
            Tu[n, pl.ds(r2, n2), :] = pltpu.bitcast(x1, U32)

        return [_bind(rnd, n, half) for n in range(8) for half in range(2)]

    def attn(seg, g, buf, mem):
        Kb, Qm, PQ, PK, VT, SB, RD = buf
        zz = ZS[0]
        mx_ = {}
        acc = {}
        fin = {}

        def qk(qb):
            nk = 128 * (qb + 1)
            s = jax.lax.dot_general(Kb[0:nk, :], Qm[qb], NT, preferred_element_type=F32)
            m8 = None
            for c in range(qb + 1):
                blk = s[c * 128:(c + 1) * 128, :]
                if c == qb:
                    cm = CM[...]
                    blk = blk + jnp.concatenate([cm, cm, cm, cm], axis=1)
                SB[qb][c * 128:(c + 1) * 128, :] = blk
                mx = jnp.max(blk.reshape(16, 8, 512), axis=0)
                m8 = mx if m8 is None else jnp.maximum(m8, mx)
            mx_[qb] = jnp.max(m8, axis=0, keepdims=True)

        def pv_tile(qb, h, c):
            m = mx_[qb][:, 128 * h:128 * (h + 1)]
            p = jnp.exp2(SB[qb][pl.ds(pl.multiple_of(zz + c * 128, 128), 128), 128 * h:128 * (h + 1)] - m)
            l8 = p[120:128]
            for r in range(14, -1, -1):
                l8 = l8 + p[8 * r:8 * r + 8]
            o = jnp.dot(VT[c, 32 * h:32 * h + 32, :], p.astype(BF16), preferred_element_type=F32)
            if c > 0:
                o0, l0 = acc[(qb, h)]
                o = o0 + o
                l8 = l0 + l8
            acc[(qb, h)] = (o, l8)
            if c == qb:
                gt = GT[g]
                l = jnp.sum(l8, axis=0, keepdims=True)
                res = o * (gt[4 + h:5 + h, :] / l)
                if mem:
                    num = RD[zz + qb, 32 * h:32 * h + 32, :]
                    den = RD[zz + qb, 128:136, :][h:h + 1, :] + 1e-06
                    res = num * (gt[h:h + 1, :] / den) + res
                fin[(qb, h)] = res.astype(BF16)
                if h == 3:
                    ot = jnp.concatenate([fin[(qb, i)] for i in range(4)], axis=0)
                    o2 = pl.multiple_of((seg % 2) * (L // 2) + 64 * qb, 64)
                    OBu[g, pl.ds(o2, 64), :] = pltpu.bitcast(ot.T, U32)

        tiles = [(qb, h, c) for qb in range(4) for h in range(4) for c in range(qb + 1)]

        def grp(i):
            for t in tiles[4 * i:4 * i + 4]:
                pv_tile(*t)

        def rd():
            r = jax.lax.dot_general(MST[g].astype(BF16), PQ[...], NT, preferred_element_type=F32)
            for c in range(4):
                RD[c] = r[0:136, c * 128:(c + 1) * 128]

        def upd():
            vall = jnp.concatenate([VT[c] for c in range(4)], axis=1)
            u = jnp.dot(vall, PK[...], preferred_element_type=F32)
            rr = jax.lax.broadcasted_iota(jnp.int32, (144, 128), 0)
            cc = jax.lax.broadcasted_iota(jnp.int32, (144, 128), 1) // DH
            keep = jnp.where(rr < 128, rr // DH, rr - 128) == cc
            u = jnp.where(keep, u, 0.0)
            MST[g] = MST[g + zz] + u if mem else u

        def act(tok):
            if tok[0] == "Q":
                qk(int(tok[1]))
            elif tok[0] == "G":
                grp(int(tok[1]))
            elif tok == "R":
                rd()
            else:
                assert tok == "U"
                upd()

        return act

    def run(sched, steps, queues):
        queues = {k: list(v) for k, v in queues.items()}
        si = 0
        for tok in sched.split():
            if tok == "|":
                si += 1
            elif tok in queues:
                queues[tok].pop(0)()
            else:
                steps[si](tok)
        assert all(not v for v in queues.values()), {k: len(v) for k, v in queues.items()}

    def ffn_patch(layer):
        r = RT[...]
        sub = jax.lax.broadcasted_iota(jnp.int32, (16, 128), 0)
        idx = (sub // 8) * 1024 + jax.lax.broadcasted_iota(jnp.int32, (16, 128), 1) * 8 + sub % 8
        m1 = jnp.max(r, keepdims=True)
        i1 = jnp.min(jnp.where(r == m1, idx, S - 1))
        r2 = jnp.where(idx == i1, -jnp.inf, r)
        m2 = jnp.max(r2, keepdims=True)
        i2 = jnp.min(jnp.where((r2 == m2) & (idx != i1), idx, S - 1))
        b1 = pl.multiple_of((jnp.clip(i1, 0, S - 1) // 16) * 16, 16)
        b2 = pl.multiple_of((jnp.clip(i2, 0, S - 1) // 16) * 16, 16)
        i16 = jax.lax.broadcasted_iota(jnp.int32, (16, 1), 0)
        s1 = i16 + b1 == i1
        s2 = i16 + b2 == i2

        def pick(b, sel):
            blk = jnp.concatenate([T[k, pl.ds(b, 16), :] for k in range(8)], axis=1)
            row = jnp.sum(jnp.where(sel, blk.astype(F32), 0.0), axis=0, keepdims=True)
            return jnp.broadcast_to(row, (8, D))

        x1 = jnp.concatenate([pick(b1, s1), pick(b2, s2)], axis=0)
        yb = _ln_f32(x1).astype(BF16)
        rsel = jnp.where(i16 < 8, m1, m2)

        def gate_up(c):
            gt = _rb(jnp.dot(yb, WG[:, c * FCH:(c + 1) * FCH], preferred_element_type=F32))
            up = _rb(jnp.dot(yb, WU[:, c * FCH:(c + 1) * FCH], preferred_element_type=F32))
            return (_rb(gt * _rb(jax.nn.sigmoid(gt))) * up).astype(BF16)

        hm = gate_up(0)
        yv = None
        for c in range(NFC):
            nxt = gate_up(c + 1) if c + 1 < NFC else None
            dn = jnp.dot(hm, WD[c * FCH:(c + 1) * FCH, :], preferred_element_type=F32)
            yv = dn if yv is None else yv + dn
            hm = nxt
        yv = _rb(_rb(yv) * _rb(jax.nn.sigmoid(rsel)))
        x2 = _rb(x1 + _rb(yb.astype(F32) + yv))
        xn = _rb(_ln_f32(x2))

        @pl.when(layer == 1)
        def _():
            for s in range(11):
                out_copy(0, 128, s).wait()
            out_copy(0, 640, 11).wait()

        for b, sel, lo in ((b1, s1, 0), (b2, s2, 8)):
            new = jnp.concatenate([x2[lo:lo + 8], x2[lo:lo + 8]], axis=0)
            R[pl.ds(b, 16), :] = jnp.where(sel, new, R[pl.ds(b, 16), :].astype(F32)).astype(BF16)

        @pl.when(layer == 0)
        def _():
            for b, sel, lo in ((b1, s1, 0), (b2, s2, 8)):
                new = jnp.concatenate([xn[lo:lo + 8], xn[lo:lo + 8]], axis=0)
                for k in range(8):
                    XN[k, pl.ds(b, 16), :] = jnp.where(sel, new[:, k * 128:(k + 1) * 128],
                                                       XN[k, pl.ds(b, 16), :].astype(F32)).astype(BF16)
            for f in proj_rounds(0, 0, bufs[0]):
                f()

        @pl.when(layer == 1)
        def _():
            c1 = out_copy(b1, 16, 0)
            c1.start()

            @pl.when(b2 != b1)
            def _():
                c2 = out_copy(b2, 16, 1)
                c2.start()
                c2.wait()

            c1.wait()

    p0 = proj_rounds(0, 0, bufs[0])
    x_copy(0, 128, 0).wait()
    for f in ln_units(0, 128, False, 2):
        f()
    for c in range(4):
        if c == 0:
            for j in range(3):
                w_copy(0, j).wait()
        if c < 3:
            x_copy(128 * (c + 1), 128, c + 1).wait()
            run("f f f f P P f f f f P P P P f f f f", [],
                {"P": p0[6 * c:6 * c + 6], "f": ln_units(128 * (c + 1), 128, False, 2)})
        else:
            run("P P P P P P", [], {"P": p0[18:24]})

    def layer_body(layer, carry):
        def a_body(gp, carry2):
            g0 = 2 * gp
            g2 = (g0 + 2) % NG

            @pl.when(layer == 0)
            def _():
                @pl.when(gp < 3)
                def _():
                    for j in range(3):
                        w_copy(g0 + 3, j).start()

                @pl.when(gp < 2)
                def _():
                    for j in range(3):
                        w_copy(g0 + 4, j).start()

                @pl.when(gp < 3)
                def _():
                    x_copy(pl.multiple_of(640 + 128 * gp, 128), 128, 5 + gp).start()

                @pl.when(gp == 1)
                def _():
                    for n in range(8):
                        wo_copy(n).start()

                @pl.when(gp >= 2)
                def _():
                    x_copy(pl.multiple_of(gp * L, L), L, 6 + gp).start()

                for j in range(3):
                    w_copy(g0 + 1, j).wait()

                @pl.when(gp < 3)
                def _():
                    for j in range(3):
                        w_copy(g2, j).wait()

                x_copy(0, 128, 4 + gp).wait()

            run(SCHED_A, [attn(0, g0, bufs[0], False), attn(0, g0 + 1, bufs[1], False)],
                {"P": proj_rounds(0, g0 + 1, bufs[1]) + proj_rounds(gp // 3, g2, bufs[0]),
                 "f": ln_units(L + gp * 128, 128, False, 2)})
            return carry2

        jax.lax.fori_loop(0, 4, a_body, 0)

        @pl.when(layer == 0)
        def _():
            for c in ffn_copies:
                c.start()
            for n in range(8):
                wo_copy(n).wait()
            x_copy(0, L, 8).wait()
            x_copy(0, L, 9).wait()

        def b_body(it, carry2):
            seg = 1 + it // 4
            gp = it % 4
            g0 = 2 * gp
            g2 = (g0 + 2) % NG
            prow = (seg - 1) * L + gp * 128
            run(SCHED_B, [attn(seg, g0, bufs[0], True), attn(seg, g0 + 1, bufs[1], True)],
                {"P": proj_rounds(seg, g0 + 1, bufs[1]) + proj_rounds(seg + gp // 3, g2, bufs[0]),
                 "O": out_rounds(seg - 1, gp * 128, 128),
                 "f": ln_units(((seg + 1) % NSEG) * L + gp * 128, 128, False, 2),
                 "t": ln_units(prow, 128, True, 0)})

            @pl.when(layer == 1)
            def _():
                out_copy(pl.multiple_of(prow, 128), 128, it).start()

            return carry2

        jax.lax.fori_loop(0, 11, b_body, 0)

        pieces = ((0, 128), (128, 128), (256, 128), (384, 64), (448, 32), (480, 32))
        run(SCHED_T, [attn(3, 6, bufs[0], True), attn(3, 7, bufs[1], True)],
            {"P": proj_rounds(3, 7, bufs[1]),
             "O": out_rounds(2, 384, 128) + [f for off, n in pieces for f in out_rounds(3, off, n)],
             "f": ln_units(384, 128, False, 2),
             "t": ln_units(2 * L + 384, 128, True, 0)
             + [f for i, (off, n) in enumerate(pieces)
                for f in ln_units(3 * L + off, n, True, 4 + 2 * (i % 2))]})

        @pl.when(layer == 0)
        def _():
            for c in ffn_copies:
                c.wait()

        @pl.when(layer == 1)
        def _():
            out_copy(S - 640, 640, 11).start()

        ffn_patch(layer)
        return carry

    jax.lax.fori_loop(0, 2, layer_body, 0)


@jax.jit
def pallas_interleave_layers__memory_aug_infini_attn__moe_arch_mod__prompt_kernel(
    A_x: jax.Array,
    A_wq: jax.Array,
    A_wk: jax.Array,
    A_wv: jax.Array,
    A_wo: jax.Array,
    A_beta: jax.Array,
    B_x: jax.Array,
    B_w_r: jax.Array,
    B_w_gate: jax.Array,
    B_w_up: jax.Array,
    B_w_down: jax.Array,
):
    hbm = pl.BlockSpec(memory_space=pl.ANY)
    vmem = pl.BlockSpec(memory_space=pltpu.VMEM)
    qkv_set = [
        pltpu.VMEM((L, 128), BF16),
        pltpu.VMEM((4, L, 128), BF16),
        pltpu.VMEM((L, 128), BF16),
        pltpu.VMEM((L, 128), BF16),
        pltpu.VMEM((4, 144, 128), BF16),
        pltpu.VMEM((128, L), F32),
        pltpu.VMEM((256, L), F32),
        pltpu.VMEM((384, L), F32),
        pltpu.VMEM((512, L), F32),
        pltpu.VMEM((4, 136, 128), F32),
    ]
    scratch = [
        pltpu.VMEM((S, D), BF16),
        pltpu.VMEM((8, S, 128), BF16),
        pltpu.VMEM((8, S, 128), BF16),
        pltpu.VMEM((NG, 3, D, 128), BF16),
        pltpu.VMEM((8, D, 128), BF16),
        pltpu.VMEM((D, FF), BF16),
        pltpu.VMEM((D, FF), BF16),
        pltpu.VMEM((FF, D), BF16),
        pltpu.VMEM((NG, 2 * L, 128), BF16),
        pltpu.VMEM((NG, 144, 128), F32),
        pltpu.VMEM((NG, 8, 128), F32),
        pltpu.VMEM((8, D), F32),
        pltpu.VMEM((128, 128), F32),
        pltpu.VMEM((PD + 8, 128), F32),
        pltpu.VMEM((16, 128), F32),
    ] + qkv_set + qkv_set + [
        pltpu.SMEM((1,), jnp.int32),
        pltpu.SemaphoreType.DMA((10,)),
        pltpu.SemaphoreType.DMA((NG, 3)),
        pltpu.SemaphoreType.DMA((11,)),
        pltpu.SemaphoreType.DMA((12,)),
    ]
    return pl.pallas_call(
        _kernel,
        out_shape=jax.ShapeDtypeStruct((1, S, D), BF16),
        in_specs=[hbm, hbm, hbm, hbm, hbm, vmem, vmem, hbm, hbm, hbm],
        out_specs=hbm,
        scratch_shapes=scratch,
        compiler_params=pltpu.CompilerParams(vmem_limit_bytes=100 * 1024 * 1024),
    )(A_x, A_wq, A_wk, A_wv, A_wo, A_beta, B_w_r, B_w_gate, B_w_up, B_w_down)
```

```python
import jax
import jax.numpy as jnp
import jax.experimental.pallas as pl
import jax.experimental.pallas.tpu as pltpu

F32 = jnp.float32
BF16 = jnp.bfloat16
U32 = jnp.uint32

S = 2048
D = 1024
H = 32
DH = 32
NSEG = 4
L = S // NSEG
NG = 8
FF = 3584
FCH = 512
NFC = FF // FCH
LOG2E = 1.4426950408889634
QSCALE = (DH ** -0.5) * LOG2E
NEG = -1000000000.0 * LOG2E
EPS_LN = 1.0013580322265625e-05
NT = (((1,), (1,)), ((), ()))
PZ = 1024
PD = 1032

SCHED_A = ("Q0 Q1 P P G0 S0 f P P G1 f f P P G2 S1 f Q2 P P G3 f f P P G4 f P P G5 S2 f P P f f f f Q3 G6 P P G7 P P "
           "G8 P P G9 S3 P P P P U | "
           "Q0 Q1 P G0 S0 P P G1 P P G2 S1 Q2 P P G3 P P G4 P P G5 S2 Q3 P P G6 P P G7 P P G8 P P G9 S3 P P P P P U")
SCHED_B = ("O O f O O f O O f O O f O O f O O f Q0 O O f Q1 R O O f G0 S0 P G1 P P t G2 S1 Q2 P P t G3 P P t G4 "
           "P P t G5 S2 f f f f Q3 P P t G6 P P t G7 P P t G8 P P t G9 S3 P P P P P P P U | "
           "Q0 Q1 R G0 S0 P G1 P P t G2 S1 Q2 P P G3 P P t G4 P P G5 S2 Q3 P P t G6 P P G7 P P t G8 P P G9 S3 "
           "P P P P P P P U")
SCHED_T = ("O O f O O f O O f Q0 Q1 R O O f G0 S0 P G1 P P f G2 S1 Q2 P P f G3 P P f G4 "
           "P P f G5 S2 f f f f Q3 P P G6 P P G7 P P G8 P P G9 S3 P P P P P P P | "
           "Q0 O O Q1 R O O G0 O O G1 S0 O O G2 Q2 O O t G3 S1 O O t G4 O O t G5 Q3 O O t t G6 S2 O O t G7 O O t t G8 "
           "O O t t G9 O O t t S3 "
           "O O t t O O t O O t t O O t O O t t O O t O O t t O O t "
           "O O t t O O t O O t t O O t O O t t O O t O O t t O O t "
           "O O t t O O t O O t t O O t O O t t O O t O O t t O O t "
           "O O t O O t O O t O O t O O t O O t O O O O "
           "O O t O O O O t O O O O t O O O O O O t t t")


def _rb(t):
    return t.astype(BF16).astype(F32)


def _rinv(var):
    return 1.0 / _rb(jnp.sqrt(_rb(_rb(var) + EPS_LN)))


def _ln_f32(x):
    mu = jnp.sum(x, axis=1, keepdims=True) * (1.0 / D)
    xc = x - mu
    var = jnp.sum(xc * xc, axis=1, keepdims=True) * (1.0 / D)
    return (x - _rb(mu)) * _rinv(var)


def _phi(t):
    return jnp.where(t > 0, t + 1.0, jnp.exp(t))


def _bind(f, *a):
    return lambda: f(*a)


def _kernel(x_hbm, wq_hbm, wk_hbm, wv_hbm, wo_hbm, beta_ref, wr_ref, wg_hbm, wu_hbm, wd_hbm,
            out_hbm,
            R, T, XN, W, WO, WG, WU, WD, OB, MST, GT, WR, CM, PN, RT,
            K0, Q0, PQ0, PK0, VT0, SA0, SB0, SC0, SD0, RD0, K1, Q1, PQ1, PK1, VT1, SA1, SB1, SC1, SD1, RD1,
            ZS, sx, sw, sm, so):
    bufs = ((K0, Q0, PQ0, PK0, VT0, (SA0, SB0, SC0, SD0), RD0), (K1, Q1, PQ1, PK1, VT1, (SA1, SB1, SC1, SD1), RD1))
    ZS[0] = 0
    XNu = XN.bitcast(U32)
    Wu = W.bitcast(U32)
    WOu = WO.bitcast(U32)
    OBu = OB.bitcast(U32)
    Tu = T.bitcast(U32)

    def x_copy(row0, n, s):
        return pltpu.make_async_copy(x_hbm.at[0, pl.ds(row0, n), :], R.at[pl.ds(row0, n), :], sx.at[s])

    def w_copy(g, j):
        src = (wq_hbm, wk_hbm, wv_hbm)[j]
        return pltpu.make_async_copy(src.at[:, pl.ds(pl.multiple_of(g * 128, 128), 128)], W.at[g, j], sw.at[g, j])

    def wo_copy(n):
        return pltpu.make_async_copy(wo_hbm.at[:, pl.ds(n * 128, 128)], WO.at[n], sm.at[n])

    ffn_copies = (pltpu.make_async_copy(wg_hbm, WG, sm.at[8]),
                  pltpu.make_async_copy(wu_hbm, WU, sm.at[9]),
                  pltpu.make_async_copy(wd_hbm, WD, sm.at[10]))

    def out_copy(row0, n, s):
        return pltpu.make_async_copy(R.at[pl.ds(row0, n), :], out_hbm.at[0, pl.ds(row0, n), :], so.at[s])

    x_copy(0, 128, 0).start()
    w_copy(0, 0).start()
    x_copy(128, 128, 1).start()
    w_copy(0, 1).start()
    w_copy(0, 2).start()
    x_copy(256, 128, 2).start()
    x_copy(384, 128, 3).start()
    for g in (1, 2):
        for j in range(3):
            w_copy(g, j).start()
    x_copy(512, 128, 4).start()

    gsig = jax.nn.sigmoid(beta_ref[...].astype(F32).reshape(1, H))
    eye = (jax.lax.broadcasted_iota(jnp.int32, (H, H), 0)
           == jax.lax.broadcasted_iota(jnp.int32, (H, H), 1))
    gcol = jnp.sum(jnp.where(eye, jnp.broadcast_to(gsig, (H, H)), 0.0), axis=1, keepdims=True)
    gfull = jnp.broadcast_to(gcol, (H, 128))
    for g in range(NG):
        GT[g, 0:4, :] = gfull[4 * g:4 * g + 4, :]
        GT[g, 4:8, :] = 1.0 - gfull[4 * g:4 * g + 4, :]
    WR[...] = jnp.broadcast_to(wr_ref[...].astype(F32).reshape(1, D), (8, D))
    kk = jax.lax.broadcasted_iota(jnp.int32, (128, 128), 0)
    qq = jax.lax.broadcasted_iota(jnp.int32, (128, 128), 1)
    CM[...] = jnp.where(qq < kk, NEG, 0.0).astype(F32)
    for c in range(4):
        VT0[c, 128:144, :] = jnp.ones((16, 128), BF16)
        VT1[c, 128:144, :] = jnp.ones((16, 128), BF16)
    RT[...] = jnp.zeros((16, 128), F32)
    PN[PZ:PZ + 8, :] = jnp.zeros((8, 128), F32)

    def ln_units(row0, nrows, router, slab):
        zz = ZS[0]

        def ld(i, k, v):
            if router:
                r2 = pl.multiple_of(row0 // 2 + 16 * i + zz * v, 16)
                return pltpu.bitcast(Tu[k, pl.ds(r2, 16), :], BF16).astype(F32)
            r1 = pl.multiple_of(row0 + 32 * i + zz * v, 32)
            return R[pl.ds(r1, 32), k * 128:(k + 1) * 128].astype(F32)

        def st_put(i, j, val):
            r = pl.multiple_of((slab + j) * 128 + 32 * i + zz, 32)
            PN[pl.ds(r, 32), :] = jnp.broadcast_to(val, (32, 128))

        def st_get(i, j, v):
            return PN[pl.ds(pl.multiple_of((slab + j) * 128 + 32 * i + zz * v, 32), 32), :]

        def mean(i):
            z = PN[pl.ds(pl.multiple_of(PZ + zz, 8), 8), :]
            acc = jnp.concatenate([z, z, z, z], axis=0)
            for k in range(8):
                acc = acc + ld(i, k, 1)
            st_put(i, 0, jnp.sum(acc, axis=1, keepdims=True) * (1.0 / D))

        def var(i):
            mu = st_get(i, 0, 2)
            acc = None
            for k in range(8):
                xc = ld(i, k, 2) - mu
                acc = xc * xc if acc is None else acc + xc * xc
            st_put(i, 0, _rb(mu))
            st_put(i, 1, _rinv(jnp.sum(acc, axis=1, keepdims=True) * (1.0 / D)))

        def norm(i):
            mu = st_get(i, 0, 3)
            ri = st_get(i, 1, 3)
            r2 = pl.multiple_of(row0 // 2 + 16 * i, 16)
            acc = None
            for k in range(8):
                x = ld(i, k, 3)
                y = ((x - mu) * ri).astype(BF16)
                if not router:
                    XNu[k, pl.ds(r2, 16), :] = pltpu.bitcast(y, U32)
                    continue
                y = y.astype(F32)
                wr = WR[:, k * 128:(k + 1) * 128]
                yw = y * jnp.concatenate([wr, wr, wr, wr], axis=0)
                acc = yw if acc is None else acc + yw
                R[pl.ds(pl.multiple_of(row0 + 32 * i, 32), 32), k * 128:(k + 1) * 128] = (x + y).astype(BF16)
            if router:
                r = jnp.broadcast_to(_rb(jnp.sum(acc, axis=1, keepdims=True)), (32, 128))
                tok = row0 + 32 * i
                rrow = pl.multiple_of((tok // 1024) * 8, 8)
                lane = jax.lax.broadcasted_iota(jnp.int32, (8, 128), 1) - (tok % 1024) // 8
                v = RT[pl.ds(rrow, 8), :]
                for j in range(4):
                    v = jnp.where(lane == j, r[8 * j:8 * j + 8], v)
                RT[pl.ds(rrow, 8), :] = v

        n = nrows // 32
        return [_bind(f, i) for f in (mean, var, norm) for i in range(n)]

    def proj_rounds(seg, g, buf):
        Kb, Qm, PQ, PK, VT, SB, RD = buf
        zz = ZS[0]
        part = {}

        def rnd(c, j, half):
            r2 = pl.multiple_of(seg * (L // 2) + c * 64 + zz * j, 64)
            xn = jnp.concatenate([pltpu.bitcast(XNu[k, pl.ds(r2, 64), :], BF16)
                                  for k in range(4 * half, 4 * half + 4)], axis=1)
            w = pltpu.bitcast(Wu[g, j, pl.ds(pl.multiple_of(256 * half + zz * c, 256), 256), :], BF16)
            t = jnp.dot(xn, w, preferred_element_type=F32)
            if half == 0:
                part[0] = t
                return
            t = part[0] + t
            PN[PD:PD + 8, :] = t[120:128]
            if j == 0:
                qs = t * QSCALE
                lh = jax.lax.broadcasted_iota(jnp.int32, (128, 128), 1) // DH
                for h in range(4):
                    Qm[c, h * 128:(h + 1) * 128, :] = jnp.where(lh == h, qs, 0.0).astype(BF16)
                PQ[c * 128:(c + 1) * 128, :] = _phi(t).astype(BF16)
            elif j == 1:
                Kb[c * 128:(c + 1) * 128, :] = t.astype(BF16)
                PK[c * 128:(c + 1) * 128, :] = _phi(t).astype(BF16)
            else:
                VT[c, 0:128, :] = t.astype(BF16).T

        return [_bind(rnd, c, j, half) for c in range(4) for j in range(3) for half in range(2)]

    def out_rounds(seg, off, nrows):
        zz = ZS[0]
        part = {}
        n2 = nrows // 2

        def rnd(n, half):
            o2 = pl.multiple_of(((seg % 2) * L + off) // 2 + zz * (n + 1), 16)
            o = jnp.concatenate([pltpu.bitcast(OBu[k, pl.ds(o2, n2), :], BF16)
                                 for k in range(4 * half, 4 * half + 4)], axis=1)
            w = pltpu.bitcast(WOu[n, pl.ds(pl.multiple_of(256 * half + zz * (seg * L + off), 256), 256), :], BF16)
            t = jnp.dot(o, w, preferred_element_type=F32)
            if half == 0:
                part[0] = t
                return
            r2 = pl.multiple_of((seg * L + off) // 2, 16)
            x = R[pl.ds(pl.multiple_of(seg * L + off, 32), nrows), n * 128:(n + 1) * 128].astype(F32)
            t = part[0] + t
            PN[PD:PD + 8, :] = t[nrows - 8:nrows]
            x1 = (x + _rb(t)).astype(BF16)
            Tu[n, pl.ds(r2, n2), :] = pltpu.bitcast(x1, U32)

        return [_bind(rnd, n, half) for n in range(8) for half in range(2)]

    def attn(seg, g, buf, mem):
        Kb, Qm, PQ, PK, VT, SB, RD = buf
        zz = ZS[0]
        mx_ = {}
        acc = {}
        fin = {}

        def qk(qb):
            nk = 128 * (qb + 1)
            s = jax.lax.dot_general(Kb[0:nk, :], Qm[qb], NT, preferred_element_type=F32)
            m8 = None
            for c in range(qb + 1):
                blk = s[c * 128:(c + 1) * 128, :]
                if c == qb:
                    cm = CM[...]
                    blk = blk + jnp.concatenate([cm, cm, cm, cm], axis=1)
                SB[qb][c * 128:(c + 1) * 128, :] = blk
                mx = jnp.max(blk.reshape(16, 8, 512), axis=0)
                m8 = mx if m8 is None else jnp.maximum(m8, mx)
            mx_[qb] = jnp.max(m8, axis=0, keepdims=True)

        def pv_tile(qb, h, c):
            m = mx_[qb][:, 128 * h:128 * (h + 1)]
            p = jnp.exp2(SB[qb][pl.ds(pl.multiple_of(zz + c * 128, 128), 128), 128 * h:128 * (h + 1)] - m)
            l8 = p[120:128]
            for r in range(14, -1, -1):
                l8 = l8 + p[8 * r:8 * r + 8]
            o = jnp.dot(VT[c, 32 * h:32 * h + 32, :], p.astype(BF16), preferred_element_type=F32)
            if c > 0:
                o0, l0 = acc[(qb, h)]
                o = o0 + o
                l8 = l0 + l8
            acc[(qb, h)] = (o, l8)
            if c == qb:
                gt = GT[g]
                l = jnp.sum(l8, axis=0, keepdims=True)
                res = o * (gt[4 + h:5 + h, :] / l)
                if mem:
                    num = RD[zz + qb, 32 * h:32 * h + 32, :]
                    den = RD[zz + qb, 128:136, :][h:h + 1, :] + 1e-06
                    res = num * (gt[h:h + 1, :] / den) + res
                fin[(qb, h)] = res.astype(BF16)

        def put(qb):
            ot = jnp.concatenate([fin[(qb, i)] for i in range(4)], axis=0)
            o2 = pl.multiple_of((seg % 2) * (L // 2) + 64 * qb, 64)
            OBu[g, pl.ds(o2, 64), :] = pltpu.bitcast(ot.T, U32)

        tiles = [(qb, h, c) for qb in range(4) for h in range(4) for c in range(qb + 1)]

        def grp(i):
            for t in tiles[4 * i:4 * i + 4]:
                pv_tile(*t)

        def rd():
            r = jax.lax.dot_general(MST[g].astype(BF16), PQ[...], NT, preferred_element_type=F32)
            for c in range(4):
                RD[c] = r[0:136, c * 128:(c + 1) * 128]

        def upd():
            vall = jnp.concatenate([VT[c] for c in range(4)], axis=1)
            u = jnp.dot(vall, PK[...], preferred_element_type=F32)
            rr = jax.lax.broadcasted_iota(jnp.int32, (144, 128), 0)
            cc = jax.lax.broadcasted_iota(jnp.int32, (144, 128), 1) // DH
            keep = jnp.where(rr < 128, rr // DH, rr - 128) == cc
            u = jnp.where(keep, u, 0.0)
            MST[g] = MST[g + zz] + u if mem else u

        def act(tok):
            if tok[0] == "Q":
                qk(int(tok[1]))
            elif tok[0] == "G":
                grp(int(tok[1]))
            elif tok[0] == "S":
                put(int(tok[1]))
            elif tok == "R":
                rd()
            else:
                assert tok == "U"
                upd()

        return act

    def run(sched, steps, queues):
        queues = {k: list(v) for k, v in queues.items()}
        si = 0
        for tok in sched.split():
            if tok == "|":
                si += 1
            elif tok in queues:
                queues[tok].pop(0)()
            else:
                steps[si](tok)
        assert all(not v for v in queues.values()), {k: len(v) for k, v in queues.items()}

    def ffn_patch(layer):
        r = RT[...]
        sub = jax.lax.broadcasted_iota(jnp.int32, (16, 128), 0)
        idx = (sub // 8) * 1024 + jax.lax.broadcasted_iota(jnp.int32, (16, 128), 1) * 8 + sub % 8
        m1 = jnp.max(r, keepdims=True)
        i1 = jnp.min(jnp.where(r == m1, idx, S - 1))
        r2 = jnp.where(idx == i1, -jnp.inf, r)
        m2 = jnp.max(r2, keepdims=True)
        i2 = jnp.min(jnp.where((r2 == m2) & (idx != i1), idx, S - 1))
        b1 = pl.multiple_of((jnp.clip(i1, 0, S - 1) // 16) * 16, 16)
        b2 = pl.multiple_of((jnp.clip(i2, 0, S - 1) // 16) * 16, 16)
        i16 = jax.lax.broadcasted_iota(jnp.int32, (16, 1), 0)
        s1 = i16 + b1 == i1
        s2 = i16 + b2 == i2

        def pick(b, sel):
            blk = jnp.concatenate([T[k, pl.ds(b, 16), :] for k in range(8)], axis=1)
            row = jnp.sum(jnp.where(sel, blk.astype(F32), 0.0), axis=0, keepdims=True)
            return jnp.broadcast_to(row, (8, D))

        x1 = jnp.concatenate([pick(b1, s1), pick(b2, s2)], axis=0)
        yb = _ln_f32(x1).astype(BF16)
        rsel = jnp.where(i16 < 8, m1, m2)

        def gate_up(c):
            gt = _rb(jnp.dot(yb, WG[:, c * FCH:(c + 1) * FCH], preferred_element_type=F32))
            up = _rb(jnp.dot(yb, WU[:, c * FCH:(c + 1) * FCH], preferred_element_type=F32))
            return (_rb(gt * _rb(jax.nn.sigmoid(gt))) * up).astype(BF16)

        hm = gate_up(0)
        yv = None
        for c in range(NFC):
            nxt = gate_up(c + 1) if c + 1 < NFC else None
            dn = jnp.dot(hm, WD[c * FCH:(c + 1) * FCH, :], preferred_element_type=F32)
            yv = dn if yv is None else yv + dn
            hm = nxt
        yv = _rb(_rb(yv) * _rb(jax.nn.sigmoid(rsel)))
        x2 = _rb(x1 + _rb(yb.astype(F32) + yv))
        xn = _rb(_ln_f32(x2))

        @pl.when(layer == 1)
        def _():
            for s in range(11):
                out_copy(0, 128, s).wait()
            out_copy(0, 640, 11).wait()

        for b, sel, lo in ((b1, s1, 0), (b2, s2, 8)):
            new = jnp.concatenate([x2[lo:lo + 8], x2[lo:lo + 8]], axis=0)
            R[pl.ds(b, 16), :] = jnp.where(sel, new, R[pl.ds(b, 16), :].astype(F32)).astype(BF16)

        @pl.when(layer == 0)
        def _():
            for b, sel, lo in ((b1, s1, 0), (b2, s2, 8)):
                new = jnp.concatenate([xn[lo:lo + 8], xn[lo:lo + 8]], axis=0)
                for k in range(8):
                    XN[k, pl.ds(b, 16), :] = jnp.where(sel, new[:, k * 128:(k + 1) * 128],
                                                       XN[k, pl.ds(b, 16), :].astype(F32)).astype(BF16)
            for f in proj_rounds(0, 0, bufs[0]):
                f()

        @pl.when(layer == 1)
        def _():
            c1 = out_copy(b1, 16, 0)
            c1.start()

            @pl.when(b2 != b1)
            def _():
                c2 = out_copy(b2, 16, 1)
                c2.start()
                c2.wait()

            c1.wait()

    p0 = proj_rounds(0, 0, bufs[0])
    x_copy(0, 128, 0).wait()
    for f in ln_units(0, 128, False, 2):
        f()
    for c in range(4):
        if c == 0:
            for j in range(3):
                w_copy(0, j).wait()
        if c < 3:
            x_copy(128 * (c + 1), 128, c + 1).wait()
            run("f f f f P P f f f f P P P P f f f f", [],
                {"P": p0[6 * c:6 * c + 6], "f": ln_units(128 * (c + 1), 128, False, 2)})
        else:
            run("P P P P P P", [], {"P": p0[18:24]})

    def layer_body(layer, carry):
        def a_body(gp, carry2):
            g0 = 2 * gp
            g2 = (g0 + 2) % NG

            @pl.when(layer == 0)
            def _():
                @pl.when(gp < 3)
                def _():
                    for j in range(3):
                        w_copy(g0 + 3, j).start()

                @pl.when(gp < 2)
                def _():
                    for j in range(3):
                        w_copy(g0 + 4, j).start()

                @pl.when(gp < 3)
                def _():
                    x_copy(pl.multiple_of(640 + 128 * gp, 128), 128, 5 + gp).start()

                @pl.when(gp == 1)
                def _():
                    for n in range(8):
                        wo_copy(n).start()

                @pl.when(gp >= 2)
                def _():
                    x_copy(pl.multiple_of(gp * L, L), L, 6 + gp).start()

                for j in range(3):
                    w_copy(g0 + 1, j).wait()

                @pl.when(gp < 3)
                def _():
                    for j in range(3):
                        w_copy(g2, j).wait()

                x_copy(0, 128, 4 + gp).wait()

            run(SCHED_A, [attn(0, g0, bufs[0], False), attn(0, g0 + 1, bufs[1], False)],
                {"P": proj_rounds(0, g0 + 1, bufs[1]) + proj_rounds(gp // 3, g2, bufs[0]),
                 "f": ln_units(L + gp * 128, 128, False, 2)})
            return carry2

        jax.lax.fori_loop(0, 4, a_body, 0)

        @pl.when(layer == 0)
        def _():
            for c in ffn_copies:
                c.start()
            for n in range(8):
                wo_copy(n).wait()
            x_copy(0, L, 8).wait()
            x_copy(0, L, 9).wait()

        def b_body(it, carry2):
            seg = 1 + it // 4
            gp = it % 4
            g0 = 2 * gp
            g2 = (g0 + 2) % NG
            prow = (seg - 1) * L + gp * 128
            run(SCHED_B, [attn(seg, g0, bufs[0], True), attn(seg, g0 + 1, bufs[1], True)],
                {"P": proj_rounds(seg, g0 + 1, bufs[1]) + proj_rounds(seg + gp // 3, g2, bufs[0]),
                 "O": out_rounds(seg - 1, gp * 128, 128),
                 "f": ln_units(((seg + 1) % NSEG) * L + gp * 128, 128, False, 2),
                 "t": ln_units(prow, 128, True, 0)})

            @pl.when(layer == 1)
            def _():
                out_copy(pl.multiple_of(prow, 128), 128, it).start()

            return carry2

        jax.lax.fori_loop(0, 11, b_body, 0)

        pieces = ((0, 128), (128, 128), (256, 128), (384, 64), (448, 32), (480, 32))
        run(SCHED_T, [attn(3, 6, bufs[0], True), attn(3, 7, bufs[1], True)],
            {"P": proj_rounds(3, 7, bufs[1]),
             "O": out_rounds(2, 384, 128) + [f for off, n in pieces for f in out_rounds(3, off, n)],
             "f": ln_units(384, 128, False, 2),
             "t": ln_units(2 * L + 384, 128, True, 0)
             + [f for i, (off, n) in enumerate(pieces)
                for f in ln_units(3 * L + off, n, True, 4 + 2 * (i % 2))]})

        @pl.when(layer == 0)
        def _():
            for c in ffn_copies:
                c.wait()

        @pl.when(layer == 1)
        def _():
            out_copy(S - 640, 640, 11).start()

        ffn_patch(layer)
        return carry

    jax.lax.fori_loop(0, 2, layer_body, 0)


@jax.jit
def pallas_interleave_layers__memory_aug_infini_attn__moe_arch_mod__prompt_kernel(
    A_x: jax.Array,
    A_wq: jax.Array,
    A_wk: jax.Array,
    A_wv: jax.Array,
    A_wo: jax.Array,
    A_beta: jax.Array,
    B_x: jax.Array,
    B_w_r: jax.Array,
    B_w_gate: jax.Array,
    B_w_up: jax.Array,
    B_w_down: jax.Array,
):
    hbm = pl.BlockSpec(memory_space=pl.ANY)
    vmem = pl.BlockSpec(memory_space=pltpu.VMEM)
    qkv_set = [
        pltpu.VMEM((L, 128), BF16),
        pltpu.VMEM((4, L, 128), BF16),
        pltpu.VMEM((L, 128), BF16),
        pltpu.VMEM((L, 128), BF16),
        pltpu.VMEM((4, 144, 128), BF16),
        pltpu.VMEM((128, L), F32),
        pltpu.VMEM((256, L), F32),
        pltpu.VMEM((384, L), F32),
        pltpu.VMEM((512, L), F32),
        pltpu.VMEM((4, 136, 128), F32),
    ]
    scratch = [
        pltpu.VMEM((S, D), BF16),
        pltpu.VMEM((8, S, 128), BF16),
        pltpu.VMEM((8, S, 128), BF16),
        pltpu.VMEM((NG, 3, D, 128), BF16),
        pltpu.VMEM((8, D, 128), BF16),
        pltpu.VMEM((D, FF), BF16),
        pltpu.VMEM((D, FF), BF16),
        pltpu.VMEM((FF, D), BF16),
        pltpu.VMEM((NG, 2 * L, 128), BF16),
        pltpu.VMEM((NG, 144, 128), F32),
        pltpu.VMEM((NG, 8, 128), F32),
        pltpu.VMEM((8, D), F32),
        pltpu.VMEM((128, 128), F32),
        pltpu.VMEM((PD + 8, 128), F32),
        pltpu.VMEM((16, 128), F32),
    ] + qkv_set + qkv_set + [
        pltpu.SMEM((1,), jnp.int32),
        pltpu.SemaphoreType.DMA((10,)),
        pltpu.SemaphoreType.DMA((NG, 3)),
        pltpu.SemaphoreType.DMA((11,)),
        pltpu.SemaphoreType.DMA((12,)),
    ]
    return pl.pallas_call(
        _kernel,
        out_shape=jax.ShapeDtypeStruct((1, S, D), BF16),
        in_specs=[hbm, hbm, hbm, hbm, hbm, vmem, vmem, hbm, hbm, hbm],
        out_specs=hbm,
        scratch_shapes=scratch,
        compiler_params=pltpu.CompilerParams(vmem_limit_bytes=100 * 1024 * 1024),
    )(A_x, A_wq, A_wk, A_wv, A_wo, A_beta, B_w_r, B_w_gate, B_w_up, B_w_down)
```

```python
import jax
import jax.numpy as jnp
import jax.experimental.pallas as pl
import jax.experimental.pallas.tpu as pltpu

F32 = jnp.float32
BF16 = jnp.bfloat16
U32 = jnp.uint32

S = 2048
D = 1024
H = 32
DH = 32
NSEG = 4
L = S // NSEG
NG = 8
FF = 3584
FCH = 512
NFC = FF // FCH
LOG2E = 1.4426950408889634
QSCALE = (DH ** -0.5) * LOG2E
NEG = -1000000000.0 * LOG2E
EPS_LN = 1.0013580322265625e-05
BIG = 3.0e38
NT = (((1,), (1,)), ((), ()))
PZ = 1024
PD = 1032

SCHED_A = ("D0 g0 n Q1 g1 n D2 n Q2 n G0 S0 P P G1 g2 m P P G2 g3 S1 m P P G3 g4 Q3 m P P G4 g5 m P P G5 g6 S2 P P G6 g7 P P G7 g8 P P "
           "G8 g9 P P G9 S3 m P P D0+ m P P Q1+ g0+ P P U | "
           "G0 g1 S0 P P D2 G1 g2 P P Q2 G2 g3 S1 P P G3 g4 P P G4 g5 Q3 P P G5 g6 S2 P P G6 g7 P P G7 g8 P P G8 g9 P P G9 S3 m P P m P P P P U")
SCHED_B = ("O O n O O n m O O n m O O n m O O m m O O m D0 O O g0 m Q1 R O O m G0 g1 S0 P P D2 G1 g2 t P P Q2 G2 g3 S1 t P P G3 g4 t P P G4 g5 "
           "Q3 t P P G5 g6 S2 t P P G6 g7 t P P G7 g8 t P P G8 g9 t P P G9 S3 t P P D0+ t P P Q1+ g0+ P P U | "
           "R G0 g1 S0 P P D2 G1 g2 P P Q2 G2 g3 S1 P P G3 g4 P P G4 g5 Q3 P P G5 g6 S2 P P G6 g7 P P G7 g8 P P G8 g9 P P G9 S3 "
           "t P P t P P P P U")
SCHED_T = ("O O n O O n O O n D0 Q1 g0 R O O n G0 g1 S0 D2 G1 g2 P P Q2 G2 g3 S1 P P G3 g4 P P G4 g5 Q3 "
           "P P G5 g6 S2 P P G6 g7 P P G7 g8 P P G8 g9 P P G9 S3 P P D0+ P P Q1+ g0+ P P P P | "
           "R O O G0 g1 O O D2 G1 g2 S0 O O Q2 G2 g3 O O G3 g4 S1 t O O G4 g5 Q3 t O O G5 g6 t O O G6 g7 S2 t t O O G7 g8 t O O G8 g9 "
           "t t O O G9 t t O O t t S3 O O "
           "O O t t O O t O O t t O O t O O t t O O t O O t t O O t "
           "O O t t O O t O O t t O O t O O t t O O t O O t t O O t "
           "O O t t O O t O O t t O O t O O t t O O t O O t t O O t "
           "O O t O O t O O t O O t O O t O O t O O O O "
           "O O t O O O O t O O O O t O O O O O O t t t")


def _rb(t):
    return t.astype(BF16).astype(F32)


def _rcp(d):
    d = jnp.minimum(d, BIG)
    r = pl.reciprocal(d, approx=True)
    return r * (2.0 - d * r)


def _rinv(var):
    v = _rb(_rb(var) + EPS_LN)
    vc = jnp.minimum(v, BIG)
    return jnp.minimum(_rcp(_rb(vc * jax.lax.rsqrt(vc))), 1e30 * pl.reciprocal(v, approx=True))


def _ln_f32(x):
    mu = jnp.sum(x, axis=1, keepdims=True) * (1.0 / D)
    xc = x - mu
    var = jnp.sum(xc * xc, axis=1, keepdims=True) * (1.0 / D)
    return (x - _rb(mu)) * _rinv(var)


def _phi(t):
    return jnp.maximum(t, 0.0) + jnp.exp(jnp.minimum(t, 0.0))


def _bind(f, *a):
    return lambda: f(*a)


def _kernel(x_hbm, wq_hbm, wk_hbm, wv_hbm, wo_hbm, beta_ref, wr_ref, wg_hbm, wu_hbm, wd_hbm,
            out_hbm,
            R, T, XN, W, WO, WG, WU, WD, OB, MST, GT, WR, CM, LM, PN, PG, RT,
            K0, Q0, PQ0, PK0, VT0, SA0, SB0, SC0, SD0, RD0, K1, Q1, PQ1, PK1, VT1, SA1, SB1, SC1, SD1, RD1,
            ZS, sx, sw, sm, so):
    bufs = ((K0, Q0, PQ0, PK0, VT0, (SA0, SB0, SC0, SD0), RD0), (K1, Q1, PQ1, PK1, VT1, (SA1, SB1, SC1, SD1), RD1))
    ZS[0] = 0
    XNu = XN.bitcast(U32)
    Wu = W.bitcast(U32)
    WOu = WO.bitcast(U32)
    OBu = OB.bitcast(U32)
    Tu = T.bitcast(U32)

    def x_copy(row0, n, s):
        return pltpu.make_async_copy(x_hbm.at[0, pl.ds(row0, n), :], R.at[pl.ds(row0, n), :], sx.at[s])

    def w_copy(g, j):
        src = (wq_hbm, wk_hbm, wv_hbm)[j]
        return pltpu.make_async_copy(src.at[:, pl.ds(pl.multiple_of(g * 128, 128), 128)], W.at[g, j], sw.at[g, j])

    def wo_copy(n):
        return pltpu.make_async_copy(wo_hbm.at[:, pl.ds(n * 128, 128)], WO.at[n], sm.at[n])

    ffn_copies = (pltpu.make_async_copy(wg_hbm, WG, sm.at[8]),
                  pltpu.make_async_copy(wu_hbm, WU, sm.at[9]),
                  pltpu.make_async_copy(wd_hbm, WD, sm.at[10]))

    def out_copy(row0, n, s):
        return pltpu.make_async_copy(R.at[pl.ds(row0, n), :], out_hbm.at[0, pl.ds(row0, n), :], so.at[s])

    x_copy(0, 128, 0).start()
    w_copy(0, 0).start()
    x_copy(128, 128, 1).start()
    w_copy(0, 1).start()
    w_copy(0, 2).start()
    x_copy(256, 128, 2).start()
    x_copy(384, 128, 3).start()
    for g in (1, 2):
        for j in range(3):
            w_copy(g, j).start()
    x_copy(512, 128, 4).start()
    x_copy(640, 128, 5).start()

    gsig = jax.nn.sigmoid(beta_ref[...].astype(F32).reshape(1, H))
    eye = (jax.lax.broadcasted_iota(jnp.int32, (H, H), 0)
           == jax.lax.broadcasted_iota(jnp.int32, (H, H), 1))
    gcol = jnp.sum(jnp.where(eye, jnp.broadcast_to(gsig, (H, H)), 0.0), axis=1, keepdims=True)
    gfull = jnp.broadcast_to(gcol, (H, 128))
    for g in range(NG):
        GT[g, 0:4, :] = gfull[4 * g:4 * g + 4, :]
        GT[g, 4:8, :] = 1.0 - gfull[4 * g:4 * g + 4, :]
    WR[...] = jnp.broadcast_to(wr_ref[...].astype(F32).reshape(1, D), (8, D))
    kk = jax.lax.broadcasted_iota(jnp.int32, (32, 128), 0)
    qq = jax.lax.broadcasted_iota(jnp.int32, (32, 128), 1) % 32
    CM[...] = jnp.where(qq < kk, NEG, 0.0).astype(F32)
    for c in range(4):
        LM[c] = jnp.where(jax.lax.broadcasted_iota(jnp.int32, (8, 128), 1) // DH == c,
                          jnp.uint32(0xFFFFFFFF), jnp.uint32(0))
        VT0[c, 64:72, :] = pltpu.bitcast(jnp.ones((16, 128), BF16), U32)
        VT1[c, 64:72, :] = pltpu.bitcast(jnp.ones((16, 128), BF16), U32)
    RT[...] = jnp.zeros((16, 128), F32)
    PN[PZ:PZ + 8, :] = jnp.zeros((8, 128), F32)

    def ln_units(row0, nrows, router, slab):
        zz = ZS[0]

        def ld(i, k, v):
            if router:
                r2 = pl.multiple_of(row0 // 2 + 16 * i + zz * v, 16)
                return pltpu.bitcast(Tu[k, pl.ds(r2, 16), :], BF16).astype(F32)
            r1 = pl.multiple_of(row0 + 32 * i + zz * v, 32)
            return R[pl.ds(r1, 32), k * 128:(k + 1) * 128].astype(F32)

        def st_put(i, j, val, last=True):
            r = pl.multiple_of((slab + j) * 128 + 32 * i + zz, 32)
            val = jnp.broadcast_to(val, (32, 128))
            PN[pl.ds(r, 32), :] = val
            if last:
                PG[pl.ds(pl.multiple_of(520 + zz, 8), 8), :] = val[24:32]

        def st_get(i, j, v):
            return PN[pl.ds(pl.multiple_of((slab + j) * 128 + 32 * i + zz * v, 32), 32), :]

        def mean(i):
            z = PN[pl.ds(pl.multiple_of(PZ + zz, 8), 8), :]
            acc = jnp.concatenate([z, z, z, z], axis=0)
            for k in range(8):
                acc = acc + ld(i, k, 1)
            st_put(i, 0, jnp.sum(acc, axis=1, keepdims=True) * (1.0 / D))

        def var(i):
            mu = st_get(i, 0, 2)
            acc = None
            for k in range(8):
                xc = ld(i, k, 2) - mu
                acc = xc * xc if acc is None else acc + xc * xc
            st_put(i, 0, _rb(mu), False)
            st_put(i, 1, _rinv(jnp.sum(acc, axis=1, keepdims=True) * (1.0 / D)))

        def norm(i):
            mu = st_get(i, 0, 3)
            ri = st_get(i, 1, 3)
            r2 = pl.multiple_of(row0 // 2 + 16 * i, 16)
            acc = None
            for k in range(8):
                x = ld(i, k, 3)
                y = (x - mu) * ri
                if k == 7:
                    PN[pl.ds(pl.multiple_of(PD + 8 + zz, 8), 8), :] = y[24:32]
                    PG[pl.ds(pl.multiple_of(520 + zz, 8), 8), :] = y[24:32]
                y = y.astype(BF16)
                if not router:
                    XNu[k, pl.ds(r2, 16), :] = pltpu.bitcast(y, U32)
                    continue
                y = y.astype(F32)
                wr = WR[:, k * 128:(k + 1) * 128]
                yw = y * jnp.concatenate([wr, wr, wr, wr], axis=0)
                acc = yw if acc is None else acc + yw
                R[pl.ds(pl.multiple_of(row0 + 32 * i, 32), 32), k * 128:(k + 1) * 128] = (x + y).astype(BF16)
            if router:
                r = jnp.broadcast_to(_rb(jnp.sum(acc, axis=1, keepdims=True)), (32, 128))
                tok = row0 + 32 * i
                rrow = pl.multiple_of((tok // 1024) * 8, 8)
                lane = jax.lax.broadcasted_iota(jnp.int32, (8, 128), 1) - (tok % 1024) // 8
                v = RT[pl.ds(rrow, 8), :]
                for j in range(4):
                    v = jnp.where(lane == j, r[8 * j:8 * j + 8], v)
                RT[pl.ds(rrow, 8), :] = v

        n = nrows // 32
        return [_bind(f, i) for f in (mean, var, norm) for i in range(n)]

    def proj_rounds(seg, g, buf):
        Kb, Qm, PQ, PK, VT, SB, RD = buf
        zz = ZS[0]
        part = {}

        def rnd(c, j, half):
            r2 = pl.multiple_of(seg * (L // 2) + c * 64 + zz * j, 64)
            xn = jnp.concatenate([pltpu.bitcast(XNu[k, pl.ds(r2, 64), :], BF16)
                                  for k in range(4 * half, 4 * half + 4)], axis=1)
            w = pltpu.bitcast(Wu[g, j, pl.ds(pl.multiple_of(256 * half + zz * c, 256), 256), :], BF16)
            t = jnp.dot(xn, w, preferred_element_type=F32)
            if half == 0:
                part[0] = t
                return
            t = t + part[0]
            PN[PD:PD + 8, :] = t[120:128]
            PG[512:520, :] = t[120:128]
            if j == 0:
                qt = pltpu.bitcast((t * QSCALE).astype(BF16).T, U32)
                for h in range(4):
                    qh = qt[16 * h:16 * h + 16]
                    Qm[c, 16 * h:16 * h + 16, :] = pltpu.roll(qh, 32 * h, 1) if h else qh
                PQ[c * 64:(c + 1) * 64, :] = pltpu.bitcast(_phi(t).astype(BF16), U32)
            elif j == 1:
                Kb[c * 64:(c + 1) * 64, :] = pltpu.bitcast(t.astype(BF16), U32)
                PK[c * 64:(c + 1) * 64, :] = pltpu.bitcast(_phi(t).astype(BF16), U32)
            else:
                VT[c, 0:64, :] = pltpu.bitcast(t.astype(BF16).T, U32)

        return [_bind(rnd, c, j, half) for c in range(4) for j in range(3) for half in range(2)]

    def out_rounds(seg, off, nrows):
        zz = ZS[0]
        part = {}
        n2 = nrows // 2

        def rnd(n, half):
            o2 = pl.multiple_of(((seg % 2) * L + off) // 2 + zz * (n + 1), 16)
            o = jnp.concatenate([pltpu.bitcast(OBu[k, pl.ds(o2, n2), :], BF16)
                                 for k in range(4 * half, 4 * half + 4)], axis=1)
            w = pltpu.bitcast(WOu[n, pl.ds(pl.multiple_of(256 * half + zz * (seg * L + off), 256), 256), :], BF16)
            t = jnp.dot(o, w, preferred_element_type=F32)
            if half == 0:
                part[0] = t
                return
            r2 = pl.multiple_of((seg * L + off) // 2, 16)
            x = R[pl.ds(pl.multiple_of(seg * L + off, 32), nrows), n * 128:(n + 1) * 128].astype(F32)
            t = t + part[0]
            PN[PD:PD + 8, :] = t[nrows - 8:nrows]
            PG[512:520, :] = t[nrows - 8:nrows]
            x1 = (x + _rb(t)).astype(BF16)
            Tu[n, pl.ds(r2, n2), :] = pltpu.bitcast(x1, U32)

        return [_bind(rnd, n, half) for n in range(8) for half in range(2)]

    def attn(seg, g, buf, mem):
        Kb, Qm, PQ, PK, VT, SB, RD = buf
        zz = ZS[0]
        pg0 = 0 if buf is bufs[0] else 256
        ml = {}
        m8_ = {}
        acc = {}
        fin = {}

        def bfly(e, rows):
            lane = jax.lax.broadcasted_iota(jnp.int32, (rows, 128), 1)
            s0 = (lane & 32) != 0
            s1 = (lane & 64) != 0

            def sel(m, x, y):
                if x is None and y is None:
                    return None
                z = jnp.zeros_like(x if y is None else y)
                return jnp.where(m, z if x is None else x, z if y is None else y)

            a = [[sel(s1, e[2 + j], e[j]), sel(s1, e[j], e[2 + j])] for j in range(2)]
            return [sel(s0, a[1][0], a[0][0]), sel(s0, a[0][0], a[1][1]),
                    sel(s0, a[1][1], a[0][1]), sel(s0, a[0][1], a[1][0])]

        def put_max(qb, m8):
            m = jnp.broadcast_to(jnp.max(m8, axis=0, keepdims=True), (8, 512))
            m = [m[:, 128 * h:128 * (h + 1)] for h in range(4)]
            for i, v in enumerate(m + bfly(m, 8)):
                if qb > 0 or i >= 4:
                    PG[pg0 + 64 * qb + 8 * i:pg0 + 64 * qb + 8 * i + 8, :] = v

        def get_max(i):
            for qb, h in [(dg.index(i), 4 + j) for j in range(4)] if i in dg else [t[:2] for t in tiles(i)]:
                if (i, h) not in ml:
                    ml[(i, h)] = PG[pl.ds(pl.multiple_of(zz * (i + 1) + pg0 + 64 * qb + 8 * h, 8), 8), :]

        def diag(qa):
            lm = [jnp.concatenate([LM[i]] * 2, axis=0) for i in range(4)]
            for qb, rev in ((qa, False), (qa + 1, True)):
                m8 = [None] * 4
                for j in range(3, -1, -1):
                    w = jnp.concatenate([Qm[qb, 16 * h:16 * h + 16, :] & lm[(j + h) % 4] for h in range(4)], axis=0)
                    rs = range(j, -1, -1) if rev else range(j + 1)
                    kq = jnp.concatenate([Kb[64 * qb + 16 * r:64 * qb + 16 * r + 16, :] for r in rs], axis=0)
                    d = jnp.dot(pltpu.bitcast(kq, BF16), pltpu.bitcast(w, BF16), preferred_element_type=F32)
                    for i, r in enumerate(rs):
                        v = d[32 * i:32 * i + 32] + CM[...] if r == j else d[32 * i:32 * i + 32]
                        SB[qb][128 * qb + 32 * r:128 * qb + 32 * r + 32, 128 * j:128 * (j + 1)] = v
                        mx = jnp.max(v.reshape(4, 8, 128), axis=0)
                        m8[j] = mx if m8[j] is None else jnp.maximum(m8[j], mx)
                m8_[qb] = jnp.concatenate(bfly(m8, 8), axis=1)
            if qa == 0:
                put_max(0, m8_[0])

        def qk(qb):
            z16 = jnp.zeros((16, 128), U32)
            w = jnp.concatenate([jnp.concatenate([Qm[qb, 16 * h:16 * h + 16, :] if i == h else z16
                                                  for i in range(4)], axis=0) for h in range(4)], axis=1)
            s = jnp.dot(pltpu.bitcast(Kb[0:64 * qb, :], BF16), pltpu.bitcast(w, BF16), preferred_element_type=F32)
            m8 = m8_[qb]
            for c in range(qb):
                blk = s[c * 128:(c + 1) * 128, :]
                SB[qb][c * 128:(c + 1) * 128, :] = blk
                m8 = jnp.maximum(m8, jnp.max(blk.reshape(16, 8, 512), axis=0))
            put_max(qb, m8)

        def pv(qb, h, c, p, l8):
            o = jnp.dot(pltpu.bitcast(VT[c, 16 * h:16 * h + 16, :], BF16), p, preferred_element_type=F32)
            if (qb, h) in acc:
                o0, l0, n = acc[(qb, h)]
                o = o + o0
                l8 = l0 + l8
            else:
                n = 0
            acc[(qb, h)] = (o, l8, n + 1)
            if n == qb:
                gt = GT[g]
                l = jnp.sum(l8, axis=0, keepdims=True)
                res = o * (gt[4 + h:5 + h, :] * _rcp(l))
                if h > 0:
                    res = pltpu.roll(res, 128 - 32 * h, 1)
                if mem:
                    num = RD[zz + qb, 32 * h:32 * h + 32, :]
                    den = RD[zz + qb, 128:136, :][h:h + 1, :] + 1e-06
                    res = num * (gt[h:h + 1, :] * _rcp(den)) + res
                fin[(qb, h)] = res.astype(BF16)

        def pv_tile(i, qb, h, c):
            m = jnp.concatenate([ml[(i, h)]] * 16, axis=0)
            p = jnp.exp2(SB[qb][pl.ds(pl.multiple_of(zz + c * 128, 128), 128), 128 * h:128 * (h + 1)] - m)
            l8 = p[120:128]
            for r in range(14, -1, -1):
                l8 = l8 + p[8 * r:8 * r + 8]
            pv(qb, h, c, p.astype(BF16), l8)

        def pv_diag(qb):
            m = [ml[(dg[qb], 4 + j)] for j in range(4)]
            l8 = [None] * 4
            w = {}
            for r in range(3, -1, -1):
                e = [None] * 4
                for j in range(r, 4):
                    row = pl.multiple_of(zz + 128 * qb + 32 * r, 32)
                    p = jnp.exp2(SB[qb][pl.ds(row, 32), 128 * j:128 * (j + 1)] - jnp.concatenate([m[j]] * 4, axis=0))
                    for i in range(3, -1, -1):
                        l8[j] = p[8 * i:8 * i + 8] if l8[j] is None else l8[j] + p[8 * i:8 * i + 8]
                    e[j] = pltpu.bitcast(p.astype(BF16), U32)
                w[r] = bfly(e, 16)
            l8 = bfly(l8, 8)
            for h in range(4):
                pv(qb, h, qb, pltpu.bitcast(jnp.concatenate([w[r][h] for r in range(4)], axis=0), BF16), l8[h])

        def put(qb):
            ot = jnp.concatenate([fin[(qb, i)] for i in range(4)], axis=0)
            o2 = pl.multiple_of((seg % 2) * (L // 2) + 64 * qb, 64)
            OBu[g, pl.ds(o2, 64), :] = pltpu.bitcast(ot.T, U32)

        dg = (0, 1, 3, 6)

        def tiles(i):
            i = (2, 4, 5, 7, 8, 9).index(i)
            return [(qb, h, c) for qb in range(4) for h in range(4) for c in range(qb)][4 * i:4 * i + 4]

        def grp(i):
            get_max(i)
            if i in dg:
                pv_diag(dg.index(i))
                return
            for t in tiles(i):
                pv_tile(i, *t)

        def rd():
            r = jax.lax.dot_general(MST[g].astype(BF16), pltpu.bitcast(PQ[...], BF16), NT, preferred_element_type=F32)
            for c in range(4):
                RD[c] = r[0:136, c * 128:(c + 1) * 128]

        def upd():
            vall = pltpu.bitcast(jnp.concatenate([VT[c] for c in range(4)], axis=1), BF16)
            u = jnp.dot(vall, pltpu.bitcast(PK[...], BF16), preferred_element_type=F32)
            rr = jax.lax.broadcasted_iota(jnp.int32, (144, 128), 0)
            cc = jax.lax.broadcasted_iota(jnp.int32, (144, 128), 1) // DH
            keep = jnp.where(rr < 128, rr // DH, rr - 128) == cc
            u = jnp.where(keep, u, 0.0)
            MST[g] = MST[g + zz] + u if mem else u

        def act(tok):
            if tok[0] == "Q":
                qk(int(tok[1]))
            elif tok[0] == "D":
                diag(int(tok[1]))
            elif tok[0] == "G":
                grp(int(tok[1]))
            elif tok[0] == "g":
                get_max(int(tok[1]))
            elif tok[0] == "S":
                put(int(tok[1]))
            elif tok == "R":
                rd()
            else:
                assert tok == "U"
                upd()

        return act

    def run(sched, steps, queues):
        queues = {k: list(v) for k, v in queues.items()}
        si = 0
        for tok in sched.split():
            if tok == "|":
                si += 1
            elif tok in queues:
                queues[tok].pop(0)()
            elif tok[-1] == "+":
                steps[si + 1](tok[:-1])
            else:
                steps[si](tok)
        assert all(not v for v in queues.values()), {k: len(v) for k, v in queues.items()}

    def ffn_patch(layer):
        r = RT[...]
        sub = jax.lax.broadcasted_iota(jnp.int32, (16, 128), 0)
        idx = (sub // 8) * 1024 + jax.lax.broadcasted_iota(jnp.int32, (16, 128), 1) * 8 + sub % 8
        m1 = jnp.max(r, keepdims=True)
        i1 = jnp.min(jnp.where(r == m1, idx, S - 1))
        r2 = jnp.where(idx == i1, -jnp.inf, r)
        m2 = jnp.max(r2, keepdims=True)
        i2 = jnp.min(jnp.where((r2 == m2) & (idx != i1), idx, S - 1))
        b1 = pl.multiple_of((jnp.clip(i1, 0, S - 1) // 16) * 16, 16)
        b2 = pl.multiple_of((jnp.clip(i2, 0, S - 1) // 16) * 16, 16)
        i16 = jax.lax.broadcasted_iota(jnp.int32, (16, 1), 0)
        s1 = i16 + b1 == i1
        s2 = i16 + b2 == i2

        def pick(b, sel):
            blk = jnp.concatenate([T[k, pl.ds(b, 16), :] for k in range(8)], axis=1)
            row = jnp.sum(jnp.where(sel, blk.astype(F32), 0.0), axis=0, keepdims=True)
            return jnp.broadcast_to(row, (8, D))

        x1 = jnp.concatenate([pick(b1, s1), pick(b2, s2)], axis=0)
        yb = _ln_f32(x1).astype(BF16)
        rsel = jnp.where(i16 < 8, m1, m2)

        def gate_up(c):
            gt = _rb(jnp.dot(yb, WG[:, c * FCH:(c + 1) * FCH], preferred_element_type=F32))
            up = _rb(jnp.dot(yb, WU[:, c * FCH:(c + 1) * FCH], preferred_element_type=F32))
            return (_rb(gt * _rb(jax.nn.sigmoid(gt))) * up).astype(BF16)

        hm = gate_up(0)
        yv = None
        for c in range(NFC):
            nxt = gate_up(c + 1) if c + 1 < NFC else None
            dn = jnp.dot(hm, WD[c * FCH:(c + 1) * FCH, :], preferred_element_type=F32)
            yv = dn if yv is None else yv + dn
            hm = nxt
        yv = _rb(_rb(yv) * _rb(jax.nn.sigmoid(rsel)))
        x2 = _rb(x1 + _rb(yb.astype(F32) + yv))
        xn = _rb(_ln_f32(x2))

        @pl.when(layer == 1)
        def _():
            for s in range(11):
                out_copy(0, 128, s).wait()
            out_copy(0, 640, 11).wait()

        for b, sel, lo in ((b1, s1, 0), (b2, s2, 8)):
            new = jnp.concatenate([x2[lo:lo + 8], x2[lo:lo + 8]], axis=0)
            R[pl.ds(b, 16), :] = jnp.where(sel, new, R[pl.ds(b, 16), :].astype(F32)).astype(BF16)

        @pl.when(layer == 0)
        def _():
            for b, sel, lo in ((b1, s1, 0), (b2, s2, 8)):
                new = jnp.concatenate([xn[lo:lo + 8], xn[lo:lo + 8]], axis=0)
                for k in range(8):
                    XN[k, pl.ds(b, 16), :] = jnp.where(sel, new[:, k * 128:(k + 1) * 128],
                                                       XN[k, pl.ds(b, 16), :].astype(F32)).astype(BF16)
            run("P P m P P m P P m P P m P P m P P m P P m P P m P P P P P P P P", [],
                {"P": proj_rounds(0, 0, bufs[0]), "m": ln_units(L, 128, False, 2)[:8]})

        @pl.when(layer == 1)
        def _():
            c1 = out_copy(b1, 16, 0)
            c1.start()

            @pl.when(b2 != b1)
            def _():
                c2 = out_copy(b2, 16, 1)
                c2.start()
                c2.wait()

            c1.wait()

    p0 = proj_rounds(0, 0, bufs[0])
    x_copy(0, 128, 0).wait()
    for f in ln_units(0, 128, False, 2):
        f()
    for c in range(4):
        if c == 0:
            for j in range(3):
                w_copy(0, j).wait()
        if c < 3:
            x_copy(128 * (c + 1), 128, c + 1).wait()
            run("f f f f P P f f f f P P P P f f f f", [],
                {"P": p0[6 * c:6 * c + 6], "f": ln_units(128 * (c + 1), 128, False, 2)})
        else:
            x_copy(0, 128, 4).wait()
            run("m m m m P P m m P P m m P P", [], {"P": p0[18:24], "m": ln_units(L, 128, False, 2)[:8]})

    def layer_body(layer, carry):
        def a_body(gp, carry2):
            g0 = 2 * gp
            g2 = (g0 + 2) % NG

            @pl.when(layer == 0)
            def _():
                @pl.when(gp < 3)
                def _():
                    for j in range(3):
                        w_copy(g0 + 3, j).start()

                @pl.when(gp < 2)
                def _():
                    for j in range(3):
                        w_copy(g0 + 4, j).start()

                @pl.when(gp < 2)
                def _():
                    x_copy(pl.multiple_of(768 + 128 * gp, 128), 128, 6 + gp).start()

                @pl.when(gp == 1)
                def _():
                    for n in range(8):
                        wo_copy(n).start()

                @pl.when(gp >= 2)
                def _():
                    x_copy(pl.multiple_of(gp * L, L), L, 6 + gp).start()

                for j in range(3):
                    w_copy(g0 + 1, j).wait()

                @pl.when(gp < 3)
                def _():
                    for j in range(3):
                        w_copy(g2, j).wait()
                    x_copy(0, 128, 5 + gp).wait()

                @pl.when(gp == 3)
                def _():
                    x_copy(0, L, 8).wait()

            run(SCHED_A, [attn(0, g0, bufs[0], False), attn(0, g0 + 1, bufs[1], False)],
                {"P": proj_rounds(0, g0 + 1, bufs[1]) + proj_rounds(gp // 3, g2, bufs[0]),
                 "n": ln_units(L + gp * 128, 128, False, 2)[8:],
                 "m": ln_units(L + 128 + gp * 128, 128, False, 2)[:8]})
            return carry2

        jax.lax.fori_loop(0, 4, a_body, 0)

        @pl.when(layer == 0)
        def _():
            for c in ffn_copies:
                c.start()
            for n in range(8):
                wo_copy(n).wait()
            x_copy(0, L, 9).wait()

        def b_body(it, carry2):
            seg = 1 + it // 4
            gp = it % 4
            g0 = 2 * gp
            g2 = (g0 + 2) % NG
            prow = (seg - 1) * L + gp * 128
            run(SCHED_B, [attn(seg, g0, bufs[0], True), attn(seg, g0 + 1, bufs[1], True)],
                {"P": proj_rounds(seg, g0 + 1, bufs[1]) + proj_rounds(seg + gp // 3, g2, bufs[0]),
                 "O": out_rounds(seg - 1, gp * 128, 128),
                 "n": ln_units((1024 + it * 128) % S, 128, False, 2)[8:],
                 "m": ln_units((1152 + it * 128) % S, 128, False, 2)[:8],
                 "t": ln_units(prow, 128, True, 0)})

            @pl.when(layer == 1)
            def _():
                out_copy(pl.multiple_of(prow, 128), 128, it).start()

            return carry2

        jax.lax.fori_loop(0, 11, b_body, 0)

        pieces = ((0, 128), (128, 128), (256, 128), (384, 64), (448, 32), (480, 32))
        run(SCHED_T, [attn(3, 6, bufs[0], True), attn(3, 7, bufs[1], True)],
            {"P": proj_rounds(3, 7, bufs[1]),
             "O": out_rounds(2, 384, 128) + [f for off, n in pieces for f in out_rounds(3, off, n)],
             "n": ln_units(384, 128, False, 2)[8:],
             "t": ln_units(2 * L + 384, 128, True, 0)
             + [f for i, (off, n) in enumerate(pieces)
                for f in ln_units(3 * L + off, n, True, 4 + 2 * (i % 2))]})

        @pl.when(layer == 0)
        def _():
            for c in ffn_copies:
                c.wait()

        @pl.when(layer == 1)
        def _():
            out_copy(S - 640, 640, 11).start()

        ffn_patch(layer)
        return carry

    jax.lax.fori_loop(0, 2, layer_body, 0)


@jax.jit
def pallas_interleave_layers__memory_aug_infini_attn__moe_arch_mod__prompt_kernel(
    A_x: jax.Array,
    A_wq: jax.Array,
    A_wk: jax.Array,
    A_wv: jax.Array,
    A_wo: jax.Array,
    A_beta: jax.Array,
    B_x: jax.Array,
    B_w_r: jax.Array,
    B_w_gate: jax.Array,
    B_w_up: jax.Array,
    B_w_down: jax.Array,
):
    hbm = pl.BlockSpec(memory_space=pl.ANY)
    vmem = pl.BlockSpec(memory_space=pltpu.VMEM)
    qkv_set = [
        pltpu.VMEM((L // 2, 128), U32),
        pltpu.VMEM((4, 64, 128), U32),
        pltpu.VMEM((L // 2, 128), U32),
        pltpu.VMEM((L // 2, 128), U32),
        pltpu.VMEM((4, 72, 128), U32),
        pltpu.VMEM((128, L), F32),
        pltpu.VMEM((256, L), F32),
        pltpu.VMEM((384, L), F32),
        pltpu.VMEM((512, L), F32),
        pltpu.VMEM((4, 136, 128), F32),
    ]
    scratch = [
        pltpu.VMEM((S, D), BF16),
        pltpu.VMEM((8, S, 128), BF16),
        pltpu.VMEM((8, S, 128), BF16),
        pltpu.VMEM((NG, 3, D, 128), BF16),
        pltpu.VMEM((8, D, 128), BF16),
        pltpu.VMEM((D, FF), BF16),
        pltpu.VMEM((D, FF), BF16),
        pltpu.VMEM((FF, D), BF16),
        pltpu.VMEM((NG, 2 * L, 128), BF16),
        pltpu.VMEM((NG, 144, 128), F32),
        pltpu.VMEM((NG, 8, 128), F32),
        pltpu.VMEM((8, D), F32),
        pltpu.VMEM((32, 128), F32),
        pltpu.VMEM((4, 8, 128), U32),
        pltpu.VMEM((PD + 16, 128), F32),
        pltpu.VMEM((528, 128), F32),
        pltpu.VMEM((16, 128), F32),
    ] + qkv_set + qkv_set + [
        pltpu.SMEM((1,), jnp.int32),
        pltpu.SemaphoreType.DMA((10,)),
        pltpu.SemaphoreType.DMA((NG, 3)),
        pltpu.SemaphoreType.DMA((11,)),
        pltpu.SemaphoreType.DMA((12,)),
    ]
    return pl.pallas_call(
        _kernel,
        out_shape=jax.ShapeDtypeStruct((1, S, D), BF16),
        in_specs=[hbm, hbm, hbm, hbm, hbm, vmem, vmem, hbm, hbm, hbm],
        out_specs=hbm,
        scratch_shapes=scratch,
        compiler_params=pltpu.CompilerParams(vmem_limit_bytes=100 * 1024 * 1024),
    )(A_x, A_wq, A_wk, A_wv, A_wo, A_beta, B_w_r, B_w_gate, B_w_up, B_w_down)
```

```python
import jax
import jax.numpy as jnp
import jax.experimental.pallas as pl
import jax.experimental.pallas.tpu as pltpu

F32 = jnp.float32
BF16 = jnp.bfloat16
U32 = jnp.uint32

S = 2048
D = 1024
H = 32
DH = 32
NSEG = 4
L = S // NSEG
NG = 8
FF = 3584
FCH = 512
NFC = FF // FCH
LOG2E = 1.4426950408889634
QSCALE = (DH ** -0.5) * LOG2E
NEG = -1000000000.0 * LOG2E
EPS_LN = 1.0013580322265625e-05
BIG = 3.0e38
NT = (((1,), (1,)), ((), ()))
PZ = 1024
PD = 1032

SCHED_A = ("D0 g0 n Q1 g1 n D2 n Q2 n G0 S0 P P G1 g2 m P P G2 g3 S1 m P P G3 g4 Q3 m P P G4 g5 m P P G5 g6 S2 m "
           "P P G6 g7 m P P G7 g8 m P P G8 g9 m P P G9 S3 P P D0+ P P Q1+ g0+ P P U | G0 g1 S0 P P D2 G1 g2 P P "
           "Q2 G2 g3 S1 P P G3 g4 P P G4 g5 Q3 P P G5 g6 S2 P P G6 g7 P P G7 g8 P P G8 g9 P P G9 S3 P P P P P P "
           "U ")
SCHED_B = ("O O n O O n m O O n m O O n m O O m m O O m D0 O O g0 m Q1 R O O g1 m G0 S0 P P D2 G1 g2 t t P P Q2 "
           "G2 g3 S1 t t P P G3 g4 t P P G4 g5 Q3 t P P G5 g6 S2 t P P G6 g7 t P P G7 g8 P P G8 g9 P P G9 S3 t P "
           "P D0+ t P P Q1+ g0+ P P U | R G0 g1 S0 P P D2 G1 g2 P P Q2 G2 g3 S1 P P G3 g4 P P G4 g5 Q3 P P G5 g6 "
           "S2 P P G6 g7 P P G7 g8 P P G8 g9 P P G9 S3 t P P t P P P P U ")
SCHED_T = ("O O n O O n O O n D0 Q1 g0 R O O n G0 g1 S0 D2 G1 g2 P P Q2 G2 g3 S1 P P G3 g4 P P G4 g5 Q3 "
           "P P G5 g6 S2 P P G6 g7 P P G7 g8 P P G8 g9 P P G9 S3 P P D0+ P P Q1+ g0+ P P P P | "
           "R O O G0 g1 O O D2 G1 g2 S0 O O Q2 G2 g3 O O G3 g4 S1 t O O G4 g5 Q3 t O O G5 g6 t O O G6 g7 S2 t t O O G7 g8 t O O G8 g9 "
           "t t O O G9 t t O O t t S3 O O "
           "O O t t O O t O O t t O O t O O t t O O t O O t t O O t "
           "O O t t O O t O O t t O O t O O t t O O t O O t t O O t "
           "O O t t O O t O O t t O O t O O t t O O t O O t t O O t "
           "O O t O O t O O t O O t O O t O O t O O O O "
           "O O t O O O O t O O O O t O O O O O O t t t")


def _rb(t):
    return t.astype(BF16).astype(F32)


def _rb2(t):
    n = t.shape[0] // 2
    p = pltpu.pack_elementwise([t[:n], t[n:]], packed_dtype=BF16)
    return jnp.concatenate([pltpu.unpack_elementwise(p, index=i, packed_dtype=BF16, unpacked_dtype=F32)
                            for i in range(2)], axis=0)


def _rcp(d):
    d = jnp.minimum(d, BIG)
    r = pl.reciprocal(d, approx=True)
    return r * (2.0 - d * r)


def _rinv(var):
    v = _rb(_rb(var) + EPS_LN)
    vc = jnp.minimum(v, BIG)
    return jnp.minimum(_rcp(_rb(vc * jax.lax.rsqrt(vc))), 1e30 * pl.reciprocal(v, approx=True))


def _ln_f32(x):
    mu = jnp.sum(x, axis=1, keepdims=True) * (1.0 / D)
    xc = x - mu
    var = jnp.sum(xc * xc, axis=1, keepdims=True) * (1.0 / D)
    return (x - _rb(mu)) * _rinv(var)


def _phi(t):
    return jnp.maximum(t, 0.0) + jnp.exp(jnp.minimum(t, 0.0))


def _bind(f, *a):
    return lambda: f(*a)


def _kernel(x_hbm, wq_hbm, wk_hbm, wv_hbm, wo_hbm, beta_ref, wr_ref, wg_hbm, wu_hbm, wd_hbm,
            out_hbm,
            R, T, XN, W, WO, WG, WU, WD, OB, MST, GT, WR, CM, LM, PN, PG, RT,
            K0, Q0, PQ0, PK0, VT0, SA0, SB0, SC0, SD0, RD0, K1, Q1, PQ1, PK1, VT1, SA1, SB1, SC1, SD1, RD1,
            ZS, sx, sw, sm, so):
    bufs = ((K0, Q0, PQ0, PK0, VT0, (SA0, SB0, SC0, SD0), RD0), (K1, Q1, PQ1, PK1, VT1, (SA1, SB1, SC1, SD1), RD1))
    ZS[0] = 0
    XNu = XN.bitcast(U32)
    Wu = W.bitcast(U32)
    WOu = WO.bitcast(U32)
    OBu = OB.bitcast(U32)
    Tu = T.bitcast(U32)

    def x_copy(row0, n, s):
        return pltpu.make_async_copy(x_hbm.at[0, pl.ds(row0, n), :], R.at[pl.ds(row0, n), :], sx.at[s])

    def w_copy(g, j):
        src = (wq_hbm, wk_hbm, wv_hbm)[j]
        return pltpu.make_async_copy(src.at[:, pl.ds(pl.multiple_of(g * 128, 128), 128)], W.at[g, j], sw.at[g, j])

    def wo_copy(n):
        return pltpu.make_async_copy(wo_hbm.at[:, pl.ds(n * 128, 128)], WO.at[n], sm.at[n])

    ffn_copies = (pltpu.make_async_copy(wg_hbm, WG, sm.at[8]),
                  pltpu.make_async_copy(wu_hbm, WU, sm.at[9]),
                  pltpu.make_async_copy(wd_hbm, WD, sm.at[10]))

    def out_copy(row0, n, s):
        return pltpu.make_async_copy(R.at[pl.ds(row0, n), :], out_hbm.at[0, pl.ds(row0, n), :], so.at[s])

    x_copy(0, 128, 0).start()
    w_copy(0, 0).start()
    x_copy(128, 128, 1).start()
    w_copy(0, 1).start()
    w_copy(0, 2).start()
    x_copy(256, 128, 2).start()
    x_copy(384, 128, 3).start()
    for g in (1, 2):
        for j in range(3):
            w_copy(g, j).start()
    x_copy(512, 128, 4).start()
    x_copy(640, 128, 5).start()

    gsig = jax.nn.sigmoid(beta_ref[...].astype(F32).reshape(1, H))
    eye = (jax.lax.broadcasted_iota(jnp.int32, (H, H), 0)
           == jax.lax.broadcasted_iota(jnp.int32, (H, H), 1))
    gcol = jnp.sum(jnp.where(eye, jnp.broadcast_to(gsig, (H, H)), 0.0), axis=1, keepdims=True)
    gfull = jnp.broadcast_to(gcol, (H, 128))
    for g in range(NG):
        GT[g, 0:4, :] = gfull[4 * g:4 * g + 4, :]
        GT[g, 4:8, :] = 1.0 - gfull[4 * g:4 * g + 4, :]
    WR[...] = jnp.broadcast_to(wr_ref[...].astype(F32).reshape(1, D), (8, D))
    kk = jax.lax.broadcasted_iota(jnp.int32, (32, 128), 0)
    qq = jax.lax.broadcasted_iota(jnp.int32, (32, 128), 1) % 32
    CM[...] = jnp.where(qq < kk, NEG, 0.0).astype(F32)
    for c in range(4):
        LM[c] = jnp.where(jax.lax.broadcasted_iota(jnp.int32, (8, 128), 1) // DH == c,
                          jnp.uint32(0xFFFFFFFF), jnp.uint32(0))
        VT0[c, 64:72, :] = pltpu.bitcast(jnp.ones((16, 128), BF16), U32)
        VT1[c, 64:72, :] = pltpu.bitcast(jnp.ones((16, 128), BF16), U32)
    RT[...] = jnp.zeros((16, 128), F32)
    PN[PZ:PZ + 8, :] = jnp.zeros((8, 128), F32)

    def ln_units(row0, nrows, router, slab):
        zz = ZS[0]

        def ld(i, k, v):
            if router:
                r2 = pl.multiple_of(row0 // 2 + 16 * i + zz * v, 16)
                return pltpu.bitcast(Tu[k, pl.ds(r2, 16), :], BF16).astype(F32)
            r1 = pl.multiple_of(row0 + 32 * i + zz * v, 32)
            return R[pl.ds(r1, 32), k * 128:(k + 1) * 128].astype(F32)

        def st_put(i, j, val):
            r = pl.multiple_of((slab + j) * 128 + 32 * i + zz, 32)
            PN[pl.ds(r, 32), :] = jnp.broadcast_to(val, (32, 128))

        def done(val):
            PG[pl.ds(pl.multiple_of(520 + zz, 8), 8), :] = val[24:32]

        def st_get(i, j, v):
            return PN[pl.ds(pl.multiple_of((slab + j) * 128 + 32 * i + zz * v, 32), 32), :]

        def mean(i):
            z = PN[pl.ds(pl.multiple_of(PZ + zz, 8), 8), :]
            acc = jnp.concatenate([z, z, z, z], axis=0)
            for k in range(8):
                acc = acc + ld(i, k, 1)
            done(acc)
            st_put(i, 0, jnp.sum(acc, axis=1, keepdims=True) * (1.0 / D))

        def var(i):
            mu = st_get(i, 0, 2)
            acc = None
            for k in range(8):
                xc = ld(i, k, 2) - mu
                acc = xc * xc if acc is None else acc + xc * xc
            done(acc)
            st_put(i, 0, _rb2(mu))
            st_put(i, 1, _rinv(jnp.sum(acc, axis=1, keepdims=True) * (1.0 / D)))

        def norm(i):
            mu = st_get(i, 0, 3)
            ri = st_get(i, 1, 3)
            acc = None
            for k in range(8):
                x = ld(i, k, 3)
                y = (x - mu) * ri
                if k == 7:
                    PN[pl.ds(pl.multiple_of(PD + 8 + zz, 8), 8), :] = y[24:32]
                    done(y)
                if not router:
                    XN[k, pl.ds(pl.multiple_of(row0 + 32 * i, 32), 32), :] = y.astype(BF16)
                    continue
                y = _rb2(y)
                wr = WR[:, k * 128:(k + 1) * 128]
                yw = y * jnp.concatenate([wr, wr, wr, wr], axis=0)
                acc = yw if acc is None else acc + yw
                R[pl.ds(pl.multiple_of(row0 + 32 * i, 32), 32), k * 128:(k + 1) * 128] = (x + y).astype(BF16)
            if router:
                r = jnp.broadcast_to(_rb(jnp.sum(acc, axis=1, keepdims=True)), (32, 128))
                tok = row0 + 32 * i
                rrow = pl.multiple_of((tok // 1024) * 8, 8)
                lane = jax.lax.broadcasted_iota(jnp.int32, (8, 128), 1) - (tok % 1024) // 8
                v = RT[pl.ds(rrow, 8), :]
                for j in range(4):
                    v = jnp.where(lane == j, r[8 * j:8 * j + 8], v)
                RT[pl.ds(rrow, 8), :] = v

        n = nrows // 32
        return [_bind(f, i) for f in (mean, var, norm) for i in range(n)]

    def proj_rounds(seg, g, buf):
        Kb, Qm, PQ, PK, VT, SB, RD = buf
        zz = ZS[0]
        part = {}

        def rnd(c, j, half):
            r2 = pl.multiple_of(seg * (L // 2) + c * 64 + zz * j, 64)
            xn = jnp.concatenate([pltpu.bitcast(XNu[k, pl.ds(r2, 64), :], BF16)
                                  for k in range(4 * half, 4 * half + 4)], axis=1)
            w = pltpu.bitcast(Wu[g, j, pl.ds(pl.multiple_of(256 * half + zz * c, 256), 256), :], BF16)
            t = jnp.dot(xn, w, preferred_element_type=F32)
            if half == 0:
                part[0] = t
                return
            t = t + part[0]
            PN[PD:PD + 8, :] = t[120:128]
            PG[512:520, :] = t[120:128]
            if j == 0:
                qt = pltpu.bitcast((t * QSCALE).astype(BF16).T, U32)
                for h in range(4):
                    qh = qt[16 * h:16 * h + 16]
                    Qm[c, 16 * h:16 * h + 16, :] = pltpu.roll(qh, 32 * h, 1) if h else qh
                PQ[c * 128:(c + 1) * 128, :] = _phi(t).astype(BF16)
            elif j == 1:
                Kb[c * 128:(c + 1) * 128, :] = t.astype(BF16)
                PK[c * 128:(c + 1) * 128, :] = _phi(t).astype(BF16)
            else:
                VT[c, 0:64, :] = pltpu.bitcast(t.astype(BF16).T, U32)

        return [_bind(rnd, c, j, half) for c in range(4) for j in range(3) for half in range(2)]

    def out_rounds(seg, off, nrows):
        zz = ZS[0]
        part = {}
        n2 = nrows // 2

        def rnd(n, half):
            o2 = pl.multiple_of(((seg % 2) * L + off) // 2 + zz * (n + 1), 16)
            o = jnp.concatenate([pltpu.bitcast(OBu[k, pl.ds(o2, n2), :], BF16)
                                 for k in range(4 * half, 4 * half + 4)], axis=1)
            w = pltpu.bitcast(WOu[n, pl.ds(pl.multiple_of(256 * half + zz * (seg * L + off), 256), 256), :], BF16)
            t = jnp.dot(o, w, preferred_element_type=F32)
            if half == 0:
                part[0] = t
                return
            x = R[pl.ds(pl.multiple_of(seg * L + off, 32), nrows), n * 128:(n + 1) * 128].astype(F32)
            t = t + part[0]
            PN[PD:PD + 8, :] = t[nrows - 8:nrows]
            PG[512:520, :] = t[nrows - 8:nrows]
            T[n, pl.ds(pl.multiple_of(seg * L + off, 32), nrows), :] = (x + _rb2(t)).astype(BF16)

        return [_bind(rnd, n, half) for n in range(8) for half in range(2)]

    def attn(seg, g, buf, mem):
        Kb, Qm, PQ, PK, VT, SB, RD = buf
        Kb, PQ, PK = Kb.bitcast(U32), PQ.bitcast(U32), PK.bitcast(U32)
        zz = ZS[0]
        pg0 = 0 if buf is bufs[0] else 256
        ml = {}
        m8_ = {}
        acc = {}
        fin = {}

        def bfly(e, rows):
            lane = jax.lax.broadcasted_iota(jnp.int32, (rows, 128), 1)
            s0 = (lane & 32) != 0
            s1 = (lane & 64) != 0

            def sel(m, x, y):
                if x is None and y is None:
                    return None
                z = jnp.zeros_like(x if y is None else y)
                return jnp.where(m, z if x is None else x, z if y is None else y)

            a = [[sel(s1, e[2 + j], e[j]), sel(s1, e[j], e[2 + j])] for j in range(2)]
            return [sel(s0, a[1][0], a[0][0]), sel(s0, a[0][0], a[1][1]),
                    sel(s0, a[1][1], a[0][1]), sel(s0, a[0][1], a[1][0])]

        def put_max(qb, m8):
            m = jnp.broadcast_to(jnp.max(m8, axis=0, keepdims=True), (8, 512))
            m = [m[:, 128 * h:128 * (h + 1)] for h in range(4)]
            for i, v in enumerate(m + bfly(m, 8)):
                if qb > 0 or i >= 4:
                    PG[pg0 + 64 * qb + 8 * i:pg0 + 64 * qb + 8 * i + 8, :] = v

        def get_max(i):
            for qb, h in [(dg.index(i), 4 + j) for j in range(4)] if i in dg else [t[:2] for t in tiles(i)]:
                if (i, h) not in ml:
                    ml[(i, h)] = PG[pl.ds(pl.multiple_of(zz * (i + 1) + pg0 + 64 * qb + 8 * h, 8), 8), :]

        def diag(qa):
            lm = [jnp.concatenate([LM[i]] * 2, axis=0) for i in range(4)]
            for qb, rev in ((qa, False), (qa + 1, True)):
                m8 = [None] * 4
                for j in range(3, -1, -1):
                    w = jnp.concatenate([Qm[qb, 16 * h:16 * h + 16, :] & lm[(j + h) % 4] for h in range(4)], axis=0)
                    rs = range(j, -1, -1) if rev else range(j + 1)
                    kq = jnp.concatenate([Kb[64 * qb + 16 * r:64 * qb + 16 * r + 16, :] for r in rs], axis=0)
                    d = jnp.dot(pltpu.bitcast(kq, BF16), pltpu.bitcast(w, BF16), preferred_element_type=F32)
                    for i, r in enumerate(rs):
                        v = d[32 * i:32 * i + 32] + CM[...] if r == j else d[32 * i:32 * i + 32]
                        SB[qb][j, 128 * qb + 32 * r:128 * qb + 32 * r + 32, :] = v
                        mx = jnp.max(v.reshape(4, 8, 128), axis=0)
                        m8[j] = mx if m8[j] is None else jnp.maximum(m8[j], mx)
                m8_[qb] = jnp.concatenate(bfly(m8, 8), axis=1)
            if qa == 0:
                put_max(0, m8_[0])

        def qk(qb):
            z16 = jnp.zeros((16, 128), U32)
            w = jnp.concatenate([jnp.concatenate([Qm[qb, 16 * h:16 * h + 16, :] if i == h else z16
                                                  for i in range(4)], axis=0) for h in range(4)], axis=1)
            s = jnp.dot(pltpu.bitcast(Kb[0:64 * qb, :], BF16), pltpu.bitcast(w, BF16), preferred_element_type=F32)
            m8 = m8_[qb]
            for c in range(qb):
                blk = s[c * 128:(c + 1) * 128, :]
                for h in range(4):
                    SB[qb][h, c * 128:(c + 1) * 128, :] = blk[:, 128 * h:128 * (h + 1)]
                m8 = jnp.maximum(m8, jnp.max(blk.reshape(16, 8, 512), axis=0))
            put_max(qb, m8)

        def pv(qb, h, c, p, l8):
            o = jnp.dot(pltpu.bitcast(VT[c, 16 * h:16 * h + 16, :], BF16), p, preferred_element_type=F32)
            if (qb, h) in acc:
                o0, l0, n = acc[(qb, h)]
                o = o + o0
                l8 = l0 + l8
            else:
                n = 0
            acc[(qb, h)] = (o, l8, n + 1)
            if n == qb:
                gt = GT[g]
                l = jnp.sum(l8, axis=0, keepdims=True)
                res = o * (gt[4 + h:5 + h, :] * _rcp(l))
                if h > 0:
                    res = pltpu.roll(res, 128 - 32 * h, 1)
                if mem:
                    num = RD[zz + qb, 32 * h:32 * h + 32, :]
                    den = RD[zz + qb, 128:136, :][h:h + 1, :] + 1e-06
                    res = num * (gt[h:h + 1, :] * _rcp(den)) + res
                fin[(qb, h)] = res

        def pv_tile(i, qb, h, c):
            m = jnp.concatenate([ml[(i, h)]] * 16, axis=0)
            p = jnp.exp2(SB[qb][h, pl.ds(pl.multiple_of(zz + c * 128, 128), 128), :] - m)
            l8 = p[120:128]
            for r in range(14, -1, -1):
                l8 = l8 + p[8 * r:8 * r + 8]
            pv(qb, h, c, p.astype(BF16), l8)

        def pv_diag(qb):
            m = [ml[(dg[qb], 4 + j)] for j in range(4)]
            l8 = [None] * 4
            w = {}
            for r in range(3, -1, -1):
                e = [None] * 4
                for j in range(r, 4):
                    mj = jnp.concatenate([m[j]] * 2, axis=0)
                    p = [jnp.exp2(SB[qb][j, pl.ds(zz + 128 * qb + 32 * r + i, 16, stride=2), :] - mj)
                         for i in range(2)]
                    for v in (p[1][8:16], p[1][0:8], p[0][8:16], p[0][0:8]):
                        l8[j] = v if l8[j] is None else l8[j] + v
                    e[j] = pltpu.pack_elementwise(p, packed_dtype=BF16)
                w[r] = bfly(e, 16)
            l8 = bfly(l8, 8)
            for h in range(4):
                pv(qb, h, qb, pltpu.bitcast(jnp.concatenate([w[r][h] for r in range(4)], axis=0), BF16), l8[h])

        def put(qb):
            ot = jnp.concatenate([fin[(qb, i)] for i in range(4)], axis=0).astype(BF16)
            o2 = pl.multiple_of((seg % 2) * (L // 2) + 64 * qb, 64)
            OBu[g, pl.ds(o2, 64), :] = pltpu.bitcast(ot.T, U32)

        dg = (0, 1, 3, 6)

        def tiles(i):
            i = (2, 4, 5, 7, 8, 9).index(i)
            return [(qb, h, c) for qb in range(4) for h in range(4) for c in range(qb)][4 * i:4 * i + 4]

        def grp(i):
            get_max(i)
            if i in dg:
                pv_diag(dg.index(i))
                return
            for t in tiles(i):
                pv_tile(i, *t)

        def rd():
            r = jax.lax.dot_general(MST[g].astype(BF16), pltpu.bitcast(PQ[...], BF16), NT, preferred_element_type=F32)
            for c in range(4):
                RD[c] = r[0:136, c * 128:(c + 1) * 128]

        def upd():
            vall = pltpu.bitcast(jnp.concatenate([VT[c] for c in range(4)], axis=1), BF16)
            u = jnp.dot(vall, pltpu.bitcast(PK[...], BF16), preferred_element_type=F32)
            rr = jax.lax.broadcasted_iota(jnp.int32, (144, 128), 0)
            cc = jax.lax.broadcasted_iota(jnp.int32, (144, 128), 1) // DH
            keep = jnp.where(rr < 128, rr // DH, rr - 128) == cc
            u = jnp.where(keep, u, 0.0)
            MST[g] = MST[g + zz] + u if mem else u

        def act(tok):
            if tok[0] == "Q":
                qk(int(tok[1]))
            elif tok[0] == "D":
                diag(int(tok[1]))
            elif tok[0] == "G":
                grp(int(tok[1]))
            elif tok[0] == "g":
                get_max(int(tok[1]))
            elif tok[0] == "S":
                put(int(tok[1]))
            elif tok == "R":
                rd()
            else:
                assert tok == "U"
                upd()

        return act

    def run(sched, steps, queues):
        queues = {k: list(v) for k, v in queues.items()}
        si = 0
        for tok in sched.split():
            if tok == "|":
                si += 1
            elif tok in queues:
                queues[tok].pop(0)()
            elif tok[-1] == "+":
                steps[si + 1](tok[:-1])
            else:
                steps[si](tok)
        assert all(not v for v in queues.values()), {k: len(v) for k, v in queues.items()}

    def ffn_patch(layer):
        r = RT[...]
        sub = jax.lax.broadcasted_iota(jnp.int32, (16, 128), 0)
        idx = (sub // 8) * 1024 + jax.lax.broadcasted_iota(jnp.int32, (16, 128), 1) * 8 + sub % 8
        m1 = jnp.max(r, keepdims=True)
        i1 = jnp.min(jnp.where(r == m1, idx, S - 1))
        r2 = jnp.where(idx == i1, -jnp.inf, r)
        m2 = jnp.max(r2, keepdims=True)
        i2 = jnp.min(jnp.where((r2 == m2) & (idx != i1), idx, S - 1))
        b1 = pl.multiple_of((jnp.clip(i1, 0, S - 1) // 16) * 16, 16)
        b2 = pl.multiple_of((jnp.clip(i2, 0, S - 1) // 16) * 16, 16)
        i16 = jax.lax.broadcasted_iota(jnp.int32, (16, 1), 0)
        s1 = i16 + b1 == i1
        s2 = i16 + b2 == i2

        def pick(b, sel):
            blk = jnp.concatenate([T[k, pl.ds(b, 16), :] for k in range(8)], axis=1)
            row = jnp.sum(jnp.where(sel, blk.astype(F32), 0.0), axis=0, keepdims=True)
            return jnp.broadcast_to(row, (8, D))

        x1 = jnp.concatenate([pick(b1, s1), pick(b2, s2)], axis=0)
        yb = _ln_f32(x1).astype(BF16)
        rsel = jnp.where(i16 < 8, m1, m2)

        def gate_up(c):
            gt = _rb(jnp.dot(yb, WG[:, c * FCH:(c + 1) * FCH], preferred_element_type=F32))
            up = _rb(jnp.dot(yb, WU[:, c * FCH:(c + 1) * FCH], preferred_element_type=F32))
            return (_rb(gt * _rb(jax.nn.sigmoid(gt))) * up).astype(BF16)

        hm = gate_up(0)
        yv = None
        for c in range(NFC):
            nxt = gate_up(c + 1) if c + 1 < NFC else None
            dn = jnp.dot(hm, WD[c * FCH:(c + 1) * FCH, :], preferred_element_type=F32)
            yv = dn if yv is None else yv + dn
            hm = nxt
        yv = _rb(_rb(yv) * _rb(jax.nn.sigmoid(rsel)))
        x2 = _rb(x1 + _rb(yb.astype(F32) + yv))
        xn = _rb(_ln_f32(x2))

        @pl.when(layer == 1)
        def _():
            for s in range(11):
                out_copy(0, 128, s).wait()
            out_copy(0, 640, 11).wait()

        for b, sel, lo in ((b1, s1, 0), (b2, s2, 8)):
            new = jnp.concatenate([x2[lo:lo + 8], x2[lo:lo + 8]], axis=0)
            R[pl.ds(b, 16), :] = jnp.where(sel, new, R[pl.ds(b, 16), :].astype(F32)).astype(BF16)

        @pl.when(layer == 0)
        def _():
            for b, sel, lo in ((b1, s1, 0), (b2, s2, 8)):
                new = jnp.concatenate([xn[lo:lo + 8], xn[lo:lo + 8]], axis=0)
                for k in range(8):
                    XN[k, pl.ds(b, 16), :] = jnp.where(sel, new[:, k * 128:(k + 1) * 128],
                                                       XN[k, pl.ds(b, 16), :].astype(F32)).astype(BF16)
            run("P P m P P m P P m P P m P P m P P m P P m P P m P P P P P P P P", [],
                {"P": proj_rounds(0, 0, bufs[0]), "m": ln_units(L, 128, False, 2)[:8]})

        @pl.when(layer == 1)
        def _():
            c1 = out_copy(b1, 16, 0)
            c1.start()

            @pl.when(b2 != b1)
            def _():
                c2 = out_copy(b2, 16, 1)
                c2.start()
                c2.wait()

            c1.wait()

    p0 = proj_rounds(0, 0, bufs[0])
    x_copy(0, 128, 0).wait()
    for f in ln_units(0, 128, False, 2):
        f()
    for c in range(4):
        if c == 0:
            for j in range(3):
                w_copy(0, j).wait()
        if c < 3:
            x_copy(128 * (c + 1), 128, c + 1).wait()
            run("f f f f P P f f f f P P P P f f f f", [],
                {"P": p0[6 * c:6 * c + 6], "f": ln_units(128 * (c + 1), 128, False, 2)})
        else:
            x_copy(0, 128, 4).wait()
            run("m m m m P P m m P P m m P P", [], {"P": p0[18:24], "m": ln_units(L, 128, False, 2)[:8]})

    def layer_body(layer, carry):
        def a_body(gp, carry2):
            g0 = 2 * gp
            g2 = (g0 + 2) % NG

            @pl.when(layer == 0)
            def _():
                @pl.when(gp < 3)
                def _():
                    for j in range(3):
                        w_copy(g0 + 3, j).start()

                @pl.when(gp < 2)
                def _():
                    for j in range(3):
                        w_copy(g0 + 4, j).start()

                @pl.when(gp < 2)
                def _():
                    x_copy(pl.multiple_of(768 + 128 * gp, 128), 128, 6 + gp).start()

                @pl.when(gp == 1)
                def _():
                    for n in range(8):
                        wo_copy(n).start()

                @pl.when(gp >= 2)
                def _():
                    x_copy(pl.multiple_of(gp * L, L), L, 6 + gp).start()

                for j in range(3):
                    w_copy(g0 + 1, j).wait()

                @pl.when(gp < 3)
                def _():
                    for j in range(3):
                        w_copy(g2, j).wait()
                    x_copy(0, 128, 5 + gp).wait()

                @pl.when(gp == 3)
                def _():
                    x_copy(0, L, 8).wait()

            run(SCHED_A, [attn(0, g0, bufs[0], False), attn(0, g0 + 1, bufs[1], False)],
                {"P": proj_rounds(0, g0 + 1, bufs[1]) + proj_rounds(gp // 3, g2, bufs[0]),
                 "n": ln_units(L + gp * 128, 128, False, 2)[8:],
                 "m": ln_units(L + 128 + gp * 128, 128, False, 2)[:8]})
            return carry2

        jax.lax.fori_loop(0, 4, a_body, 0)

        @pl.when(layer == 0)
        def _():
            for c in ffn_copies:
                c.start()
            for n in range(8):
                wo_copy(n).wait()
            x_copy(0, L, 9).wait()

        def b_body(it, carry2):
            seg = 1 + it // 4
            gp = it % 4
            g0 = 2 * gp
            g2 = (g0 + 2) % NG
            prow = (seg - 1) * L + gp * 128
            run(SCHED_B, [attn(seg, g0, bufs[0], True), attn(seg, g0 + 1, bufs[1], True)],
                {"P": proj_rounds(seg, g0 + 1, bufs[1]) + proj_rounds(seg + gp // 3, g2, bufs[0]),
                 "O": out_rounds(seg - 1, gp * 128, 128),
                 "n": ln_units((1024 + it * 128) % S, 128, False, 2)[8:],
                 "m": ln_units((1152 + it * 128) % S, 128, False, 2)[:8],
                 "t": ln_units(prow, 128, True, 0)})

            @pl.when(layer == 1)
            def _():
                out_copy(pl.multiple_of(prow, 128), 128, it).start()

            return carry2

        jax.lax.fori_loop(0, 11, b_body, 0)

        pieces = ((0, 128), (128, 128), (256, 128), (384, 64), (448, 32), (480, 32))
        run(SCHED_T, [attn(3, 6, bufs[0], True), attn(3, 7, bufs[1], True)],
            {"P": proj_rounds(3, 7, bufs[1]),
             "O": out_rounds(2, 384, 128) + [f for off, n in pieces for f in out_rounds(3, off, n)],
             "n": ln_units(384, 128, False, 2)[8:],
             "t": ln_units(2 * L + 384, 128, True, 0)
             + [f for i, (off, n) in enumerate(pieces)
                for f in ln_units(3 * L + off, n, True, 4 + 2 * (i % 2))]})

        @pl.when(layer == 0)
        def _():
            for c in ffn_copies:
                c.wait()

        @pl.when(layer == 1)
        def _():
            out_copy(S - 640, 640, 11).start()

        ffn_patch(layer)
        return carry

    jax.lax.fori_loop(0, 2, layer_body, 0)


@jax.jit
def pallas_interleave_layers__memory_aug_infini_attn__moe_arch_mod__prompt_kernel(
    A_x: jax.Array,
    A_wq: jax.Array,
    A_wk: jax.Array,
    A_wv: jax.Array,
    A_wo: jax.Array,
    A_beta: jax.Array,
    B_x: jax.Array,
    B_w_r: jax.Array,
    B_w_gate: jax.Array,
    B_w_up: jax.Array,
    B_w_down: jax.Array,
):
    hbm = pl.BlockSpec(memory_space=pl.ANY)
    vmem = pl.BlockSpec(memory_space=pltpu.VMEM)
    qkv_set = [
        pltpu.VMEM((L, 128), BF16),
        pltpu.VMEM((4, 64, 128), U32),
        pltpu.VMEM((L, 128), BF16),
        pltpu.VMEM((L, 128), BF16),
        pltpu.VMEM((4, 72, 128), U32),
        pltpu.VMEM((4, 128, 128), F32),
        pltpu.VMEM((4, 256, 128), F32),
        pltpu.VMEM((4, 384, 128), F32),
        pltpu.VMEM((4, 512, 128), F32),
        pltpu.VMEM((4, 136, 128), F32),
    ]
    scratch = [
        pltpu.VMEM((S, D), BF16),
        pltpu.VMEM((8, S, 128), BF16),
        pltpu.VMEM((8, S, 128), BF16),
        pltpu.VMEM((NG, 3, D, 128), BF16),
        pltpu.VMEM((8, D, 128), BF16),
        pltpu.VMEM((D, FF), BF16),
        pltpu.VMEM((D, FF), BF16),
        pltpu.VMEM((FF, D), BF16),
        pltpu.VMEM((NG, 2 * L, 128), BF16),
        pltpu.VMEM((NG, 144, 128), F32),
        pltpu.VMEM((NG, 8, 128), F32),
        pltpu.VMEM((8, D), F32),
        pltpu.VMEM((32, 128), F32),
        pltpu.VMEM((4, 8, 128), U32),
        pltpu.VMEM((PD + 16, 128), F32),
        pltpu.VMEM((528, 128), F32),
        pltpu.VMEM((16, 128), F32),
    ] + qkv_set + qkv_set + [
        pltpu.SMEM((1,), jnp.int32),
        pltpu.SemaphoreType.DMA((10,)),
        pltpu.SemaphoreType.DMA((NG, 3)),
        pltpu.SemaphoreType.DMA((11,)),
        pltpu.SemaphoreType.DMA((12,)),
    ]
    return pl.pallas_call(
        _kernel,
        out_shape=jax.ShapeDtypeStruct((1, S, D), BF16),
        in_specs=[hbm, hbm, hbm, hbm, hbm, vmem, vmem, hbm, hbm, hbm],
        out_specs=hbm,
        scratch_shapes=scratch,
        compiler_params=pltpu.CompilerParams(vmem_limit_bytes=100 * 1024 * 1024),
    )(A_x, A_wq, A_wk, A_wv, A_wo, A_beta, B_w_r, B_w_gate, B_w_up, B_w_down)
```

```python
import jax
import jax.numpy as jnp
import jax.experimental.pallas as pl
import jax.experimental.pallas.tpu as pltpu

F32 = jnp.float32
BF16 = jnp.bfloat16
U32 = jnp.uint32

S = 2048
D = 1024
H = 32
DH = 32
NSEG = 4
L = S // NSEG
NG = 8
FF = 3584
FCH = 512
NFC = FF // FCH
LOG2E = 1.4426950408889634
QSCALE = (DH ** -0.5) * LOG2E
NEG = -1000000000.0 * LOG2E
EPS_LN = 1.0013580322265625e-05
BIG = 3.0e38
NT = (((1,), (1,)), ((), ()))
PZ = 1024
PD = 1032

SCHED_A = ("D0 g0 n Q1 g1 n D2 n Q2 n G0 S0 P P G1 g2 m P P G2 g3 S1 m P P G3 g4 Q3 m P P G4 g5 m P P G5 g6 S2 m "
           "P P G6 g7 m P P G7 g8 m P P G8 g9 m P P G9 S3 P P D0+ P P Q1+ g0+ P P U | G0 g1 S0 P P D2 G1 g2 P P "
           "Q2 G2 g3 S1 P P G3 g4 P P G4 g5 Q3 P P G5 g6 S2 P P G6 g7 P P G7 g8 P P G8 g9 P P G9 S3 P P P P P P "
           "U ")
SCHED_B = ("O O n O O n m O O n m O O n m O O m m O O m D0 O O g0 m Q1 R O O g1 m G0 S0 P P D2 G1 g2 t t P P Q2 "
           "G2 g3 S1 t t P P G3 g4 t P P G4 g5 Q3 t P P G5 g6 S2 t P P G6 g7 t P P G7 g8 P P G8 g9 P P G9 S3 t P "
           "P D0+ t P P Q1+ g0+ P P U | R G0 g1 S0 P P D2 G1 g2 P P Q2 G2 g3 S1 P P G3 g4 P P G4 g5 Q3 P P G5 g6 "
           "S2 P P G6 g7 P P G7 g8 P P G8 g9 P P G9 S3 t P P t P P P P U ")
SCHED_T = ("O O n O O n O O n D0 Q1 g0 R O O n G0 g1 S0 D2 G1 g2 P P Q2 G2 g3 S1 P P G3 g4 P P G4 g5 Q3 P P G5 "
           "g6 S2 P P G6 g7 P P G7 g8 P P G8 g9 P P G9 S3 P P D0+ P P Q1+ g0+ P P P P | R O O G0 g1 O O S0 D2 G1 "
           "g2 O O Q2 G2 g3 O O S1 G3 g4 O O G4 g5 Q3 t O O G5 g6 t O O S2 G6 g7 t O O G7 g8 t O O G8 g9 t O O "
           "G9 t O O S3 t z O O t z O O t z Z O t z Z O t z Z O t z Z O t z Z O t z Z O t z Z O t z Z O t z O O "
           "t z Z O t z O O z Z O t z Z O t z Z O z Z O t z Z O t z Z O z Z O t z Z O t z Z O t z Z O z Z O t z "
           "Z O z Z O t z Z O t z Z O t z Z O z Z O t z Z O z Z O t z Z O z Z O t z Z O Z O t z O O Z O O O t z "
           "Z O Z O t z O O t z Z O O O t O O Z O O O t Z O Z O t t t ")


def _rb(t):
    return t.astype(BF16).astype(F32)


def _rb2(t):
    n = t.shape[0] // 2
    p = pltpu.pack_elementwise([t[:n], t[n:]], packed_dtype=BF16)
    return jnp.concatenate([pltpu.unpack_elementwise(p, index=i, packed_dtype=BF16, unpacked_dtype=F32)
                            for i in range(2)], axis=0)


def _rcp(d):
    d = jnp.minimum(d, BIG)
    r = pl.reciprocal(d, approx=True)
    return r * (2.0 - d * r)


def _rinv(var):
    v = _rb(_rb(var) + EPS_LN)
    vc = jnp.minimum(v, BIG)
    return jnp.minimum(_rcp(_rb(vc * jax.lax.rsqrt(vc))), 1e30 * pl.reciprocal(v, approx=True))


def _ln_f32(x):
    mu = jnp.sum(x, axis=1, keepdims=True) * (1.0 / D)
    xc = x - mu
    var = jnp.sum(xc * xc, axis=1, keepdims=True) * (1.0 / D)
    return (x - _rb(mu)) * _rinv(var)


def _phi(t):
    return jnp.maximum(t, 0.0) + jnp.exp(jnp.minimum(t, 0.0))


def _bind(f, *a):
    return lambda **kw: f(*a, **kw)


def _kernel(x_hbm, wq_hbm, wk_hbm, wv_hbm, wo_hbm, beta_ref, wr_ref, wg_hbm, wu_hbm, wd_hbm,
            out_hbm,
            R, T, XN, W, WO, WG, WU, WD, OB, MST, GT, WR, CM, LM, PN, PG, RT,
            K0, Q0, PQ0, PK0, VT0, SA0, SB0, SC0, SD0, RD0, K1, Q1, PQ1, PK1, VT1, SA1, SB1, SC1, SD1, RD1,
            OL0, OL1, OL2, OL3, ZS, sx, sw, sm, so):
    bufs = ((K0, Q0, PQ0, PK0, VT0, (SA0, SB0, SC0, SD0), RD0), (K1, Q1, PQ1, PK1, VT1, (SA1, SB1, SC1, SD1), RD1))
    OL = (OL0, OL1, OL2, OL3)
    ZS[0] = 0
    XNu = XN.bitcast(U32)
    Wu = W.bitcast(U32)
    WOu = WO.bitcast(U32)
    OBu = OB.bitcast(U32)
    Tu = T.bitcast(U32)

    def x_copy(row0, n, s):
        return pltpu.make_async_copy(x_hbm.at[0, pl.ds(row0, n), :], R.at[pl.ds(row0, n), :], sx.at[s])

    def w_copy(g, j):
        src = (wq_hbm, wk_hbm, wv_hbm)[j]
        return pltpu.make_async_copy(src.at[:, pl.ds(pl.multiple_of(g * 128, 128), 128)], W.at[g, j], sw.at[g, j])

    def wo_copy(n):
        return pltpu.make_async_copy(wo_hbm.at[:, pl.ds(n * 128, 128)], WO.at[n], sm.at[n])

    ffn_copies = (pltpu.make_async_copy(wg_hbm, WG, sm.at[8]),
                  pltpu.make_async_copy(wu_hbm, WU, sm.at[9]),
                  pltpu.make_async_copy(wd_hbm, WD, sm.at[10]))

    def out_copy(row0, n, s):
        return pltpu.make_async_copy(R.at[pl.ds(row0, n), :], out_hbm.at[0, pl.ds(row0, n), :], so.at[s])

    x_copy(0, 128, 0).start()
    w_copy(0, 0).start()
    x_copy(128, 128, 1).start()
    w_copy(0, 1).start()
    w_copy(0, 2).start()
    x_copy(256, 128, 2).start()
    x_copy(384, 128, 3).start()
    for g in (1, 2):
        for j in range(3):
            w_copy(g, j).start()
    x_copy(512, 128, 4).start()
    x_copy(640, 128, 5).start()

    gsig = jax.nn.sigmoid(beta_ref[...].astype(F32).reshape(1, H))
    eye = (jax.lax.broadcasted_iota(jnp.int32, (H, H), 0)
           == jax.lax.broadcasted_iota(jnp.int32, (H, H), 1))
    gcol = jnp.sum(jnp.where(eye, jnp.broadcast_to(gsig, (H, H)), 0.0), axis=1, keepdims=True)
    gfull = jnp.broadcast_to(gcol, (H, 128))
    for g in range(NG):
        GT[g, 0:4, :] = gfull[4 * g:4 * g + 4, :]
        GT[g, 4:8, :] = 1.0 - gfull[4 * g:4 * g + 4, :]
    WR[...] = jnp.broadcast_to(wr_ref[...].astype(F32).reshape(1, D), (8, D))
    kk = jax.lax.broadcasted_iota(jnp.int32, (32, 128), 0)
    qq = jax.lax.broadcasted_iota(jnp.int32, (32, 128), 1) % 32
    CM[...] = jnp.where(qq < kk, NEG, 0.0).astype(F32)
    for c in range(4):
        LM[c] = jnp.where(jax.lax.broadcasted_iota(jnp.int32, (8, 128), 1) // DH == c,
                          jnp.uint32(0xFFFFFFFF), jnp.uint32(0))
        VT0[c, 64:72, :] = pltpu.bitcast(jnp.ones((16, 128), BF16), U32)
        VT1[c, 64:72, :] = pltpu.bitcast(jnp.ones((16, 128), BF16), U32)
    RT[...] = jnp.zeros((16, 128), F32)
    PN[PZ:PZ + 8, :] = jnp.zeros((8, 128), F32)
    PG[528:536, :] = jnp.zeros((8, 128), F32)
    R[S:S + 16, 0:128] = jnp.zeros((16, 128), BF16)
    T[0, S:S + 16, :] = jnp.zeros((16, 128), BF16)

    def ln_units(row0, nrows, router, slab, late=False):
        zz = ZS[0]

        def ld(i, k, v):
            if router:
                r2 = pl.multiple_of(row0 // 2 + 16 * i + zz * v, 16)
                return pltpu.bitcast(Tu[k, pl.ds(r2, 16), :], BF16).astype(F32)
            r1 = pl.multiple_of(row0 + 32 * i + zz * v, 32)
            return R[pl.ds(r1, 32), k * 128:(k + 1) * 128].astype(F32)

        def st_put(i, j, val):
            r = pl.multiple_of((slab + j) * 128 + 32 * i + zz, 32)
            PN[pl.ds(r, 32), :] = jnp.broadcast_to(val, (32, 128))

        def done(val):
            PG[pl.ds(pl.multiple_of(520 + zz, 8), 8), :] = val[-8:]

        def st_get(i, j, v):
            return PN[pl.ds(pl.multiple_of((slab + j) * 128 + 32 * i + zz * v, 32), 32), :]

        def mean(*ii):
            z = PN[pl.ds(pl.multiple_of(PZ + zz, 8), 8), :]
            accs = []
            for i in ii:
                acc = jnp.concatenate([z, z, z, z], axis=0)
                for k in range(8):
                    acc = acc + ld(i, k, 1)
                accs.append(acc)
            for i, acc in zip(ii, accs):
                done(acc)
                st_put(i, 0, jnp.sum(acc, axis=1, keepdims=True) * (1.0 / D))

        def var(*ii):
            mus = [st_get(i, 0, 2) for i in ii]
            for i, mu in zip(ii, mus):
                acc = None
                for k in range(8):
                    xc = ld(i, k, 2) - mu
                    acc = xc * xc if acc is None else acc + xc * xc
                done(acc)
                st_put(i, 0, _rb2(mu))
                st_put(i, 1, _rinv(jnp.sum(acc, axis=1, keepdims=True) * (1.0 / D)))

        def norm(i):
            mu = st_get(i, 0, 3)
            ri = st_get(i, 1, 3)
            acc = None
            for k in range(8):
                x = ld(i, k, 3)
                y = (x - mu) * ri
                if k == 7:
                    PN[pl.ds(pl.multiple_of(PD + 8 + zz, 8), 8), :] = y[24:32]
                    if not late:
                        done(y)
                if not router:
                    XN[k, pl.ds(pl.multiple_of(row0 + 32 * i, 32), 32), :] = y.astype(BF16)
                    continue
                y = _rb2(y)
                wr = WR[:, k * 128:(k + 1) * 128]
                yw = y * jnp.concatenate([wr, wr, wr, wr], axis=0)
                acc = yw if acc is None else acc + yw
                R[pl.ds(pl.multiple_of(row0 + 32 * i, 32), 32), k * 128:(k + 1) * 128] = (x + y).astype(BF16)
            if router:
                r = jnp.broadcast_to(_rb(jnp.sum(acc, axis=1, keepdims=True)), (32, 128))
                tok = row0 + 32 * i
                rrow = pl.multiple_of((tok // 1024) * 8, 8)
                lane = jax.lax.broadcasted_iota(jnp.int32, (8, 128), 1) - (tok % 1024) // 8
                v = RT[pl.ds(rrow, 8), :]
                for j in range(4):
                    v = jnp.where(lane == j, r[8 * j:8 * j + 8], v)
                RT[pl.ds(rrow, 8), :] = v
                if late:
                    done(v)

        n = nrows // 32
        if late and n > 1:
            return ([_bind(f, i, i + 1) for f in (mean, var) for i in range(0, n, 2)]
                    + [_bind(norm, i) for i in range(n)])
        return [_bind(f, i) for f in (mean, var, norm) for i in range(n)]

    def proj_rounds(seg, g, buf):
        Kb, Qm, PQ, PK, VT, SB, RD = buf
        zz = ZS[0]
        part = {}

        def rnd(c, j, half):
            r2 = pl.multiple_of(seg * (L // 2) + c * 64 + zz * j, 64)
            xn = jnp.concatenate([pltpu.bitcast(XNu[k, pl.ds(r2, 64), :], BF16)
                                  for k in range(4 * half, 4 * half + 4)], axis=1)
            w = pltpu.bitcast(Wu[g, j, pl.ds(pl.multiple_of(256 * half + zz * c, 256), 256), :], BF16)
            t = jnp.dot(xn, w, preferred_element_type=F32)
            if half == 0:
                part[0] = t
                return
            t = t + part[0]
            PN[PD:PD + 8, :] = t[120:128]
            PG[512:520, :] = t[120:128]
            if j == 0:
                qt = pltpu.bitcast((t * QSCALE).astype(BF16).T, U32)
                for h in range(4):
                    qh = qt[16 * h:16 * h + 16]
                    Qm[c, 16 * h:16 * h + 16, :] = pltpu.roll(qh, 32 * h, 1) if h else qh
                PQ[c * 128:(c + 1) * 128, :] = _phi(t).astype(BF16)
            elif j == 1:
                Kb[c * 128:(c + 1) * 128, :] = t.astype(BF16)
                PK[c * 128:(c + 1) * 128, :] = _phi(t).astype(BF16)
            else:
                VT[c, 0:64, :] = pltpu.bitcast(t.astype(BF16).T, U32)

        return [_bind(rnd, c, j, half) for c in range(4) for j in range(3) for half in range(2)]

    pins = [None]

    def pin_load():
        pins.append(pltpu.bitcast(PG[pl.ds(pl.multiple_of(528 + ZS[0], 8), 8), :], U32)
                    | pltpu.bitcast(R[pl.ds(pl.multiple_of(S + ZS[0], 16), 16), 0:128], U32)
                    | Tu[0, pl.ds(pl.multiple_of(S // 2 + ZS[0], 8), 8), :])

    def out_rounds(seg, off, nrows, last=False):
        zz = ZS[0]
        part = {}
        n2 = nrows // 2

        def rnd(n, half, pin=False):
            o2 = pl.multiple_of(((seg % 2) * L + off) // 2 + zz * (n + 1), 16)
            o = [OBu[k, pl.ds(o2, n2), :] for k in range(4 * half, 4 * half + 4 - (last and half))]
            if last and half:
                o.append(OL[off // 128][pl.ds(pl.multiple_of((off % 128) // 2 + zz * (n + 1), 16), n2), :])
            if pin:
                pins[0:2] = pins[1:2]
            if last and pins[0] is not None:
                o = [jnp.concatenate([v[0:8] | pins[0], v[8:]], axis=0) for v in o]
            o = jnp.concatenate([pltpu.bitcast(v, BF16) for v in o], axis=1)
            w = pltpu.bitcast(WOu[n, pl.ds(pl.multiple_of(256 * half + zz * (seg * L + off), 256), 256), :], BF16)
            t = jnp.dot(o, w, preferred_element_type=F32)
            if half == 0:
                part[0] = t
                return
            x = R[pl.ds(pl.multiple_of(seg * L + off, 32), nrows), n * 128:(n + 1) * 128].astype(F32)
            t = t + part[0]
            PN[PD:PD + 8, :] = t[nrows - 8:nrows]
            PG[512:520, :] = t[nrows - 8:nrows]
            T[n, pl.ds(pl.multiple_of(seg * L + off, 32), nrows), :] = (x + _rb2(t)).astype(BF16)

        return [_bind(rnd, n, half) for n in range(8) for half in range(2)]

    def attn(seg, g, buf, mem, last=False):
        Kb, Qm, PQ, PK, VT, SB, RD = buf
        Kb, PQ, PK = Kb.bitcast(U32), PQ.bitcast(U32), PK.bitcast(U32)
        zz = ZS[0]
        pg0 = 0 if buf is bufs[0] else 256
        ml = {}
        m8_ = {}
        acc = {}
        fin = {}

        def bfly(e, rows):
            lane = jax.lax.broadcasted_iota(jnp.int32, (rows, 128), 1)
            s0 = (lane & 32) != 0
            s1 = (lane & 64) != 0

            def sel(m, x, y):
                if x is None and y is None:
                    return None
                z = jnp.zeros_like(x if y is None else y)
                return jnp.where(m, z if x is None else x, z if y is None else y)

            a = [[sel(s1, e[2 + j], e[j]), sel(s1, e[j], e[2 + j])] for j in range(2)]
            return [sel(s0, a[1][0], a[0][0]), sel(s0, a[0][0], a[1][1]),
                    sel(s0, a[1][1], a[0][1]), sel(s0, a[0][1], a[1][0])]

        def put_max(qb, m8):
            m = jnp.broadcast_to(jnp.max(m8, axis=0, keepdims=True), (8, 512))
            m = [m[:, 128 * h:128 * (h + 1)] for h in range(4)]
            for i, v in enumerate(m + bfly(m, 8)):
                if qb > 0 or i >= 4:
                    PG[pg0 + 64 * qb + 8 * i:pg0 + 64 * qb + 8 * i + 8, :] = v

        def get_max(i):
            for qb, h in [(dg.index(i), 4 + j) for j in range(4)] if i in dg else [t[:2] for t in tiles(i)]:
                if (i, h) not in ml:
                    ml[(i, h)] = PG[pl.ds(pl.multiple_of(zz * (i + 1) + pg0 + 64 * qb + 8 * h, 8), 8), :]

        def diag(qa):
            lm = [jnp.concatenate([LM[i]] * 2, axis=0) for i in range(4)]
            for qb, rev in ((qa, False), (qa + 1, True)):
                m8 = [None] * 4
                for j in range(3, -1, -1):
                    w = jnp.concatenate([Qm[qb, 16 * h:16 * h + 16, :] & lm[(j + h) % 4] for h in range(4)], axis=0)
                    rs = range(j, -1, -1) if rev else range(j + 1)
                    kq = jnp.concatenate([Kb[64 * qb + 16 * r:64 * qb + 16 * r + 16, :] for r in rs], axis=0)
                    d = jnp.dot(pltpu.bitcast(kq, BF16), pltpu.bitcast(w, BF16), preferred_element_type=F32)
                    for i, r in enumerate(rs):
                        v = d[32 * i:32 * i + 32] + CM[...] if r == j else d[32 * i:32 * i + 32]
                        SB[qb][j, 128 * qb + 32 * r:128 * qb + 32 * r + 32, :] = v
                        mx = jnp.max(v.reshape(4, 8, 128), axis=0)
                        m8[j] = mx if m8[j] is None else jnp.maximum(m8[j], mx)
                m8_[qb] = jnp.concatenate(bfly(m8, 8), axis=1)
            if qa == 0:
                put_max(0, m8_[0])

        def qk(qb):
            z16 = jnp.zeros((16, 128), U32)
            w = jnp.concatenate([jnp.concatenate([Qm[qb, 16 * h:16 * h + 16, :] if i == h else z16
                                                  for i in range(4)], axis=0) for h in range(4)], axis=1)
            s = jnp.dot(pltpu.bitcast(Kb[0:64 * qb, :], BF16), pltpu.bitcast(w, BF16), preferred_element_type=F32)
            m8 = m8_[qb]
            for c in range(qb):
                blk = s[c * 128:(c + 1) * 128, :]
                for h in range(4):
                    SB[qb][h, c * 128:(c + 1) * 128, :] = blk[:, 128 * h:128 * (h + 1)]
                m8 = jnp.maximum(m8, jnp.max(blk.reshape(16, 8, 512), axis=0))
            put_max(qb, m8)

        def pv(qb, h, c, p, l8):
            o = jnp.dot(pltpu.bitcast(VT[c, 16 * h:16 * h + 16, :], BF16), p, preferred_element_type=F32)
            if (qb, h) in acc:
                o0, l0, n = acc[(qb, h)]
                o = o + o0
                l8 = l0 + l8
            else:
                n = 0
            acc[(qb, h)] = (o, l8, n + 1)
            if n == qb:
                gt = GT[g]
                l = jnp.sum(l8, axis=0, keepdims=True)
                res = o * (gt[4 + h:5 + h, :] * _rcp(l))
                if h > 0:
                    res = pltpu.roll(res, 128 - 32 * h, 1)
                if mem:
                    num = RD[zz + qb, 32 * h:32 * h + 32, :]
                    den = RD[zz + qb, 128:136, :][h:h + 1, :] + 1e-06
                    res = num * (gt[h:h + 1, :] * _rcp(den)) + res
                fin[(qb, h)] = res

        def pv_tile(i, qb, h, c):
            m = jnp.concatenate([ml[(i, h)]] * 16, axis=0)
            p = jnp.exp2(SB[qb][h, pl.ds(pl.multiple_of(zz + c * 128, 128), 128), :] - m)
            l8 = p[120:128]
            for r in range(14, -1, -1):
                l8 = l8 + p[8 * r:8 * r + 8]
            pv(qb, h, c, p.astype(BF16), l8)

        def pv_diag(qb):
            m = [ml[(dg[qb], 4 + j)] for j in range(4)]
            l8 = [None] * 4
            w = {}
            for r in range(3, -1, -1):
                e = [None] * 4
                for j in range(r, 4):
                    mj = jnp.concatenate([m[j]] * 2, axis=0)
                    p = [jnp.exp2(SB[qb][j, pl.ds(zz + 128 * qb + 32 * r + i, 16, stride=2), :] - mj)
                         for i in range(2)]
                    for v in (p[1][8:16], p[1][0:8], p[0][8:16], p[0][0:8]):
                        l8[j] = v if l8[j] is None else l8[j] + v
                    e[j] = pltpu.pack_elementwise(p, packed_dtype=BF16)
                w[r] = bfly(e, 16)
            l8 = bfly(l8, 8)
            for h in range(4):
                pv(qb, h, qb, pltpu.bitcast(jnp.concatenate([w[r][h] for r in range(4)], axis=0), BF16), l8[h])

        def put(qb):
            ot = jnp.concatenate([fin[(qb, i)] for i in range(4)], axis=0).astype(BF16)
            if last:
                ot = pltpu.bitcast(ot.T, U32)
                OL[qb][...] = ot
                PG[pl.ds(pl.multiple_of(520 + zz, 8), 8), :] = pltpu.bitcast(ot[56:64], F32)
                return
            o2 = pl.multiple_of((seg % 2) * (L // 2) + 64 * qb, 64)
            OBu[g, pl.ds(o2, 64), :] = pltpu.bitcast(ot.T, U32)

        dg = (0, 1, 3, 6)

        def tiles(i):
            i = (2, 4, 5, 7, 8, 9).index(i)
            return [(qb, h, c) for qb in range(4) for h in range(4) for c in range(qb)][4 * i:4 * i + 4]

        def grp(i):
            get_max(i)
            if i in dg:
                pv_diag(dg.index(i))
                return
            for t in tiles(i):
                pv_tile(i, *t)

        def rd():
            r = jax.lax.dot_general(MST[g].astype(BF16), pltpu.bitcast(PQ[...], BF16), NT, preferred_element_type=F32)
            for c in range(4):
                RD[c] = r[0:136, c * 128:(c + 1) * 128]

        def upd():
            vall = pltpu.bitcast(jnp.concatenate([VT[c] for c in range(4)], axis=1), BF16)
            u = jnp.dot(vall, pltpu.bitcast(PK[...], BF16), preferred_element_type=F32)
            rr = jax.lax.broadcasted_iota(jnp.int32, (144, 128), 0)
            cc = jax.lax.broadcasted_iota(jnp.int32, (144, 128), 1) // DH
            keep = jnp.where(rr < 128, rr // DH, rr - 128) == cc
            u = jnp.where(keep, u, 0.0)
            MST[g] = MST[g + zz] + u if mem else u

        def act(tok):
            if tok[0] == "Q":
                qk(int(tok[1]))
            elif tok[0] == "D":
                diag(int(tok[1]))
            elif tok[0] == "G":
                grp(int(tok[1]))
            elif tok[0] == "g":
                get_max(int(tok[1]))
            elif tok[0] == "S":
                put(int(tok[1]))
            elif tok == "R":
                rd()
            else:
                assert tok == "U"
                upd()

        return act

    def run(sched, steps, queues):
        queues = {k: list(v) for k, v in queues.items()}
        si = 0
        for tok in sched.split():
            if tok == "|":
                si += 1
            elif tok == "z":
                pin_load()
            elif tok == "Z":
                queues["O"].pop(0)(pin=True)
            elif tok in queues:
                queues[tok].pop(0)()
            elif tok[-1] == "+":
                steps[si + 1](tok[:-1])
            else:
                steps[si](tok)
        assert all(not v for v in queues.values()), {k: len(v) for k, v in queues.items()}

    def ffn_patch(layer):
        r = RT[...]
        sub = jax.lax.broadcasted_iota(jnp.int32, (16, 128), 0)
        idx = (sub // 8) * 1024 + jax.lax.broadcasted_iota(jnp.int32, (16, 128), 1) * 8 + sub % 8
        m1 = jnp.max(r, keepdims=True)
        i1 = jnp.min(jnp.where(r == m1, idx, S - 1))
        r2 = jnp.where(idx == i1, -jnp.inf, r)
        m2 = jnp.max(r2, keepdims=True)
        i2 = jnp.min(jnp.where((r2 == m2) & (idx != i1), idx, S - 1))
        b1 = pl.multiple_of((jnp.clip(i1, 0, S - 1) // 16) * 16, 16)
        b2 = pl.multiple_of((jnp.clip(i2, 0, S - 1) // 16) * 16, 16)
        i16 = jax.lax.broadcasted_iota(jnp.int32, (16, 1), 0)
        s1 = i16 + b1 == i1
        s2 = i16 + b2 == i2

        def pick(b, sel):
            blk = jnp.concatenate([T[k, pl.ds(b, 16), :] for k in range(8)], axis=1)
            row = jnp.sum(jnp.where(sel, blk.astype(F32), 0.0), axis=0, keepdims=True)
            return jnp.broadcast_to(row, (8, D))

        x1 = jnp.concatenate([pick(b1, s1), pick(b2, s2)], axis=0)
        yb = _ln_f32(x1).astype(BF16)
        rsel = jnp.where(i16 < 8, m1, m2)

        def dot512(x, ref, r, c):
            return jnp.dot(x, ref[512 * r:512 * (r + 1), 128 * c:128 * (c + 1)], preferred_element_type=F32)

        def gate_up(c):
            hs = []
            for n in range(4 * c, 4 * c + 4):
                gt, up = [_rb(dot512(yb[:, :512], w, 0, n) + dot512(yb[:, 512:], w, 1, n)) for w in (WG, WU)]
                hs.append(_rb(gt * _rb(jax.nn.sigmoid(gt))) * up)
            return jnp.concatenate(hs, axis=1).astype(BF16)

        hm = gate_up(0)
        yv = None
        for c in range(NFC):
            nxt = gate_up(c + 1) if c + 1 < NFC else None
            dn = jnp.concatenate([dot512(hm, WD, c, n) for n in range(8)], axis=1)
            yv = dn if yv is None else yv + dn
            hm = nxt
        yv = _rb(_rb(yv) * _rb(jax.nn.sigmoid(rsel)))
        x2 = _rb(x1 + _rb(yb.astype(F32) + yv))
        xn = _rb(_ln_f32(x2))

        @pl.when(layer == 1)
        def _():
            for s in range(11):
                out_copy(0, 128, s).wait()
            out_copy(0, 640, 11).wait()

        for b, sel, lo in ((b1, s1, 0), (b2, s2, 8)):
            new = jnp.concatenate([x2[lo:lo + 8], x2[lo:lo + 8]], axis=0)
            R[pl.ds(b, 16), :] = jnp.where(sel, new, R[pl.ds(b, 16), :].astype(F32)).astype(BF16)

        @pl.when(layer == 0)
        def _():
            for b, sel, lo in ((b1, s1, 0), (b2, s2, 8)):
                new = jnp.concatenate([xn[lo:lo + 8], xn[lo:lo + 8]], axis=0)
                for k in range(8):
                    XN[k, pl.ds(b, 16), :] = jnp.where(sel, new[:, k * 128:(k + 1) * 128],
                                                       XN[k, pl.ds(b, 16), :].astype(F32)).astype(BF16)
            run("P P m P P m P P m P P m P P m P P m P P m P P m P P P P P P P P", [],
                {"P": proj_rounds(0, 0, bufs[0]), "m": ln_units(L, 128, False, 2)[:8]})

        @pl.when(layer == 1)
        def _():
            c1 = out_copy(b1, 16, 0)
            c1.start()

            @pl.when(b2 != b1)
            def _():
                c2 = out_copy(b2, 16, 1)
                c2.start()
                c2.wait()

            c1.wait()

    p0 = proj_rounds(0, 0, bufs[0])
    x_copy(0, 128, 0).wait()
    for f in ln_units(0, 128, False, 2):
        f()
    for c in range(4):
        if c == 0:
            for j in range(3):
                w_copy(0, j).wait()
        if c < 3:
            x_copy(128 * (c + 1), 128, c + 1).wait()
            run("f f f f P P f f f f P P P P f f f f", [],
                {"P": p0[6 * c:6 * c + 6], "f": ln_units(128 * (c + 1), 128, False, 2)})
        else:
            x_copy(0, 128, 4).wait()
            run("m m m m P P m m P P m m P P", [], {"P": p0[18:24], "m": ln_units(L, 128, False, 2)[:8]})

    def layer_body(layer, carry):
        def a_body(gp, carry2):
            g0 = 2 * gp
            g2 = (g0 + 2) % NG

            @pl.when(layer == 0)
            def _():
                @pl.when(gp < 3)
                def _():
                    for j in range(3):
                        w_copy(g0 + 3, j).start()

                @pl.when(gp < 2)
                def _():
                    for j in range(3):
                        w_copy(g0 + 4, j).start()

                @pl.when(gp < 2)
                def _():
                    x_copy(pl.multiple_of(768 + 128 * gp, 128), 128, 6 + gp).start()

                @pl.when(gp == 1)
                def _():
                    for n in range(8):
                        wo_copy(n).start()

                @pl.when(gp >= 2)
                def _():
                    x_copy(pl.multiple_of(gp * L, L), L, 6 + gp).start()

                for j in range(3):
                    w_copy(g0 + 1, j).wait()

                @pl.when(gp < 3)
                def _():
                    for j in range(3):
                        w_copy(g2, j).wait()
                    x_copy(0, 128, 5 + gp).wait()

                @pl.when(gp == 3)
                def _():
                    x_copy(0, L, 8).wait()

            run(SCHED_A, [attn(0, g0, bufs[0], False), attn(0, g0 + 1, bufs[1], False)],
                {"P": proj_rounds(0, g0 + 1, bufs[1]) + proj_rounds(gp // 3, g2, bufs[0]),
                 "n": ln_units(L + gp * 128, 128, False, 2)[8:],
                 "m": ln_units(L + 128 + gp * 128, 128, False, 2)[:8]})
            return carry2

        jax.lax.fori_loop(0, 4, a_body, 0)

        @pl.when(layer == 0)
        def _():
            for c in ffn_copies:
                c.start()
            for n in range(8):
                wo_copy(n).wait()
            x_copy(0, L, 9).wait()

        def b_body(it, carry2):
            seg = 1 + it // 4
            gp = it % 4
            g0 = 2 * gp
            g2 = (g0 + 2) % NG
            prow = (seg - 1) * L + gp * 128
            run(SCHED_B, [attn(seg, g0, bufs[0], True), attn(seg, g0 + 1, bufs[1], True)],
                {"P": proj_rounds(seg, g0 + 1, bufs[1]) + proj_rounds(seg + gp // 3, g2, bufs[0]),
                 "O": out_rounds(seg - 1, gp * 128, 128),
                 "n": ln_units((1024 + it * 128) % S, 128, False, 2)[8:],
                 "m": ln_units((1152 + it * 128) % S, 128, False, 2)[:8],
                 "t": ln_units(prow, 128, True, 0)})

            @pl.when(layer == 1)
            def _():
                out_copy(pl.multiple_of(prow, 128), 128, it).start()

            return carry2

        jax.lax.fori_loop(0, 11, b_body, 0)

        pieces = ((0, 128), (128, 128), (256, 64), (320, 64), (384, 64), (448, 32), (480, 32))
        run(SCHED_T, [attn(3, 6, bufs[0], True), attn(3, 7, bufs[1], True, True)],
            {"P": proj_rounds(3, 7, bufs[1]),
             "O": out_rounds(2, 384, 128) + [f for off, n in pieces for f in out_rounds(3, off, n, True)],
             "n": ln_units(384, 128, False, 2)[8:],
             "t": ln_units(2 * L + 384, 128, True, 0, True)
             + [f for i, (off, n) in enumerate(pieces)
                for f in ln_units(3 * L + off, n, True, 4 + 2 * (i % 2), True)]})

        @pl.when(layer == 0)
        def _():
            for c in ffn_copies:
                c.wait()

        @pl.when(layer == 1)
        def _():
            out_copy(S - 640, 640, 11).start()

        ffn_patch(layer)
        return carry

    jax.lax.fori_loop(0, 2, layer_body, 0)


@jax.jit
def pallas_interleave_layers__memory_aug_infini_attn__moe_arch_mod__prompt_kernel(
    A_x: jax.Array,
    A_wq: jax.Array,
    A_wk: jax.Array,
    A_wv: jax.Array,
    A_wo: jax.Array,
    A_beta: jax.Array,
    B_x: jax.Array,
    B_w_r: jax.Array,
    B_w_gate: jax.Array,
    B_w_up: jax.Array,
    B_w_down: jax.Array,
):
    hbm = pl.BlockSpec(memory_space=pl.ANY)
    vmem = pl.BlockSpec(memory_space=pltpu.VMEM)
    qkv_set = [
        pltpu.VMEM((L, 128), BF16),
        pltpu.VMEM((4, 64, 128), U32),
        pltpu.VMEM((L, 128), BF16),
        pltpu.VMEM((L, 128), BF16),
        pltpu.VMEM((4, 72, 128), U32),
        pltpu.VMEM((4, 128, 128), F32),
        pltpu.VMEM((4, 256, 128), F32),
        pltpu.VMEM((4, 384, 128), F32),
        pltpu.VMEM((4, 512, 128), F32),
        pltpu.VMEM((4, 136, 128), F32),
    ]
    scratch = [
        pltpu.VMEM((S + 16, D), BF16),
        pltpu.VMEM((8, S + 16, 128), BF16),
        pltpu.VMEM((8, S, 128), BF16),
        pltpu.VMEM((NG, 3, D, 128), BF16),
        pltpu.VMEM((8, D, 128), BF16),
        pltpu.VMEM((D, FF), BF16),
        pltpu.VMEM((D, FF), BF16),
        pltpu.VMEM((FF, D), BF16),
        pltpu.VMEM((NG, 2 * L, 128), BF16),
        pltpu.VMEM((NG, 144, 128), F32),
        pltpu.VMEM((NG, 8, 128), F32),
        pltpu.VMEM((8, D), F32),
        pltpu.VMEM((32, 128), F32),
        pltpu.VMEM((4, 8, 128), U32),
        pltpu.VMEM((PD + 16, 128), F32),
        pltpu.VMEM((536, 128), F32),
        pltpu.VMEM((16, 128), F32),
    ] + qkv_set + qkv_set + [pltpu.VMEM((64, 128), U32)] * 4 + [
        pltpu.SMEM((1,), jnp.int32),
        pltpu.SemaphoreType.DMA((10,)),
        pltpu.SemaphoreType.DMA((NG, 3)),
        pltpu.SemaphoreType.DMA((11,)),
        pltpu.SemaphoreType.DMA((12,)),
    ]
    return pl.pallas_call(
        _kernel,
        out_shape=jax.ShapeDtypeStruct((1, S, D), BF16),
        in_specs=[hbm, hbm, hbm, hbm, hbm, vmem, vmem, hbm, hbm, hbm],
        out_specs=hbm,
        scratch_shapes=scratch,
        compiler_params=pltpu.CompilerParams(vmem_limit_bytes=100 * 1024 * 1024),
    )(A_x, A_wq, A_wk, A_wv, A_wo, A_beta, B_w_r, B_w_gate, B_w_up, B_w_down)
```

```python
import jax
import jax.numpy as jnp
import jax.experimental.pallas as pl
import jax.experimental.pallas.tpu as pltpu

F32 = jnp.float32
BF16 = jnp.bfloat16
U32 = jnp.uint32

S = 2048
D = 1024
H = 32
DH = 32
NSEG = 4
L = S // NSEG
NG = 8
FF = 3584
FCH = 512
NFC = FF // FCH
LOG2E = 1.4426950408889634
QSCALE = (DH ** -0.5) * LOG2E
NEG = -1000000000.0 * LOG2E
EPS_LN = 1.0013580322265625e-05
BIG = 3.0e38
NT = (((1,), (1,)), ((), ()))
PZ = 1024
PD = 1032

SCHED_A = ("D0 g0 n Q1 g1 n D2 n Q2 n G0 S0 P P G1 g2 m P P G2 g3 S1 m P P G3 g4 Q3 m P P G4 g5 m P P G5 g6 S2 m "
           "P P G6 g7 m P P G7 g8 m P P G8 g9 m P P G9 S3 P P D0+ P P Q1+ g0+ P P U | G0 g1 S0 P P D2 G1 g2 P P "
           "Q2 G2 g3 S1 P P G3 g4 P P G4 g5 Q3 P P G5 g6 S2 P P G6 g7 P P G7 g8 P P G8 g9 P P G9 S3 P P P P P P "
           "U ")
SCHED_B = ("O O n O O n m O O n m O O n m O O m m O O m D0 O O g0 m Q1 R O O g1 m G0 S0 P P D2 G1 g2 t t P P Q2 "
           "G2 g3 S1 t t P P G3 g4 t P P G4 g5 Q3 t P P G5 g6 S2 t P P G6 g7 t P P G7 g8 P P G8 g9 P P G9 S3 t P "
           "P D0+ t P P Q1+ g0+ P P U | R G0 g1 S0 P P D2 G1 g2 P P Q2 G2 g3 S1 P P G3 g4 P P G4 g5 Q3 P P G5 g6 "
           "S2 P P G6 g7 P P G7 g8 P P G8 g9 P P G9 S3 t P P t P P P P U ")
SCHED_T = ("O O n O O n O O n D0 Q1 g0 R O O n G0 g1 S0 D2 G1 g2 P P Q2 G2 g3 S1 P P G3 g4 P P G4 g5 Q3 P P G5 "
           "g6 S2 P P G6 g7 P P G7 g8 P P G8 g9 P P G9 S3 P P D0+ P P Q1+ g0+ P P P P | R O O G0 g1 O O S0 D2 G1 "
           "g2 O O Q2 G2 g3 O O S1 G3 g4 O O G4 g5 Q3 t t O O G5 g6 t t t O O S2 G6 g7 t O O G7 g8 t O O G8 g9 t "
           "O O G9 t O O S3 t z O O t t z O O t z Z O t z Z O t z Z O t z Z O t z Z O t z Z O t z Z O t z Z O t "
           "z O O t z Z O t z O O z Z O t z Z O t z Z O z Z O t z Z O t z Z O z Z O t z Z O t z Z O t z Z O z Z "
           "O t z Z O z Z O t z Z O t z Z O t z Z O z Z O t z Z O z Z O t z Z O z Z O t z Z O Z O t z O O Z O O "
           "O t z Z O Z O t z O O t z Z O O O t O O Z O O O t Z O Z O t t t ")


def _rb(t):
    return t.astype(BF16).astype(F32)


def _rb2(t):
    n = t.shape[0] // 2
    p = pltpu.pack_elementwise([t[:n], t[n:]], packed_dtype=BF16)
    return jnp.concatenate([pltpu.unpack_elementwise(p, index=i, packed_dtype=BF16, unpacked_dtype=F32)
                            for i in range(2)], axis=0)


def _rcp(d):
    d = jnp.minimum(d, BIG)
    r = pl.reciprocal(d, approx=True)
    return r * (2.0 - d * r)


def _rinv(var):
    v = _rb(_rb(var) + EPS_LN)
    vc = jnp.minimum(v, BIG)
    return jnp.minimum(_rcp(_rb(vc * jax.lax.rsqrt(vc))), 1e30 * pl.reciprocal(v, approx=True))


def _ln_f32(x):
    mu = jnp.sum(x, axis=1, keepdims=True) * (1.0 / D)
    xc = x - mu
    var = jnp.sum(xc * xc, axis=1, keepdims=True) * (1.0 / D)
    return (x - _rb(mu)) * _rinv(var)


def _phi(t):
    return jnp.maximum(t, 0.0) + jnp.exp(jnp.minimum(t, 0.0))


def _bind(f, *a):
    return lambda **kw: f(*a, **kw)


def _kernel(x_hbm, wq_hbm, wk_hbm, wv_hbm, wo_hbm, beta_ref, wr_ref, wg_hbm, wu_hbm, wd_hbm,
            out_hbm,
            R, T, XN, W, WO, WG, WU, WD, OB, MST, GT, WR, CM, LM, PN, PG, RT,
            K0, Q0, PQ0, PK0, VT0, SA0, SB0, SC0, SD0, RD0, K1, Q1, PQ1, PK1, VT1, SA1, SB1, SC1, SD1, RD1,
            OL0, OL1, OL2, OL3, PS, ZS, sx, sw, sm, so):
    bufs = ((K0, Q0, PQ0, PK0, VT0, (SA0, SB0, SC0, SD0), RD0), (K1, Q1, PQ1, PK1, VT1, (SA1, SB1, SC1, SD1), RD1))
    OL = (OL0, OL1, OL2, OL3)
    ZS[0] = 0
    XNu = XN.bitcast(U32)
    Wu = W.bitcast(U32)
    WOu = WO.bitcast(U32)
    OBu = OB.bitcast(U32)
    Tu = T.bitcast(U32)

    def x_copy(row0, n, s):
        return pltpu.make_async_copy(x_hbm.at[0, pl.ds(row0, n), :], R.at[pl.ds(row0, n), :], sx.at[s])

    def w_copy(g, j):
        src = (wq_hbm, wk_hbm, wv_hbm)[j]
        return pltpu.make_async_copy(src.at[:, pl.ds(pl.multiple_of(g * 128, 128), 128)], W.at[g, j], sw.at[g, j])

    def wo_copy(n):
        return pltpu.make_async_copy(wo_hbm.at[:, pl.ds(n * 128, 128)], WO.at[n], sm.at[n])

    ffn_copies = (pltpu.make_async_copy(wg_hbm, WG, sm.at[8]),
                  pltpu.make_async_copy(wu_hbm, WU, sm.at[9]),
                  pltpu.make_async_copy(wd_hbm, WD, sm.at[10]))

    def out_copy(row0, n, s):
        return pltpu.make_async_copy(R.at[pl.ds(row0, n), :], out_hbm.at[0, pl.ds(row0, n), :], so.at[s])

    x_copy(0, 128, 0).start()
    w_copy(0, 0).start()
    x_copy(128, 128, 1).start()
    w_copy(0, 1).start()
    w_copy(0, 2).start()
    x_copy(256, 128, 2).start()
    x_copy(384, 128, 3).start()
    for g in (1, 2):
        for j in range(3):
            w_copy(g, j).start()
    x_copy(512, 128, 4).start()
    x_copy(640, 128, 5).start()

    gsig = jax.nn.sigmoid(beta_ref[...].astype(F32).reshape(1, H))
    eye = (jax.lax.broadcasted_iota(jnp.int32, (H, H), 0)
           == jax.lax.broadcasted_iota(jnp.int32, (H, H), 1))
    gcol = jnp.sum(jnp.where(eye, jnp.broadcast_to(gsig, (H, H)), 0.0), axis=1, keepdims=True)
    gfull = jnp.broadcast_to(gcol, (H, 128))
    for g in range(NG):
        GT[g, 0:4, :] = gfull[4 * g:4 * g + 4, :]
        GT[g, 4:8, :] = 1.0 - gfull[4 * g:4 * g + 4, :]
    WR[...] = jnp.broadcast_to(wr_ref[...].astype(F32).reshape(1, D), (8, D))
    kk = jax.lax.broadcasted_iota(jnp.int32, (32, 128), 0)
    qq = jax.lax.broadcasted_iota(jnp.int32, (32, 128), 1) % 32
    CM[...] = jnp.where(qq < kk, NEG, 0.0).astype(F32)
    for c in range(4):
        LM[c] = jnp.where(jax.lax.broadcasted_iota(jnp.int32, (8, 128), 1) // DH == c,
                          jnp.uint32(0xFFFFFFFF), jnp.uint32(0))
        VT0[c, 64:72, :] = pltpu.bitcast(jnp.ones((16, 128), BF16), U32)
        VT1[c, 64:72, :] = pltpu.bitcast(jnp.ones((16, 128), BF16), U32)
    RT[...] = jnp.zeros((16, 128), F32)
    PN[PZ:PZ + 8, :] = jnp.zeros((8, 128), F32)
    PG[528:536, :] = jnp.zeros((8, 128), F32)
    R[S:S + 16, 0:128] = jnp.zeros((16, 128), BF16)
    T[0, S:S + 16, :] = jnp.zeros((16, 128), BF16)

    def ln_units(row0, nrows, router, slab, late=0):
        zz = ZS[0]
        st = PS if late else PN

        def ld(i, k, v):
            if router:
                r2 = pl.multiple_of(row0 // 2 + 16 * i + zz * v, 16)
                return pltpu.bitcast(Tu[k, pl.ds(r2, 16), :], BF16).astype(F32)
            r1 = pl.multiple_of(row0 + 32 * i + zz * v, 32)
            return R[pl.ds(r1, 32), k * 128:(k + 1) * 128].astype(F32)

        def st_put(i, j, val):
            r = pl.multiple_of((slab + j) * 128 + 32 * i + zz, 32)
            st[pl.ds(r, 32), :] = jnp.broadcast_to(val, (32, 128))

        def done(val):
            PG[pl.ds(pl.multiple_of(520 + zz, 8), 8), :] = val[-8:]

        def st_get(i, j, v):
            return st[pl.ds(pl.multiple_of((slab + j) * 128 + 32 * i + zz * v, 32), 32), :]

        def mean(*ii):
            z = PN[pl.ds(pl.multiple_of(PZ + zz, 8), 8), :]
            accs = []
            for i in ii:
                acc = jnp.concatenate([z, z, z, z], axis=0)
                for k in range(8):
                    acc = acc + ld(i, k, 1)
                accs.append(acc)
            for i, acc in zip(ii, accs):
                done(acc)
                st_put(i, 0, jnp.sum(acc, axis=1, keepdims=True) * (1.0 / D))

        def var(*ii):
            mus = [st_get(i, 0, 2) for i in ii]
            for i, mu in zip(ii, mus):
                acc = None
                for k in range(8):
                    xc = ld(i, k, 2) - mu
                    acc = xc * xc if acc is None else acc + xc * xc
                done(acc)
                st_put(i, 1, _rinv(jnp.sum(acc, axis=1, keepdims=True) * (1.0 / D)))

        def norm(i):
            mu = _rb2(st_get(i, 0, 3))
            ri = st_get(i, 1, 3)
            acc = None
            for k in range(8):
                x = ld(i, k, 3)
                y = (x - mu) * ri
                if k == 7 and not late:
                    PN[pl.ds(pl.multiple_of(PD + 8 + zz, 8), 8), :] = y[24:32]
                    done(y)
                if not router:
                    XN[k, pl.ds(pl.multiple_of(row0 + 32 * i, 32), 32), :] = y.astype(BF16)
                    continue
                y = _rb2(y)
                wr = WR[:, k * 128:(k + 1) * 128]
                yw = y * jnp.concatenate([wr, wr, wr, wr], axis=0)
                acc = yw if acc is None else acc + yw
                R[pl.ds(pl.multiple_of(row0 + 32 * i, 32), 32), k * 128:(k + 1) * 128] = (x + y).astype(BF16)
            if router:
                r = jnp.broadcast_to(_rb(jnp.sum(acc, axis=1, keepdims=True)), (32, 128))
                tok = row0 + 32 * i
                rrow = pl.multiple_of((tok // 1024) * 8, 8)
                lane = jax.lax.broadcasted_iota(jnp.int32, (8, 128), 1) - (tok % 1024) // 8
                v = RT[pl.ds(rrow, 8), :]
                for j in range(4):
                    v = jnp.where(lane == j, r[8 * j:8 * j + 8], v)
                RT[pl.ds(rrow, 8), :] = v
                if late:
                    done(v)

        n = nrows // 32
        if late > 1 and n > 1:
            return ([_bind(f, i, i + 1) for f in (mean, var) for i in range(0, n, 2)]
                    + [_bind(norm, i) for i in range(n)])
        return [_bind(f, i) for f in (mean, var, norm) for i in range(n)]

    def proj_rounds(seg, g, buf):
        Kb, Qm, PQ, PK, VT, SB, RD = buf
        zz = ZS[0]
        part = {}

        def rnd(c, j, half):
            r2 = pl.multiple_of(seg * (L // 2) + c * 64 + zz * j, 64)
            xn = jnp.concatenate([pltpu.bitcast(XNu[k, pl.ds(r2, 64), :], BF16)
                                  for k in range(4 * half, 4 * half + 4)], axis=1)
            w = pltpu.bitcast(Wu[g, j, pl.ds(pl.multiple_of(256 * half + zz * c, 256), 256), :], BF16)
            t = jnp.dot(xn, w, preferred_element_type=F32)
            if half == 0:
                part[0] = t
                return
            t = t + part[0]
            PN[PD:PD + 8, :] = t[120:128]
            PG[512:520, :] = t[120:128]
            if j == 0:
                qt = pltpu.bitcast((t * QSCALE).astype(BF16).T, U32)
                for h in range(4):
                    qh = qt[16 * h:16 * h + 16]
                    Qm[c, 16 * h:16 * h + 16, :] = pltpu.roll(qh, 32 * h, 1) if h else qh
                PQ[c * 128:(c + 1) * 128, :] = _phi(t).astype(BF16)
            elif j == 1:
                Kb[c * 128:(c + 1) * 128, :] = t.astype(BF16)
                PK[c * 128:(c + 1) * 128, :] = _phi(t).astype(BF16)
            else:
                VT[c, 0:64, :] = pltpu.bitcast(t.astype(BF16).T, U32)

        return [_bind(rnd, c, j, half) for c in range(4) for j in range(3) for half in range(2)]

    pins = [None]

    def pin_load():
        pins.append(pltpu.bitcast(PG[pl.ds(pl.multiple_of(528 + ZS[0], 8), 8), :], U32)
                    | pltpu.bitcast(R[pl.ds(pl.multiple_of(S + ZS[0], 16), 16), 0:128], U32)
                    | Tu[0, pl.ds(pl.multiple_of(S // 2 + ZS[0], 8), 8), :])

    def out_rounds(seg, off, nrows, last=False):
        zz = ZS[0]
        part = {}
        n2 = nrows // 2

        def rnd(n, half, pin=False):
            o2 = pl.multiple_of(((seg % 2) * L + off) // 2 + zz * (n + 1), 16)
            o = [OBu[k, pl.ds(o2, n2), :] for k in range(4 * half, 4 * half + 4 - (last and half))]
            if last and half:
                o.append(OL[off // 128][pl.ds(pl.multiple_of((off % 128) // 2 + zz * (n + 1), 16), n2), :])
            if pin:
                pins[0:2] = pins[1:2]
            if last and pins[0] is not None:
                o = [jnp.concatenate([v[0:8] | pins[0], v[8:]], axis=0) for v in o]
            o = jnp.concatenate([pltpu.bitcast(v, BF16) for v in o], axis=1)
            w = pltpu.bitcast(WOu[n, pl.ds(pl.multiple_of(256 * half + zz * (seg * L + off), 256), 256), :], BF16)
            t = jnp.dot(o, w, preferred_element_type=F32)
            if half == 0:
                part[0] = t
                return
            x = R[pl.ds(pl.multiple_of(seg * L + off, 32), nrows), n * 128:(n + 1) * 128].astype(F32)
            t = t + part[0]
            PN[PD:PD + 8, :] = t[nrows - 8:nrows]
            PG[512:520, :] = t[nrows - 8:nrows]
            T[n, pl.ds(pl.multiple_of(seg * L + off, 32), nrows), :] = (x + _rb2(t)).astype(BF16)

        return [_bind(rnd, n, half) for n in range(8) for half in range(2)]

    def attn(seg, g, buf, mem, last=False):
        Kb, Qm, PQ, PK, VT, SB, RD = buf
        Kb, PQ, PK = Kb.bitcast(U32), PQ.bitcast(U32), PK.bitcast(U32)
        zz = ZS[0]
        pg0 = 0 if buf is bufs[0] else 256
        ml = {}
        m8_ = {}
        acc = {}
        fin = {}

        def bfly(e, rows):
            lane = jax.lax.broadcasted_iota(jnp.int32, (rows, 128), 1)
            s0 = (lane & 32) != 0
            s1 = (lane & 64) != 0

            def sel(m, x, y):
                if x is None and y is None:
                    return None
                z = jnp.zeros_like(x if y is None else y)
                return jnp.where(m, z if x is None else x, z if y is None else y)

            a = [[sel(s1, e[2 + j], e[j]), sel(s1, e[j], e[2 + j])] for j in range(2)]
            return [sel(s0, a[1][0], a[0][0]), sel(s0, a[0][0], a[1][1]),
                    sel(s0, a[1][1], a[0][1]), sel(s0, a[0][1], a[1][0])]

        def put_max(qb, m8):
            m = jnp.broadcast_to(jnp.max(m8, axis=0, keepdims=True), (8, 512))
            m = [m[:, 128 * h:128 * (h + 1)] for h in range(4)]
            for i, v in enumerate(m + bfly(m, 8)):
                if qb > 0 or i >= 4:
                    PG[pg0 + 64 * qb + 8 * i:pg0 + 64 * qb + 8 * i + 8, :] = v

        def get_max(i):
            for qb, h in [(dg.index(i), 4 + j) for j in range(4)] if i in dg else [t[:2] for t in tiles(i)]:
                if (i, h) not in ml:
                    ml[(i, h)] = PG[pl.ds(pl.multiple_of(zz * (i + 1) + pg0 + 64 * qb + 8 * h, 8), 8), :]

        def diag(qa):
            lm = [jnp.concatenate([LM[i]] * 2, axis=0) for i in range(4)]
            for qb, rev in ((qa, False), (qa + 1, True)):
                m8 = [None] * 4
                for j in range(3, -1, -1):
                    w = jnp.concatenate([Qm[qb, 16 * h:16 * h + 16, :] & lm[(j + h) % 4] for h in range(4)], axis=0)
                    rs = range(j, -1, -1) if rev else range(j + 1)
                    kq = jnp.concatenate([Kb[64 * qb + 16 * r:64 * qb + 16 * r + 16, :] for r in rs], axis=0)
                    d = jnp.dot(pltpu.bitcast(kq, BF16), pltpu.bitcast(w, BF16), preferred_element_type=F32)
                    for i, r in enumerate(rs):
                        v = d[32 * i:32 * i + 32] + CM[...] if r == j else d[32 * i:32 * i + 32]
                        SB[qb][j, 128 * qb + 32 * r:128 * qb + 32 * r + 32, :] = v
                        mx = jnp.max(v.reshape(4, 8, 128), axis=0)
                        m8[j] = mx if m8[j] is None else jnp.maximum(m8[j], mx)
                m8_[qb] = jnp.concatenate(bfly(m8, 8), axis=1)
            if qa == 0:
                put_max(0, m8_[0])

        def qk(qb):
            z16 = jnp.zeros((16, 128), U32)
            w = jnp.concatenate([jnp.concatenate([Qm[qb, 16 * h:16 * h + 16, :] if i == h else z16
                                                  for i in range(4)], axis=0) for h in range(4)], axis=1)
            s = jnp.dot(pltpu.bitcast(Kb[0:64 * qb, :], BF16), pltpu.bitcast(w, BF16), preferred_element_type=F32)
            m8 = m8_[qb]
            for c in range(qb):
                blk = s[c * 128:(c + 1) * 128, :]
                for h in range(4):
                    SB[qb][h, c * 128:(c + 1) * 128, :] = blk[:, 128 * h:128 * (h + 1)]
                m8 = jnp.maximum(m8, jnp.max(blk.reshape(16, 8, 512), axis=0))
            put_max(qb, m8)

        def pv(qb, h, c, p, l8):
            o = jnp.dot(pltpu.bitcast(VT[c, 16 * h:16 * h + 16, :], BF16), p, preferred_element_type=F32)
            if (qb, h) in acc:
                o0, l0, n = acc[(qb, h)]
                o = o + o0
                l8 = l0 + l8
            else:
                n = 0
            acc[(qb, h)] = (o, l8, n + 1)
            if n == qb:
                gt = GT[g]
                l = jnp.sum(l8, axis=0, keepdims=True)
                res = o * (gt[4 + h:5 + h, :] * _rcp(l))
                if h > 0:
                    res = pltpu.roll(res, 128 - 32 * h, 1)
                if mem:
                    num = RD[zz + qb, 32 * h:32 * h + 32, :]
                    den = RD[zz + qb, 128:136, :][h:h + 1, :] + 1e-06
                    res = num * (gt[h:h + 1, :] * _rcp(den)) + res
                fin[(qb, h)] = res

        def pv_tile(i, qb, h, c):
            m = jnp.concatenate([ml[(i, h)]] * 16, axis=0)
            p = jnp.exp2(SB[qb][h, pl.ds(pl.multiple_of(zz + c * 128, 128), 128), :] - m)
            l8 = p[120:128]
            for r in range(14, -1, -1):
                l8 = l8 + p[8 * r:8 * r + 8]
            pv(qb, h, c, p.astype(BF16), l8)

        def pv_diag(qb):
            m = [ml[(dg[qb], 4 + j)] for j in range(4)]
            l8 = [None] * 4
            w = {}
            for r in range(3, -1, -1):
                e = [None] * 4
                for j in range(r, 4):
                    mj = jnp.concatenate([m[j]] * 2, axis=0)
                    p = [jnp.exp2(SB[qb][j, pl.ds(zz + 128 * qb + 32 * r + i, 16, stride=2), :] - mj)
                         for i in range(2)]
                    for v in (p[1][8:16], p[1][0:8], p[0][8:16], p[0][0:8]):
                        l8[j] = v if l8[j] is None else l8[j] + v
                    e[j] = pltpu.pack_elementwise(p, packed_dtype=BF16)
                w[r] = bfly(e, 16)
            l8 = bfly(l8, 8)
            for h in range(4):
                pv(qb, h, qb, pltpu.bitcast(jnp.concatenate([w[r][h] for r in range(4)], axis=0), BF16), l8[h])

        def put(qb):
            ot = jnp.concatenate([fin[(qb, i)] for i in range(4)], axis=0).astype(BF16)
            if last:
                ot = pltpu.bitcast(ot.T, U32)
                OL[qb][...] = ot
                PG[pl.ds(pl.multiple_of(520 + zz, 8), 8), :] = pltpu.bitcast(ot[56:64], F32)
                return
            o2 = pl.multiple_of((seg % 2) * (L // 2) + 64 * qb, 64)
            OBu[g, pl.ds(o2, 64), :] = pltpu.bitcast(ot.T, U32)

        dg = (0, 1, 3, 6)

        def tiles(i):
            i = (2, 4, 5, 7, 8, 9).index(i)
            return [(qb, h, c) for qb in range(4) for h in range(4) for c in range(qb)][4 * i:4 * i + 4]

        def grp(i):
            get_max(i)
            if i in dg:
                pv_diag(dg.index(i))
                return
            for t in tiles(i):
                pv_tile(i, *t)

        def rd():
            r = jax.lax.dot_general(MST[g].astype(BF16), pltpu.bitcast(PQ[...], BF16), NT, preferred_element_type=F32)
            for c in range(4):
                RD[c] = r[0:136, c * 128:(c + 1) * 128]

        def upd():
            vall = pltpu.bitcast(jnp.concatenate([VT[c] for c in range(4)], axis=1), BF16)
            u = jnp.dot(vall, pltpu.bitcast(PK[...], BF16), preferred_element_type=F32)
            rr = jax.lax.broadcasted_iota(jnp.int32, (144, 128), 0)
            cc = jax.lax.broadcasted_iota(jnp.int32, (144, 128), 1) // DH
            keep = jnp.where(rr < 128, rr // DH, rr - 128) == cc
            u = jnp.where(keep, u, 0.0)
            MST[g] = MST[g + zz] + u if mem else u

        def act(tok):
            if tok[0] == "Q":
                qk(int(tok[1]))
            elif tok[0] == "D":
                diag(int(tok[1]))
            elif tok[0] == "G":
                grp(int(tok[1]))
            elif tok[0] == "g":
                get_max(int(tok[1]))
            elif tok[0] == "S":
                put(int(tok[1]))
            elif tok == "R":
                rd()
            else:
                assert tok == "U"
                upd()

        return act

    def run(sched, steps, queues):
        queues = {k: list(v) for k, v in queues.items()}
        si = 0
        for tok in sched.split():
            if tok == "|":
                si += 1
            elif tok == "z":
                pin_load()
            elif tok == "Z":
                queues["O"].pop(0)(pin=True)
            elif tok in queues:
                queues[tok].pop(0)()
            elif tok[-1] == "+":
                steps[si + 1](tok[:-1])
            else:
                steps[si](tok)
        assert all(not v for v in queues.values()), {k: len(v) for k, v in queues.items()}

    def ffn_patch(layer):
        r = RT[...]
        sub = jax.lax.broadcasted_iota(jnp.int32, (16, 128), 0)
        idx = (sub // 8) * 1024 + jax.lax.broadcasted_iota(jnp.int32, (16, 128), 1) * 8 + sub % 8
        m1 = jnp.max(r, keepdims=True)
        i1 = jnp.min(jnp.where(r == m1, idx, S - 1))
        r2 = jnp.where(idx == i1, -jnp.inf, r)
        m2 = jnp.max(r2, keepdims=True)
        i2 = jnp.min(jnp.where((r2 == m2) & (idx != i1), idx, S - 1))
        b1 = pl.multiple_of((jnp.clip(i1, 0, S - 1) // 16) * 16, 16)
        b2 = pl.multiple_of((jnp.clip(i2, 0, S - 1) // 16) * 16, 16)
        i16 = jax.lax.broadcasted_iota(jnp.int32, (16, 1), 0)
        s1 = i16 + b1 == i1
        s2 = i16 + b2 == i2

        def pick(b, sel):
            blk = jnp.concatenate([T[k, pl.ds(b, 16), :] for k in range(8)], axis=1)
            row = jnp.sum(jnp.where(sel, blk.astype(F32), 0.0), axis=0, keepdims=True)
            return jnp.broadcast_to(row, (8, D))

        x1 = jnp.concatenate([pick(b1, s1), pick(b2, s2)], axis=0)
        yb = _ln_f32(x1).astype(BF16)
        rsel = jnp.where(i16 < 8, m1, m2)

        def dot512(x, ref, r, c):
            return jnp.dot(x, ref[512 * r:512 * (r + 1), 128 * c:128 * (c + 1)], preferred_element_type=F32)

        def gate_up(c):
            hs = []
            for n in range(4 * c, 4 * c + 4):
                gt, up = [_rb(dot512(yb[:, :512], w, 0, n) + dot512(yb[:, 512:], w, 1, n)) for w in (WG, WU)]
                hs.append(_rb(gt * _rb(jax.nn.sigmoid(gt))) * up)
            return jnp.concatenate(hs, axis=1).astype(BF16)

        hm = gate_up(0)
        yv = None
        for c in range(NFC):
            nxt = gate_up(c + 1) if c + 1 < NFC else None
            dn = jnp.concatenate([dot512(hm, WD, c, n) for n in range(8)], axis=1)
            yv = dn if yv is None else yv + dn
            hm = nxt
        yv = _rb(_rb(yv) * _rb(jax.nn.sigmoid(rsel)))
        x2 = _rb(x1 + _rb(yb.astype(F32) + yv))
        xn = _rb(_ln_f32(x2))

        @pl.when(layer == 1)
        def _():
            for s in range(11):
                out_copy(0, 128, s).wait()
            out_copy(0, 640, 11).wait()

        for b, sel, lo in ((b1, s1, 0), (b2, s2, 8)):
            new = jnp.concatenate([x2[lo:lo + 8], x2[lo:lo + 8]], axis=0)
            R[pl.ds(b, 16), :] = jnp.where(sel, new, R[pl.ds(b, 16), :].astype(F32)).astype(BF16)

        @pl.when(layer == 0)
        def _():
            for b, sel, lo in ((b1, s1, 0), (b2, s2, 8)):
                new = jnp.concatenate([xn[lo:lo + 8], xn[lo:lo + 8]], axis=0)
                for k in range(8):
                    XN[k, pl.ds(b, 16), :] = jnp.where(sel, new[:, k * 128:(k + 1) * 128],
                                                       XN[k, pl.ds(b, 16), :].astype(F32)).astype(BF16)
            run("P P m P P m P P m P P m P P m P P m P P m P P m P P P P P P P P", [],
                {"P": proj_rounds(0, 0, bufs[0]), "m": ln_units(L, 128, False, 2)[:8]})

        @pl.when(layer == 1)
        def _():
            c1 = out_copy(b1, 16, 0)
            c1.start()

            @pl.when(b2 != b1)
            def _():
                c2 = out_copy(b2, 16, 1)
                c2.start()
                c2.wait()

            c1.wait()

    p0 = proj_rounds(0, 0, bufs[0])
    x_copy(0, 128, 0).wait()
    for f in ln_units(0, 128, False, 2):
        f()
    for c in range(4):
        if c == 0:
            for j in range(3):
                w_copy(0, j).wait()
        if c < 3:
            x_copy(128 * (c + 1), 128, c + 1).wait()
            run("f f f f P P f f f f P P P P f f f f", [],
                {"P": p0[6 * c:6 * c + 6], "f": ln_units(128 * (c + 1), 128, False, 2)})
        else:
            x_copy(0, 128, 4).wait()
            run("m m m m P P m m P P m m P P", [], {"P": p0[18:24], "m": ln_units(L, 128, False, 2)[:8]})

    def layer_body(layer, carry):
        def a_body(gp, carry2):
            g0 = 2 * gp
            g2 = (g0 + 2) % NG

            @pl.when(layer == 0)
            def _():
                @pl.when(gp < 3)
                def _():
                    for j in range(3):
                        w_copy(g0 + 3, j).start()

                @pl.when(gp < 2)
                def _():
                    for j in range(3):
                        w_copy(g0 + 4, j).start()

                @pl.when(gp < 2)
                def _():
                    x_copy(pl.multiple_of(768 + 128 * gp, 128), 128, 6 + gp).start()

                @pl.when(gp == 1)
                def _():
                    for n in range(8):
                        wo_copy(n).start()

                @pl.when(gp >= 2)
                def _():
                    x_copy(pl.multiple_of(gp * L, L), L, 6 + gp).start()

                for j in range(3):
                    w_copy(g0 + 1, j).wait()

                @pl.when(gp < 3)
                def _():
                    for j in range(3):
                        w_copy(g2, j).wait()
                    x_copy(0, 128, 5 + gp).wait()

                @pl.when(gp == 3)
                def _():
                    x_copy(0, L, 8).wait()

            run(SCHED_A, [attn(0, g0, bufs[0], False), attn(0, g0 + 1, bufs[1], False)],
                {"P": proj_rounds(0, g0 + 1, bufs[1]) + proj_rounds(gp // 3, g2, bufs[0]),
                 "n": ln_units(L + gp * 128, 128, False, 2)[8:],
                 "m": ln_units(L + 128 + gp * 128, 128, False, 2)[:8]})
            return carry2

        jax.lax.fori_loop(0, 4, a_body, 0)

        @pl.when(layer == 0)
        def _():
            for c in ffn_copies:
                c.start()
            for n in range(8):
                wo_copy(n).wait()
            x_copy(0, L, 9).wait()

        def b_body(it, carry2):
            seg = 1 + it // 4
            gp = it % 4
            g0 = 2 * gp
            g2 = (g0 + 2) % NG
            prow = (seg - 1) * L + gp * 128
            run(SCHED_B, [attn(seg, g0, bufs[0], True), attn(seg, g0 + 1, bufs[1], True)],
                {"P": proj_rounds(seg, g0 + 1, bufs[1]) + proj_rounds(seg + gp // 3, g2, bufs[0]),
                 "O": out_rounds(seg - 1, gp * 128, 128),
                 "n": ln_units((1024 + it * 128) % S, 128, False, 2)[8:],
                 "m": ln_units((1152 + it * 128) % S, 128, False, 2)[:8],
                 "t": ln_units(prow, 128, True, 0)})

            @pl.when(layer == 1)
            def _():
                out_copy(pl.multiple_of(prow, 128), 128, it).start()

            return carry2

        jax.lax.fori_loop(0, 11, b_body, 0)

        pieces = ((0, 128), (128, 128), (256, 64), (320, 64), (384, 64), (448, 32), (480, 32))
        run(SCHED_T, [attn(3, 6, bufs[0], True), attn(3, 7, bufs[1], True, True)],
            {"P": proj_rounds(3, 7, bufs[1]),
             "O": out_rounds(2, 384, 128) + [f for off, n in pieces for f in out_rounds(3, off, n, True)],
             "n": ln_units(384, 128, False, 2)[8:],
             "t": ln_units(2 * L + 384, 128, True, 0, 1)
             + [f for i, (off, n) in enumerate(pieces)
                for f in ln_units(3 * L + off, n, True, 4 + 2 * (i % 2), 2)]})

        @pl.when(layer == 0)
        def _():
            for c in ffn_copies:
                c.wait()

        @pl.when(layer == 1)
        def _():
            out_copy(S - 640, 640, 11).start()

        ffn_patch(layer)
        return carry

    jax.lax.fori_loop(0, 2, layer_body, 0)


@jax.jit
def pallas_interleave_layers__memory_aug_infini_attn__moe_arch_mod__prompt_kernel(
    A_x: jax.Array,
    A_wq: jax.Array,
    A_wk: jax.Array,
    A_wv: jax.Array,
    A_wo: jax.Array,
    A_beta: jax.Array,
    B_x: jax.Array,
    B_w_r: jax.Array,
    B_w_gate: jax.Array,
    B_w_up: jax.Array,
    B_w_down: jax.Array,
):
    hbm = pl.BlockSpec(memory_space=pl.ANY)
    vmem = pl.BlockSpec(memory_space=pltpu.VMEM)
    qkv_set = [
        pltpu.VMEM((L, 128), BF16),
        pltpu.VMEM((4, 64, 128), U32),
        pltpu.VMEM((L, 128), BF16),
        pltpu.VMEM((L, 128), BF16),
        pltpu.VMEM((4, 72, 128), U32),
        pltpu.VMEM((4, 128, 128), F32),
        pltpu.VMEM((4, 256, 128), F32),
        pltpu.VMEM((4, 384, 128), F32),
        pltpu.VMEM((4, 512, 128), F32),
        pltpu.VMEM((4, 136, 128), F32),
    ]
    scratch = [
        pltpu.VMEM((S + 16, D), BF16),
        pltpu.VMEM((8, S + 16, 128), BF16),
        pltpu.VMEM((8, S, 128), BF16),
        pltpu.VMEM((NG, 3, D, 128), BF16),
        pltpu.VMEM((8, D, 128), BF16),
        pltpu.VMEM((D, FF), BF16),
        pltpu.VMEM((D, FF), BF16),
        pltpu.VMEM((FF, D), BF16),
        pltpu.VMEM((NG, 2 * L, 128), BF16),
        pltpu.VMEM((NG, 144, 128), F32),
        pltpu.VMEM((NG, 8, 128), F32),
        pltpu.VMEM((8, D), F32),
        pltpu.VMEM((32, 128), F32),
        pltpu.VMEM((4, 8, 128), U32),
        pltpu.VMEM((PD + 16, 128), F32),
        pltpu.VMEM((536, 128), F32),
        pltpu.VMEM((16, 128), F32),
    ] + qkv_set + qkv_set + [pltpu.VMEM((64, 128), U32)] * 4 + [
        pltpu.VMEM((1024, 128), F32),
        pltpu.SMEM((1,), jnp.int32),
        pltpu.SemaphoreType.DMA((10,)),
        pltpu.SemaphoreType.DMA((NG, 3)),
        pltpu.SemaphoreType.DMA((11,)),
        pltpu.SemaphoreType.DMA((12,)),
    ]
    return pl.pallas_call(
        _kernel,
        out_shape=jax.ShapeDtypeStruct((1, S, D), BF16),
        in_specs=[hbm, hbm, hbm, hbm, hbm, vmem, vmem, hbm, hbm, hbm],
        out_specs=hbm,
        scratch_shapes=scratch,
        compiler_params=pltpu.CompilerParams(vmem_limit_bytes=100 * 1024 * 1024),
    )(A_x, A_wq, A_wk, A_wv, A_wo, A_beta, B_w_r, B_w_gate, B_w_up, B_w_down)
```

```python
import jax
import jax.numpy as jnp
import jax.experimental.pallas as pl
import jax.experimental.pallas.tpu as pltpu

F32 = jnp.float32
BF16 = jnp.bfloat16
U32 = jnp.uint32
I32 = jnp.int32
IMIN = -2147483648

S = 2048
D = 1024
H = 32
DH = 32
NSEG = 4
L = S // NSEG
NG = 8
FF = 3584
FCH = 512
NFC = FF // FCH
LOG2E = 1.4426950408889634
QSCALE = (DH ** -0.5) * LOG2E
NEG = -1000000000.0 * LOG2E
EPS_LN = 1.0013580322265625e-05
BIG = 3.0e38
NT = (((1,), (1,)), ((), ()))
PZ = 1024
PD = 1032

SCHED_A = ("D0 g0 n Q1 g1 n D2 n Q2 n G0 S0 P P G1 g2 m P P G2 g3 S1 m P P G3 g4 Q3 m P P G4 g5 m P P G5 g6 S2 m "
           "P P G6 g7 m P P G7 g8 m P P G8 g9 m P P G9 S3 P P D0+ P P Q1+ g0+ P P U | G0 g1 S0 P P D2 G1 g2 P P "
           "Q2 G2 g3 S1 P P G3 g4 P P G4 g5 Q3 P P G5 g6 S2 P P G6 g7 P P G7 g8 P P G8 g9 P P G9 S3 P P P P P P "
           "U ")
SCHED_B = ("O O n O O n m O O n m O O n m O O m m O O m D0 O O g0 m Q1 R O O g1 m G0 S0 P P D2 G1 g2 t t P P Q2 "
           "G2 g3 S1 t t P P G3 g4 t P P G4 g5 Q3 t P P G5 g6 S2 t P P G6 g7 t P P G7 g8 P P G8 g9 P P G9 S3 t P "
           "P D0+ t P P Q1+ g0+ P P U | R G0 g1 S0 P P D2 G1 g2 P P Q2 G2 g3 S1 P P G3 g4 P P G4 g5 Q3 P P G5 g6 "
           "S2 P P G6 g7 P P G7 g8 P P G8 g9 P P G9 S3 t P P t P P P P U ")
SCHED_T = ("O O n O O n O O n D0 Q1 g0 R O O n G0 g1 S0 D2 G1 g2 P P Q2 G2 g3 S1 P P G3 g4 P P G4 g5 Q3 P P G5 "
           "g6 S2 P P G6 g7 P P G7 g8 P P G8 g9 P P G9 S3 P P D0+ P P Q1+ g0+ P P P P | R O O G0 g1 O O S0 D2 G1 "
           "g2 O O Q2 G2 g3 O O S1 G3 g4 O O G4 g5 Q3 t t O O G5 g6 t t t O O S2 G6 g7 t O O G7 g8 t O O G8 g9 t "
           "O O G9 t O O S3 t z O O t t z O O t z Z O t z Z O t z Z O t z Z O t z Z O t z Z O t z Z O t z Z O t "
           "z O O t z Z O t z O O z Z O t z Z O t z Z O z Z O t z Z O t z Z O z Z O t z Z O t z Z O t z Z O z Z "
           "O t z Z O z Z O t z Z O t z Z O t z Z O z Z O t z Z O z Z O t z Z O z Z O t z Z O Z O t z O O Z O O "
           "O t z Z O Z O t z O O t z Z O O O t O O Z O O O t Z O Z O t t t ")


def _rb(t):
    return t.astype(BF16).astype(F32)


def _rb2(t):
    n = t.shape[0] // 2
    p = pltpu.pack_elementwise([t[:n], t[n:]], packed_dtype=BF16)
    return jnp.concatenate([pltpu.unpack_elementwise(p, index=i, packed_dtype=BF16, unpacked_dtype=F32)
                            for i in range(2)], axis=0)


def _rcp(d):
    d = jnp.minimum(d, BIG)
    r = pl.reciprocal(d, approx=True)
    return r * (2.0 - d * r)


def _rinv(var):
    v = _rb(_rb(var) + EPS_LN)
    vc = jnp.minimum(v, BIG)
    return jnp.minimum(_rcp(_rb(vc * jax.lax.rsqrt(vc))), 1e30 * pl.reciprocal(v, approx=True))


def _ln_f32(x):
    mu = jnp.sum(x, axis=1, keepdims=True) * (1.0 / D)
    xc = x - mu
    var = jnp.sum(xc * xc, axis=1, keepdims=True) * (1.0 / D)
    return (x - _rb(mu)) * _rinv(var)


def _phi(t):
    return jnp.maximum(t, 0.0) + jnp.exp(jnp.minimum(t, 0.0))


def _bind(f, *a):
    return lambda **kw: f(*a, **kw)


def _kernel(x_hbm, wq_hbm, wk_hbm, wv_hbm, wo_hbm, beta_ref, wr_ref, wg_hbm, wu_hbm, wd_hbm,
            out_hbm,
            R, T, XN, W, WO, WG, WU, WD, OB, MST, GT, WR, CM, LM, PN, PG, RT,
            K0, Q0, PQ0, PK0, VT0, SA0, SB0, SC0, SD0, RD0, K1, Q1, PQ1, PK1, VT1, SA1, SB1, SC1, SD1, RD1,
            OL0, OL1, OL2, OL3, PS, ZS, sx, sw, sm, so):
    bufs = ((K0, Q0, PQ0, PK0, VT0, (SA0, SB0, SC0, SD0), RD0), (K1, Q1, PQ1, PK1, VT1, (SA1, SB1, SC1, SD1), RD1))
    OL = (OL0, OL1, OL2, OL3)
    ZS[0] = 0
    XNu = XN.bitcast(U32)
    Wu = W.bitcast(U32)
    WOu = WO.bitcast(U32)
    OBu = OB.bitcast(U32)
    Tu = T.bitcast(U32)

    def x_copy(row0, n, s):
        return pltpu.make_async_copy(x_hbm.at[0, pl.ds(row0, n), :], R.at[pl.ds(row0, n), :], sx.at[s])

    def w_copy(g, j):
        src = (wq_hbm, wk_hbm, wv_hbm)[j]
        return pltpu.make_async_copy(src.at[:, pl.ds(pl.multiple_of(g * 128, 128), 128)], W.at[g, j], sw.at[g, j])

    def wo_copy(n):
        return pltpu.make_async_copy(wo_hbm.at[:, pl.ds(n * 128, 128)], WO.at[n], sm.at[n])

    ffn_copies = (pltpu.make_async_copy(wg_hbm, WG, sm.at[8]),
                  pltpu.make_async_copy(wu_hbm, WU, sm.at[9]),
                  pltpu.make_async_copy(wd_hbm, WD, sm.at[10]))

    def out_copy(row0, n, s):
        return pltpu.make_async_copy(R.at[pl.ds(row0, n), :], out_hbm.at[0, pl.ds(row0, n), :], so.at[s])

    x_copy(0, 128, 0).start()
    w_copy(0, 0).start()
    x_copy(128, 128, 1).start()
    w_copy(0, 1).start()
    w_copy(0, 2).start()
    x_copy(256, 128, 2).start()
    x_copy(384, 128, 3).start()
    for g in (1, 2):
        for j in range(3):
            w_copy(g, j).start()
    x_copy(512, 128, 4).start()
    x_copy(640, 128, 5).start()

    gsig = jax.nn.sigmoid(beta_ref[...].astype(F32).reshape(1, H))
    eye = (jax.lax.broadcasted_iota(jnp.int32, (H, H), 0)
           == jax.lax.broadcasted_iota(jnp.int32, (H, H), 1))
    gcol = jnp.sum(jnp.where(eye, jnp.broadcast_to(gsig, (H, H)), 0.0), axis=1, keepdims=True)
    gfull = jnp.broadcast_to(gcol, (H, 128))
    for g in range(NG):
        GT[g, 0:4, :] = gfull[4 * g:4 * g + 4, :]
        GT[g, 4:8, :] = 1.0 - gfull[4 * g:4 * g + 4, :]
    WR[...] = jnp.broadcast_to(wr_ref[...].astype(F32).reshape(1, D), (8, D))
    kk = jax.lax.broadcasted_iota(jnp.int32, (32, 128), 0)
    qq = jax.lax.broadcasted_iota(jnp.int32, (32, 128), 1) % 32
    CM[...] = jnp.where(qq < kk, NEG, 0.0).astype(F32)
    for c in range(4):
        LM[c] = jnp.where(jax.lax.broadcasted_iota(jnp.int32, (8, 128), 1) // DH == c,
                          jnp.uint32(0xFFFFFFFF), jnp.uint32(0))
        VT0[c, 64:72, :] = pltpu.bitcast(jnp.ones((16, 128), BF16), U32)
        VT1[c, 64:72, :] = pltpu.bitcast(jnp.ones((16, 128), BF16), U32)
    RT[...] = jnp.full((16, 128), IMIN, I32)
    PN[PZ:PZ + 8, :] = jnp.zeros((8, 128), F32)
    PG[528:536, :] = jnp.zeros((8, 128), F32)
    R[S:S + 16, 0:128] = jnp.zeros((16, 128), BF16)
    T[0, S:S + 16, :] = jnp.zeros((16, 128), BF16)

    def ln_units(row0, nrows, router, slab, late=0):
        zz = ZS[0]
        st = PS if late else PN

        def ld(i, k, v):
            if router:
                r2 = pl.multiple_of(row0 // 2 + 16 * i + zz * v, 16)
                return pltpu.bitcast(Tu[k, pl.ds(r2, 16), :], BF16).astype(F32)
            r1 = pl.multiple_of(row0 + 32 * i + zz * v, 32)
            return R[pl.ds(r1, 32), k * 128:(k + 1) * 128].astype(F32)

        def st_put(i, j, val):
            r = pl.multiple_of((slab + j) * 128 + 32 * i + zz, 32)
            st[pl.ds(r, 32), :] = jnp.broadcast_to(val, (32, 128))

        def done(val):
            PG[pl.ds(pl.multiple_of(520 + zz, 8), 8), :] = val[-8:]

        def st_get(i, j, v):
            return st[pl.ds(pl.multiple_of((slab + j) * 128 + 32 * i + zz * v, 32), 32), :]

        def mean(*ii):
            z = PN[pl.ds(pl.multiple_of(PZ + zz, 8), 8), :]
            accs = []
            for i in ii:
                acc = jnp.concatenate([z, z, z, z], axis=0)
                for k in range(8):
                    acc = acc + ld(i, k, 1)
                accs.append(acc)
            for i, acc in zip(ii, accs):
                done(acc)
                st_put(i, 0, jnp.sum(acc, axis=1, keepdims=True) * (1.0 / D))

        def var(*ii):
            mus = [st_get(i, 0, 2) for i in ii]
            for i, mu in zip(ii, mus):
                acc = None
                for k in range(8):
                    xc = ld(i, k, 2) - mu
                    acc = xc * xc if acc is None else acc + xc * xc
                done(acc)
                st_put(i, 1, _rinv(jnp.sum(acc, axis=1, keepdims=True) * (1.0 / D)))

        def norm(i):
            mu = _rb2(st_get(i, 0, 3))
            ri = st_get(i, 1, 3)
            acc = None
            for k in range(8):
                x = ld(i, k, 3)
                y = (x - mu) * ri
                if k == 7 and not late:
                    PN[pl.ds(pl.multiple_of(PD + 8 + zz, 8), 8), :] = y[24:32]
                    done(y)
                if not router:
                    XN[k, pl.ds(pl.multiple_of(row0 + 32 * i, 32), 32), :] = y.astype(BF16)
                    continue
                y = _rb2(y)
                wr = WR[:, k * 128:(k + 1) * 128]
                yw = y * jnp.concatenate([wr, wr, wr, wr], axis=0)
                acc = yw if acc is None else acc + yw
                R[pl.ds(pl.multiple_of(row0 + 32 * i, 32), 32), k * 128:(k + 1) * 128] = (x + y).astype(BF16)
            if router:
                r = jnp.broadcast_to(_rb(jnp.sum(acc, axis=1, keepdims=True)), (32, 128))
                b = pltpu.bitcast(r, I32)
                sg = b >> 31
                tok = jax.lax.broadcasted_iota(I32, (32, 128), 0) + (row0 + 32 * i - (S - 1))
                key = ((b & 0x7FFF0000) ^ sg) - (sg + tok)
                hi = RT[0:8, :]
                lo = RT[8:16, :]
                for j in range(4):
                    kj = key[8 * j:8 * j + 8]
                    lo = jnp.maximum(lo, jnp.minimum(hi, kj))
                    hi = jnp.maximum(hi, kj)
                RT[0:8, :] = hi
                RT[8:16, :] = lo
                if late:
                    done(pltpu.bitcast(lo, F32))

        n = nrows // 32
        if late > 1 and n > 1:
            return ([_bind(f, i, i + 1) for f in (mean, var) for i in range(0, n, 2)]
                    + [_bind(norm, i) for i in range(n)])
        return [_bind(f, i) for f in (mean, var, norm) for i in range(n)]

    def proj_rounds(seg, g, buf):
        Kb, Qm, PQ, PK, VT, SB, RD = buf
        zz = ZS[0]
        part = {}

        def rnd(c, j, half):
            r2 = pl.multiple_of(seg * (L // 2) + c * 64 + zz * j, 64)
            xn = jnp.concatenate([pltpu.bitcast(XNu[k, pl.ds(r2, 64), :], BF16)
                                  for k in range(4 * half, 4 * half + 4)], axis=1)
            w = pltpu.bitcast(Wu[g, j, pl.ds(pl.multiple_of(256 * half + zz * c, 256), 256), :], BF16)
            t = jnp.dot(xn, w, preferred_element_type=F32)
            if half == 0:
                part[0] = t
                return
            t = t + part[0]
            PN[PD:PD + 8, :] = t[120:128]
            PG[512:520, :] = t[120:128]
            if j == 0:
                qt = pltpu.bitcast((t * QSCALE).astype(BF16).T, U32)
                for h in range(4):
                    qh = qt[16 * h:16 * h + 16]
                    Qm[c, 16 * h:16 * h + 16, :] = pltpu.roll(qh, 32 * h, 1) if h else qh
                PQ[c * 128:(c + 1) * 128, :] = _phi(t).astype(BF16)
            elif j == 1:
                Kb[c * 128:(c + 1) * 128, :] = t.astype(BF16)
                PK[c * 128:(c + 1) * 128, :] = _phi(t).astype(BF16)
            else:
                VT[c, 0:64, :] = pltpu.bitcast(t.astype(BF16).T, U32)

        return [_bind(rnd, c, j, half) for c in range(4) for j in range(3) for half in range(2)]

    pins = [None]

    def pin_load():
        pins.append(pltpu.bitcast(PG[pl.ds(pl.multiple_of(528 + ZS[0], 8), 8), :], U32)
                    | pltpu.bitcast(R[pl.ds(pl.multiple_of(S + ZS[0], 16), 16), 0:128], U32)
                    | Tu[0, pl.ds(pl.multiple_of(S // 2 + ZS[0], 8), 8), :])

    def out_rounds(seg, off, nrows, last=False):
        zz = ZS[0]
        part = {}
        n2 = nrows // 2

        def rnd(n, half, pin=False):
            o2 = pl.multiple_of(((seg % 2) * L + off) // 2 + zz * (n + 1), 16)
            o = [OBu[k, pl.ds(o2, n2), :] for k in range(4 * half, 4 * half + 4 - (last and half))]
            if last and half:
                o.append(OL[off // 128][pl.ds(pl.multiple_of((off % 128) // 2 + zz * (n + 1), 16), n2), :])
            if pin:
                pins[0:2] = pins[1:2]
            if last and pins[0] is not None:
                o = [jnp.concatenate([v[0:8] | pins[0], v[8:]], axis=0) for v in o]
            o = jnp.concatenate([pltpu.bitcast(v, BF16) for v in o], axis=1)
            w = pltpu.bitcast(WOu[n, pl.ds(pl.multiple_of(256 * half + zz * (seg * L + off), 256), 256), :], BF16)
            t = jnp.dot(o, w, preferred_element_type=F32)
            if half == 0:
                part[0] = t
                return
            x = R[pl.ds(pl.multiple_of(seg * L + off, 32), nrows), n * 128:(n + 1) * 128].astype(F32)
            t = t + part[0]
            PN[PD:PD + 8, :] = t[nrows - 8:nrows]
            PG[512:520, :] = t[nrows - 8:nrows]
            T[n, pl.ds(pl.multiple_of(seg * L + off, 32), nrows), :] = (x + _rb2(t)).astype(BF16)

        return [_bind(rnd, n, half) for n in range(8) for half in range(2)]

    def attn(seg, g, buf, mem, last=False):
        Kb, Qm, PQ, PK, VT, SB, RD = buf
        Kb, PQ, PK = Kb.bitcast(U32), PQ.bitcast(U32), PK.bitcast(U32)
        zz = ZS[0]
        pg0 = 0 if buf is bufs[0] else 256
        ml = {}
        m8_ = {}
        acc = {}
        fin = {}

        def bfly(e, rows):
            lane = jax.lax.broadcasted_iota(jnp.int32, (rows, 128), 1)
            s0 = (lane & 32) != 0
            s1 = (lane & 64) != 0

            def sel(m, x, y):
                if x is None and y is None:
                    return None
                z = jnp.zeros_like(x if y is None else y)
                return jnp.where(m, z if x is None else x, z if y is None else y)

            a = [[sel(s1, e[2 + j], e[j]), sel(s1, e[j], e[2 + j])] for j in range(2)]
            return [sel(s0, a[1][0], a[0][0]), sel(s0, a[0][0], a[1][1]),
                    sel(s0, a[1][1], a[0][1]), sel(s0, a[0][1], a[1][0])]

        def put_max(qb, m8):
            m = jnp.broadcast_to(jnp.max(m8, axis=0, keepdims=True), (8, 512))
            m = [m[:, 128 * h:128 * (h + 1)] for h in range(4)]
            for i, v in enumerate(m + bfly(m, 8)):
                if qb > 0 or i >= 4:
                    PG[pg0 + 64 * qb + 8 * i:pg0 + 64 * qb + 8 * i + 8, :] = v

        def get_max(i):
            for qb, h in [(dg.index(i), 4 + j) for j in range(4)] if i in dg else [t[:2] for t in tiles(i)]:
                if (i, h) not in ml:
                    ml[(i, h)] = PG[pl.ds(pl.multiple_of(zz * (i + 1) + pg0 + 64 * qb + 8 * h, 8), 8), :]

        def diag(qa):
            lm = [jnp.concatenate([LM[i]] * 2, axis=0) for i in range(4)]
            for qb, rev in ((qa, False), (qa + 1, True)):
                m8 = [None] * 4
                for j in range(3, -1, -1):
                    w = jnp.concatenate([Qm[qb, 16 * h:16 * h + 16, :] & lm[(j + h) % 4] for h in range(4)], axis=0)
                    rs = range(j, -1, -1) if rev else range(j + 1)
                    kq = jnp.concatenate([Kb[64 * qb + 16 * r:64 * qb + 16 * r + 16, :] for r in rs], axis=0)
                    d = jnp.dot(pltpu.bitcast(kq, BF16), pltpu.bitcast(w, BF16), preferred_element_type=F32)
                    for i, r in enumerate(rs):
                        v = d[32 * i:32 * i + 32] + CM[...] if r == j else d[32 * i:32 * i + 32]
                        SB[qb][j, 128 * qb + 32 * r:128 * qb + 32 * r + 32, :] = v
                        mx = jnp.max(v.reshape(4, 8, 128), axis=0)
                        m8[j] = mx if m8[j] is None else jnp.maximum(m8[j], mx)
                m8_[qb] = jnp.concatenate(bfly(m8, 8), axis=1)
            if qa == 0:
                put_max(0, m8_[0])

        def qk(qb):
            z16 = jnp.zeros((16, 128), U32)
            w = jnp.concatenate([jnp.concatenate([Qm[qb, 16 * h:16 * h + 16, :] if i == h else z16
                                                  for i in range(4)], axis=0) for h in range(4)], axis=1)
            s = jnp.dot(pltpu.bitcast(Kb[0:64 * qb, :], BF16), pltpu.bitcast(w, BF16), preferred_element_type=F32)
            m8 = m8_[qb]
            for c in range(qb):
                blk = s[c * 128:(c + 1) * 128, :]
                for h in range(4):
                    SB[qb][h, c * 128:(c + 1) * 128, :] = blk[:, 128 * h:128 * (h + 1)]
                m8 = jnp.maximum(m8, jnp.max(blk.reshape(16, 8, 512), axis=0))
            put_max(qb, m8)

        def pv(qb, h, c, p, l8):
            o = jnp.dot(pltpu.bitcast(VT[c, 16 * h:16 * h + 16, :], BF16), p, preferred_element_type=F32)
            if (qb, h) in acc:
                o0, l0, n = acc[(qb, h)]
                o = o + o0
                l8 = l0 + l8
            else:
                n = 0
            acc[(qb, h)] = (o, l8, n + 1)
            if n == qb:
                gt = GT[g]
                l = jnp.sum(l8, axis=0, keepdims=True)
                res = o * (gt[4 + h:5 + h, :] * _rcp(l))
                if h > 0:
                    res = pltpu.roll(res, 128 - 32 * h, 1)
                if mem:
                    num = RD[zz + qb, 32 * h:32 * h + 32, :]
                    den = RD[zz + qb, 128:136, :][h:h + 1, :] + 1e-06
                    res = num * (gt[h:h + 1, :] * _rcp(den)) + res
                fin[(qb, h)] = res

        def pv_tile(i, qb, h, c):
            m = jnp.concatenate([ml[(i, h)]] * 16, axis=0)
            p = jnp.exp2(SB[qb][h, pl.ds(pl.multiple_of(zz + c * 128, 128), 128), :] - m)
            l8 = p[120:128]
            for r in range(14, -1, -1):
                l8 = l8 + p[8 * r:8 * r + 8]
            pv(qb, h, c, p.astype(BF16), l8)

        def pv_diag(qb):
            m = [ml[(dg[qb], 4 + j)] for j in range(4)]
            l8 = [None] * 4
            w = {}
            for r in range(3, -1, -1):
                e = [None] * 4
                for j in range(r, 4):
                    mj = jnp.concatenate([m[j]] * 2, axis=0)
                    p = [jnp.exp2(SB[qb][j, pl.ds(zz + 128 * qb + 32 * r + i, 16, stride=2), :] - mj)
                         for i in range(2)]
                    for v in (p[1][8:16], p[1][0:8], p[0][8:16], p[0][0:8]):
                        l8[j] = v if l8[j] is None else l8[j] + v
                    e[j] = pltpu.pack_elementwise(p, packed_dtype=BF16)
                w[r] = bfly(e, 16)
            l8 = bfly(l8, 8)
            for h in range(4):
                pv(qb, h, qb, pltpu.bitcast(jnp.concatenate([w[r][h] for r in range(4)], axis=0), BF16), l8[h])

        def put(qb):
            ot = jnp.concatenate([fin[(qb, i)] for i in range(4)], axis=0).astype(BF16)
            if last:
                ot = pltpu.bitcast(ot.T, U32)
                OL[qb][...] = ot
                PG[pl.ds(pl.multiple_of(520 + zz, 8), 8), :] = pltpu.bitcast(ot[56:64], F32)
                return
            o2 = pl.multiple_of((seg % 2) * (L // 2) + 64 * qb, 64)
            OBu[g, pl.ds(o2, 64), :] = pltpu.bitcast(ot.T, U32)

        dg = (0, 1, 3, 6)

        def tiles(i):
            i = (2, 4, 5, 7, 8, 9).index(i)
            return [(qb, h, c) for qb in range(4) for h in range(4) for c in range(qb)][4 * i:4 * i + 4]

        def grp(i):
            get_max(i)
            if i in dg:
                pv_diag(dg.index(i))
                return
            for t in tiles(i):
                pv_tile(i, *t)

        def rd():
            r = jax.lax.dot_general(MST[g].astype(BF16), pltpu.bitcast(PQ[...], BF16), NT, preferred_element_type=F32)
            for c in range(4):
                RD[c] = r[0:136, c * 128:(c + 1) * 128]

        def upd():
            vall = pltpu.bitcast(jnp.concatenate([VT[c] for c in range(4)], axis=1), BF16)
            u = jnp.dot(vall, pltpu.bitcast(PK[...], BF16), preferred_element_type=F32)
            rr = jax.lax.broadcasted_iota(jnp.int32, (144, 128), 0)
            cc = jax.lax.broadcasted_iota(jnp.int32, (144, 128), 1) // DH
            keep = jnp.where(rr < 128, rr // DH, rr - 128) == cc
            u = jnp.where(keep, u, 0.0)
            MST[g] = MST[g + zz] + u if mem else u

        def act(tok):
            if tok[0] == "Q":
                qk(int(tok[1]))
            elif tok[0] == "D":
                diag(int(tok[1]))
            elif tok[0] == "G":
                grp(int(tok[1]))
            elif tok[0] == "g":
                get_max(int(tok[1]))
            elif tok[0] == "S":
                put(int(tok[1]))
            elif tok == "R":
                rd()
            else:
                assert tok == "U"
                upd()

        return act

    def run(sched, steps, queues):
        queues = {k: list(v) for k, v in queues.items()}
        si = 0
        for tok in sched.split():
            if tok == "|":
                si += 1
            elif tok == "z":
                pin_load()
            elif tok == "Z":
                queues["O"].pop(0)(pin=True)
            elif tok in queues:
                queues[tok].pop(0)()
            elif tok[-1] == "+":
                steps[si + 1](tok[:-1])
            else:
                steps[si](tok)
        assert all(not v for v in queues.values()), {k: len(v) for k, v in queues.items()}

    def ffn_patch(layer):
        hi = RT[0:8, :]
        lo = RT[8:16, :]
        RT[...] = jnp.full((16, 128), IMIN, I32)
        for sh in (4, 2, 1):
            h2 = pltpu.roll(hi, sh, 0)
            lo = jnp.maximum(jnp.minimum(hi, h2), jnp.maximum(lo, pltpu.roll(lo, sh, 0)))
            hi = jnp.maximum(hi, h2)
        i1 = jnp.clip(S - 1 - (hi[0, 0] & (S - 1)), 0, S - 1)
        i2 = jnp.clip(S - 1 - (lo[0, 0] & (S - 1)), 0, S - 1)
        b1 = pl.multiple_of((i1 // 16) * 16, 16)
        b2 = pl.multiple_of((i2 // 16) * 16, 16)
        i16 = jax.lax.broadcasted_iota(jnp.int32, (16, 1), 0)
        s1 = i16 + b1 == i1
        s2 = i16 + b2 == i2

        def pick(i):
            u = jnp.concatenate([jnp.broadcast_to(Tu[k, pl.ds(i // 2, 1), :], (8, 128)) for k in range(8)], axis=1)
            sh = (16 - 16 * (i % 2)).astype(U32)
            return pltpu.bitcast((u << sh) & jnp.uint32(0xFFFF0000), F32)

        x1 = jnp.concatenate([pick(i1), pick(i2)], axis=0)
        yb = _ln_f32(x1).astype(BF16)
        kv = jnp.concatenate([hi, lo], axis=0) & -65536
        rsel = pltpu.bitcast(jnp.where(kv < 0, (-kv) | IMIN, kv), F32)[:, 0:1]

        def dot512(x, ref, r, c):
            return jnp.dot(x, ref[512 * r:512 * (r + 1), 128 * c:128 * (c + 1)], preferred_element_type=F32)

        def gate_up(c):
            hs = []
            for n in range(4 * c, 4 * c + 4):
                gt, up = [_rb(dot512(yb[:, :512], w, 0, n) + dot512(yb[:, 512:], w, 1, n)) for w in (WG, WU)]
                hs.append(_rb(gt * _rb(jax.nn.sigmoid(gt))) * up)
            return jnp.concatenate(hs, axis=1).astype(BF16)

        hm = gate_up(0)
        yv = None
        for c in range(NFC):
            nxt = gate_up(c + 1) if c + 1 < NFC else None
            dn = jnp.concatenate([dot512(hm, WD, c, n) for n in range(8)], axis=1)
            yv = dn if yv is None else yv + dn
            hm = nxt
        yv = _rb(_rb(yv) * _rb(jax.nn.sigmoid(rsel)))
        x2 = _rb(x1 + _rb(yb.astype(F32) + yv))
        xn = _rb(_ln_f32(x2))

        @pl.when(layer == 1)
        def _():
            for s in range(11):
                out_copy(0, 128, s).wait()
            out_copy(0, 640, 11).wait()

        for b, sel, lo in ((b1, s1, 0), (b2, s2, 8)):
            new = jnp.concatenate([x2[lo:lo + 8], x2[lo:lo + 8]], axis=0)
            R[pl.ds(b, 16), :] = jnp.where(sel, new, R[pl.ds(b, 16), :].astype(F32)).astype(BF16)

        @pl.when(layer == 0)
        def _():
            for b, sel, lo in ((b1, s1, 0), (b2, s2, 8)):
                new = jnp.concatenate([xn[lo:lo + 8], xn[lo:lo + 8]], axis=0)
                for k in range(8):
                    XN[k, pl.ds(b, 16), :] = jnp.where(sel, new[:, k * 128:(k + 1) * 128],
                                                       XN[k, pl.ds(b, 16), :].astype(F32)).astype(BF16)
            run("P P m P P m P P m P P m P P m P P m P P m P P m P P P P P P P P", [],
                {"P": proj_rounds(0, 0, bufs[0]), "m": ln_units(L, 128, False, 2)[:8]})

        @pl.when(layer == 1)
        def _():
            c1 = out_copy(b1, 16, 0)
            c1.start()

            @pl.when(b2 != b1)
            def _():
                c2 = out_copy(b2, 16, 1)
                c2.start()
                c2.wait()

            c1.wait()

    p0 = proj_rounds(0, 0, bufs[0])
    x_copy(0, 128, 0).wait()
    for f in ln_units(0, 128, False, 2):
        f()
    for c in range(4):
        if c == 0:
            for j in range(3):
                w_copy(0, j).wait()
        if c < 3:
            x_copy(128 * (c + 1), 128, c + 1).wait()
            run("f f f f P P f f f f P P P P f f f f", [],
                {"P": p0[6 * c:6 * c + 6], "f": ln_units(128 * (c + 1), 128, False, 2)})
        else:
            x_copy(0, 128, 4).wait()
            run("m m m m P P m m P P m m P P", [], {"P": p0[18:24], "m": ln_units(L, 128, False, 2)[:8]})

    def layer_body(layer, carry):
        def a_body(gp, carry2):
            g0 = 2 * gp
            g2 = (g0 + 2) % NG

            @pl.when(layer == 0)
            def _():
                @pl.when(gp < 3)
                def _():
                    for j in range(3):
                        w_copy(g0 + 3, j).start()

                @pl.when(gp < 2)
                def _():
                    for j in range(3):
                        w_copy(g0 + 4, j).start()

                @pl.when(gp < 2)
                def _():
                    x_copy(pl.multiple_of(768 + 128 * gp, 128), 128, 6 + gp).start()

                @pl.when(gp == 1)
                def _():
                    for n in range(8):
                        wo_copy(n).start()

                @pl.when(gp >= 2)
                def _():
                    x_copy(pl.multiple_of(gp * L, L), L, 6 + gp).start()

                for j in range(3):
                    w_copy(g0 + 1, j).wait()

                @pl.when(gp < 3)
                def _():
                    for j in range(3):
                        w_copy(g2, j).wait()
                    x_copy(0, 128, 5 + gp).wait()

                @pl.when(gp == 3)
                def _():
                    x_copy(0, L, 8).wait()

            run(SCHED_A, [attn(0, g0, bufs[0], False), attn(0, g0 + 1, bufs[1], False)],
                {"P": proj_rounds(0, g0 + 1, bufs[1]) + proj_rounds(gp // 3, g2, bufs[0]),
                 "n": ln_units(L + gp * 128, 128, False, 2)[8:],
                 "m": ln_units(L + 128 + gp * 128, 128, False, 2)[:8]})
            return carry2

        jax.lax.fori_loop(0, 4, a_body, 0)

        @pl.when(layer == 0)
        def _():
            for c in ffn_copies:
                c.start()
            for n in range(8):
                wo_copy(n).wait()
            x_copy(0, L, 9).wait()

        def b_body(it, carry2):
            seg = 1 + it // 4
            gp = it % 4
            g0 = 2 * gp
            g2 = (g0 + 2) % NG
            prow = (seg - 1) * L + gp * 128
            run(SCHED_B, [attn(seg, g0, bufs[0], True), attn(seg, g0 + 1, bufs[1], True)],
                {"P": proj_rounds(seg, g0 + 1, bufs[1]) + proj_rounds(seg + gp // 3, g2, bufs[0]),
                 "O": out_rounds(seg - 1, gp * 128, 128),
                 "n": ln_units((1024 + it * 128) % S, 128, False, 2)[8:],
                 "m": ln_units((1152 + it * 128) % S, 128, False, 2)[:8],
                 "t": ln_units(prow, 128, True, 0)})

            @pl.when(layer == 1)
            def _():
                out_copy(pl.multiple_of(prow, 128), 128, it).start()

            return carry2

        jax.lax.fori_loop(0, 11, b_body, 0)

        pieces = ((0, 128), (128, 128), (256, 64), (320, 64), (384, 64), (448, 32), (480, 32))
        run(SCHED_T, [attn(3, 6, bufs[0], True), attn(3, 7, bufs[1], True, True)],
            {"P": proj_rounds(3, 7, bufs[1]),
             "O": out_rounds(2, 384, 128) + [f for off, n in pieces for f in out_rounds(3, off, n, True)],
             "n": ln_units(384, 128, False, 2)[8:],
             "t": ln_units(2 * L + 384, 128, True, 0, 1)
             + [f for i, (off, n) in enumerate(pieces)
                for f in ln_units(3 * L + off, n, True, 4 + 2 * (i % 2), 2)]})

        @pl.when(layer == 0)
        def _():
            for c in ffn_copies:
                c.wait()

        @pl.when(layer == 1)
        def _():
            out_copy(S - 640, 640, 11).start()

        ffn_patch(layer)
        return carry

    jax.lax.fori_loop(0, 2, layer_body, 0)


@jax.jit
def pallas_interleave_layers__memory_aug_infini_attn__moe_arch_mod__prompt_kernel(
    A_x: jax.Array,
    A_wq: jax.Array,
    A_wk: jax.Array,
    A_wv: jax.Array,
    A_wo: jax.Array,
    A_beta: jax.Array,
    B_x: jax.Array,
    B_w_r: jax.Array,
    B_w_gate: jax.Array,
    B_w_up: jax.Array,
    B_w_down: jax.Array,
):
    hbm = pl.BlockSpec(memory_space=pl.ANY)
    vmem = pl.BlockSpec(memory_space=pltpu.VMEM)
    qkv_set = [
        pltpu.VMEM((L, 128), BF16),
        pltpu.VMEM((4, 64, 128), U32),
        pltpu.VMEM((L, 128), BF16),
        pltpu.VMEM((L, 128), BF16),
        pltpu.VMEM((4, 72, 128), U32),
        pltpu.VMEM((4, 128, 128), F32),
        pltpu.VMEM((4, 256, 128), F32),
        pltpu.VMEM((4, 384, 128), F32),
        pltpu.VMEM((4, 512, 128), F32),
        pltpu.VMEM((4, 136, 128), F32),
    ]
    scratch = [
        pltpu.VMEM((S + 16, D), BF16),
        pltpu.VMEM((8, S + 16, 128), BF16),
        pltpu.VMEM((8, S, 128), BF16),
        pltpu.VMEM((NG, 3, D, 128), BF16),
        pltpu.VMEM((8, D, 128), BF16),
        pltpu.VMEM((D, FF), BF16),
        pltpu.VMEM((D, FF), BF16),
        pltpu.VMEM((FF, D), BF16),
        pltpu.VMEM((NG, 2 * L, 128), BF16),
        pltpu.VMEM((NG, 144, 128), F32),
        pltpu.VMEM((NG, 8, 128), F32),
        pltpu.VMEM((8, D), F32),
        pltpu.VMEM((32, 128), F32),
        pltpu.VMEM((4, 8, 128), U32),
        pltpu.VMEM((PD + 16, 128), F32),
        pltpu.VMEM((536, 128), F32),
        pltpu.VMEM((16, 128), I32),
    ] + qkv_set + qkv_set + [pltpu.VMEM((64, 128), U32)] * 4 + [
        pltpu.VMEM((1024, 128), F32),
        pltpu.SMEM((1,), jnp.int32),
        pltpu.SemaphoreType.DMA((10,)),
        pltpu.SemaphoreType.DMA((NG, 3)),
        pltpu.SemaphoreType.DMA((11,)),
        pltpu.SemaphoreType.DMA((12,)),
    ]
    return pl.pallas_call(
        _kernel,
        out_shape=jax.ShapeDtypeStruct((1, S, D), BF16),
        in_specs=[hbm, hbm, hbm, hbm, hbm, vmem, vmem, hbm, hbm, hbm],
        out_specs=hbm,
        scratch_shapes=scratch,
        compiler_params=pltpu.CompilerParams(vmem_limit_bytes=100 * 1024 * 1024),
    )(A_x, A_wq, A_wk, A_wv, A_wo, A_beta, B_w_r, B_w_gate, B_w_up, B_w_down)
```

```python
import jax
import jax.numpy as jnp
import jax.experimental.pallas as pl
import jax.experimental.pallas.tpu as pltpu

F32 = jnp.float32
BF16 = jnp.bfloat16
U32 = jnp.uint32
I32 = jnp.int32
IMIN = -2147483648

S = 2048
D = 1024
H = 32
DH = 32
NSEG = 4
L = S // NSEG
NG = 8
FF = 3584
FCH = 512
NFC = FF // FCH
LOG2E = 1.4426950408889634
QSCALE = (DH ** -0.5) * LOG2E
NEG = -1000000000.0 * LOG2E
EPS_LN = 1.0013580322265625e-05
BIG = 3.0e38
NT = (((1,), (1,)), ((), ()))
PZ = 1024
PD = 1032

SCHED_A = ("D0 g0 n Q1 g1 n D2 n Q2 n G0 S0 P P G1 g2 m P P G2 g3 S1 m P P G3 g4 Q3 m P P G4 g5 m P P G5 g6 S2 m "
           "P P G6 g7 m P P G7 g8 m P P G8 g9 m P P G9 S3 P P D0+ P P Q1+ g0+ P P U | G0 g1 S0 P P D2 G1 g2 P P "
           "Q2 G2 g3 S1 P P G3 g4 P P G4 g5 Q3 P P G5 g6 S2 P P G6 g7 P P G7 g8 P P G8 g9 P P G9 S3 P P P P P P "
           "U ")
SCHED_B = ("O O n O O n m O O n m O O n m O O m m O O m D0 O O g0 m Q1 R O O g1 m G0 S0 P P D2 G1 g2 t t P P Q2 "
           "G2 g3 S1 t t P P G3 g4 t P P G4 g5 Q3 t P P G5 g6 S2 t P P G6 g7 t P P G7 g8 P P G8 g9 P P G9 S3 t P "
           "P D0+ t P P Q1+ g0+ P P U | R G0 g1 S0 P P D2 G1 g2 P P Q2 G2 g3 S1 P P G3 g4 P P G4 g5 Q3 P P G5 g6 "
           "S2 P P G6 g7 P P G7 g8 P P G8 g9 P P G9 S3 t P P t P P P P U ")
SCHED_T = ("O O n O O n O O n D0 Q1 g0 R O O n G0 g1 S0 D2 G1 g2 P P Q2 G2 g3 S1 P P G3 g4 P P G4 g5 Q3 P P G5 "
           "g6 S2 P P G6 g7 P P G7 g8 P P G8 g9 P P G9 S3 P P D0+ P P Q1+ g0+ P P P P | R O O G0 g1 O O S0 D2 G1 "
           "g2 O O Q2 G2 g3 O O S1 G3 g4 O O G4 g5 Q3 t t O O G5 g6 t t t O O S2 G6 g7 t O O G7 g8 t O O G8 g9 t "
           "O O G9 t O O S3 t z O O t t z O O t z Z O t z Z O t z Z O t z Z O t z Z O t z Z O t z Z O t z Z O t "
           "z O O t z Z O t z O O z Z O t z Z O t z Z O z Z O t z Z O t z Z O z Z O t z Z O t z Z O t z Z O z Z "
           "O t z Z O z Z O t z Z O t z Z O t z Z O z Z O t z Z O z Z O t z Z O z Z O t z Z O Z O t z O O Z O O "
           "O t z Z O Z O t z O O t z Z O O O t O O Z O O O t Z O Z O t t t ")


def _rb(t):
    return t.astype(BF16).astype(F32)


def _rb2(t):
    n = t.shape[0] // 2
    p = pltpu.pack_elementwise([t[:n], t[n:]], packed_dtype=BF16)
    return jnp.concatenate([pltpu.unpack_elementwise(p, index=i, packed_dtype=BF16, unpacked_dtype=F32)
                            for i in range(2)], axis=0)


def _rcp(d):
    d = jnp.minimum(d, BIG)
    r = pl.reciprocal(d, approx=True)
    return r * (2.0 - d * r)


def _rinv(var):
    v = _rb(_rb(var) + EPS_LN)
    vc = jnp.minimum(v, BIG)
    return jnp.minimum(_rcp(_rb(vc * jax.lax.rsqrt(vc))), 1e30 * pl.reciprocal(v, approx=True))


def _ln_f32(x):
    mu = jnp.sum(x, axis=1, keepdims=True) * (1.0 / D)
    xc = x - mu
    var = jnp.sum(xc * xc, axis=1, keepdims=True) * (1.0 / D)
    return (x - _rb(mu)) * _rinv(var)


def _phi(t):
    return jnp.maximum(t, 0.0) + jnp.exp(jnp.minimum(t, 0.0))


def _bind(f, *a):
    return lambda **kw: f(*a, **kw)


def _kernel(x_hbm, wq_hbm, wk_hbm, wv_hbm, wo_hbm, beta_ref, wr_ref, wg_hbm, wu_hbm, wd_hbm,
            out_hbm,
            R, T, XN, W, WO, WG, WU, WD, OB, MST, GT, WR, CM, LM, PN, PG, RT,
            K0, Q0, PQ0, PK0, VT0, SA0, SB0, SC0, SD0, RD0, K1, Q1, PQ1, PK1, VT1, SA1, SB1, SC1, SD1, RD1,
            OL0, OL1, OL2, OL3, PS, ZS, sx, sw, sm, so):
    bufs = ((K0, Q0, PQ0, PK0, VT0, (SA0, SB0, SC0, SD0), RD0), (K1, Q1, PQ1, PK1, VT1, (SA1, SB1, SC1, SD1), RD1))
    OL = (OL0, OL1, OL2, OL3)
    ZS[0] = 0
    XNu = XN.bitcast(U32)
    Wu = W.bitcast(U32)
    WOu = WO.bitcast(U32)
    OBu = OB.bitcast(U32)
    Tu = T.bitcast(U32)

    def x_copy(row0, n, s):
        return pltpu.make_async_copy(x_hbm.at[0, pl.ds(row0, n), :], R.at[pl.ds(row0, n), :], sx.at[s])

    def w_copy(g, j):
        src = (wq_hbm, wk_hbm, wv_hbm)[j]
        return pltpu.make_async_copy(src.at[:, pl.ds(pl.multiple_of(g * 128, 128), 128)], W.at[g, j], sw.at[g, j])

    def wo_copy(n):
        return pltpu.make_async_copy(wo_hbm.at[:, pl.ds(n * 128, 128)], WO.at[n], sm.at[n])

    ffn_copies = (pltpu.make_async_copy(wg_hbm, WG, sm.at[8]),
                  pltpu.make_async_copy(wu_hbm, WU, sm.at[9]),
                  pltpu.make_async_copy(wd_hbm, WD, sm.at[10]))

    def out_copy(row0, n, s):
        return pltpu.make_async_copy(R.at[pl.ds(row0, n), :], out_hbm.at[0, pl.ds(row0, n), :], so.at[s])

    x_copy(0, 128, 0).start()
    w_copy(0, 0).start()
    x_copy(128, 128, 1).start()
    w_copy(0, 1).start()
    w_copy(0, 2).start()
    x_copy(256, 128, 2).start()
    x_copy(384, 128, 3).start()
    for g in (1, 2):
        for j in range(3):
            w_copy(g, j).start()
    x_copy(512, 128, 4).start()
    x_copy(640, 128, 5).start()

    gsig = jax.nn.sigmoid(beta_ref[...].astype(F32).reshape(1, H))
    eye = (jax.lax.broadcasted_iota(jnp.int32, (H, H), 0)
           == jax.lax.broadcasted_iota(jnp.int32, (H, H), 1))
    gcol = jnp.sum(jnp.where(eye, jnp.broadcast_to(gsig, (H, H)), 0.0), axis=1, keepdims=True)
    gfull = jnp.broadcast_to(gcol, (H, 128))
    for g in range(NG):
        GT[g, 0:4, :] = gfull[4 * g:4 * g + 4, :]
        GT[g, 4:8, :] = 1.0 - gfull[4 * g:4 * g + 4, :]
    WR[...] = jnp.broadcast_to(wr_ref[...].astype(F32).reshape(1, D), (8, D))
    kk = jax.lax.broadcasted_iota(jnp.int32, (32, 128), 0)
    qq = jax.lax.broadcasted_iota(jnp.int32, (32, 128), 1) % 32
    CM[...] = jnp.where(qq < kk, NEG, 0.0).astype(F32)
    for c in range(4):
        LM[c] = jnp.where(jax.lax.broadcasted_iota(jnp.int32, (8, 128), 1) // DH == c,
                          jnp.uint32(0xFFFFFFFF), jnp.uint32(0))
        VT0[c, 64:72, :] = pltpu.bitcast(jnp.ones((16, 128), BF16), U32)
        VT1[c, 64:72, :] = pltpu.bitcast(jnp.ones((16, 128), BF16), U32)
    RT[...] = jnp.full((16, 128), IMIN, I32)
    PN[PZ:PZ + 8, :] = jnp.zeros((8, 128), F32)
    PG[528:536, :] = jnp.zeros((8, 128), F32)
    R[S:S + 16, 0:128] = jnp.zeros((16, 128), BF16)
    T[0, S:S + 16, :] = jnp.zeros((16, 128), BF16)

    def ln_units(row0, nrows, router, slab, late=0):
        zz = ZS[0]
        st = PS if late else PN

        def ld(i, k, v):
            if router:
                r2 = pl.multiple_of(row0 // 2 + 16 * i + zz * v, 16)
                return pltpu.bitcast(Tu[k, pl.ds(r2, 16), :], BF16).astype(F32)
            r1 = pl.multiple_of(row0 + 32 * i + zz * v, 32)
            return R[pl.ds(r1, 32), k * 128:(k + 1) * 128].astype(F32)

        def st_put(i, j, val):
            r = pl.multiple_of((slab + j) * 128 + 32 * i + zz, 32)
            st[pl.ds(r, 32), :] = jnp.broadcast_to(val, (32, 128))

        def done(val):
            PG[pl.ds(pl.multiple_of(520 + zz, 8), 8), :] = val[-8:]

        def st_get(i, j, v):
            return st[pl.ds(pl.multiple_of((slab + j) * 128 + 32 * i + zz * v, 32), 32), :]

        def mean(*ii):
            z = PN[pl.ds(pl.multiple_of(PZ + zz, 8), 8), :]
            accs = []
            for i in ii:
                acc = jnp.concatenate([z, z, z, z], axis=0)
                for k in range(8):
                    acc = acc + ld(i, k, 1)
                accs.append(acc)
            for i, acc in zip(ii, accs):
                done(acc)
                st_put(i, 0, jnp.sum(acc, axis=1, keepdims=True) * (1.0 / D))

        def var(*ii):
            mus = [st_get(i, 0, 2) for i in ii]
            for i, mu in zip(ii, mus):
                acc = None
                for k in range(8):
                    xc = ld(i, k, 2) - mu
                    acc = xc * xc if acc is None else acc + xc * xc
                done(acc)
                st_put(i, 1, _rinv(jnp.sum(acc, axis=1, keepdims=True) * (1.0 / D)))

        def norm(i):
            mu = _rb2(st_get(i, 0, 3))
            ri = st_get(i, 1, 3)
            acc = None
            for k in range(8):
                x = ld(i, k, 3)
                y = (x - mu) * ri
                if k == 7 and not late:
                    PN[pl.ds(pl.multiple_of(PD + 8 + zz, 8), 8), :] = y[24:32]
                    done(y)
                if not router:
                    XN[k, pl.ds(pl.multiple_of(row0 + 32 * i, 32), 32), :] = y.astype(BF16)
                    continue
                y = _rb2(y)
                wr = WR[:, k * 128:(k + 1) * 128]
                yw = y * jnp.concatenate([wr, wr, wr, wr], axis=0)
                acc = yw if acc is None else acc + yw
                R[pl.ds(pl.multiple_of(row0 + 32 * i, 32), 32), k * 128:(k + 1) * 128] = (x + y).astype(BF16)
            if router:
                r = jnp.broadcast_to(_rb(jnp.sum(acc, axis=1, keepdims=True)), (32, 128))
                b = pltpu.bitcast(r, I32)
                sg = b >> 31
                tok = jax.lax.broadcasted_iota(I32, (32, 128), 0) + (row0 + 32 * i - (S - 1))
                key = ((b & 0x7FFF0000) ^ sg) - (sg + tok)
                hi = RT[0:8, :]
                lo = RT[8:16, :]
                for j in range(4):
                    kj = key[8 * j:8 * j + 8]
                    lo = jnp.maximum(lo, jnp.minimum(hi, kj))
                    hi = jnp.maximum(hi, kj)
                RT[0:8, :] = hi
                RT[8:16, :] = lo
                if late:
                    done(pltpu.bitcast(lo, F32))

        n = nrows // 32
        if late > 1 and n > 1:
            return ([_bind(f, i, i + 1) for f in (mean, var) for i in range(0, n, 2)]
                    + [_bind(norm, i) for i in range(n)])
        return [_bind(f, i) for f in (mean, var, norm) for i in range(n)]

    def proj_rounds(seg, g, buf, order=(0, 1, 2, 3)):
        Kb, Qm, PQ, PK, VT, SB, RD = buf
        zz = ZS[0]
        part = {}

        def rnd(c, j, half):
            r2 = pl.multiple_of(seg * (L // 2) + c * 64 + zz * j, 64)
            xn = jnp.concatenate([pltpu.bitcast(XNu[k, pl.ds(r2, 64), :], BF16)
                                  for k in range(4 * half, 4 * half + 4)], axis=1)
            w = pltpu.bitcast(Wu[g, j, pl.ds(pl.multiple_of(256 * half + zz * c, 256), 256), :], BF16)
            t = jnp.dot(xn, w, preferred_element_type=F32)
            if half == 0:
                part[0] = t
                return
            t = t + part[0]
            PN[PD:PD + 8, :] = t[120:128]
            PG[512:520, :] = t[120:128]
            rows = pl.ds(c * 128 if isinstance(c, int) else pl.multiple_of(c * 128, 128), 128)
            if j == 0:
                qt = pltpu.bitcast((t * QSCALE).astype(BF16).T, U32)
                for h in range(4):
                    qh = qt[16 * h:16 * h + 16]
                    Qm[c, 16 * h:16 * h + 16, :] = pltpu.roll(qh, 32 * h, 1) if h else qh
                PQ[rows, :] = _phi(t).astype(BF16)
            elif j == 1:
                Kb[rows, :] = t.astype(BF16)
                PK[rows, :] = _phi(t).astype(BF16)
            else:
                VT[c, 0:64, :] = pltpu.bitcast(t.astype(BF16).T, U32)

        return [_bind(rnd, c, j, half) for c in order for j in range(3) for half in range(2)]

    pins = [None]

    def pin_load():
        pins.append(pltpu.bitcast(PG[pl.ds(pl.multiple_of(528 + ZS[0], 8), 8), :], U32)
                    | pltpu.bitcast(R[pl.ds(pl.multiple_of(S + ZS[0], 16), 16), 0:128], U32)
                    | Tu[0, pl.ds(pl.multiple_of(S // 2 + ZS[0], 8), 8), :])

    def out_rounds(seg, off, nrows, last=False):
        zz = ZS[0]
        part = {}
        n2 = nrows // 2

        def rnd(n, half, pin=False):
            o2 = pl.multiple_of(((seg % 2) * L + off) // 2 + zz * (n + 1), 16)
            o = [OBu[k, pl.ds(o2, n2), :] for k in range(4 * half, 4 * half + 4 - (last and half))]
            if last and half:
                o.append(OL[off // 128][pl.ds(pl.multiple_of((off % 128) // 2 + zz * (n + 1), 16), n2), :])
            if pin:
                pins[0:2] = pins[1:2]
            if last and pins[0] is not None:
                o = [jnp.concatenate([v[0:8] | pins[0], v[8:]], axis=0) for v in o]
            o = jnp.concatenate([pltpu.bitcast(v, BF16) for v in o], axis=1)
            w = pltpu.bitcast(WOu[n, pl.ds(pl.multiple_of(256 * half + zz * (seg * L + off), 256), 256), :], BF16)
            t = jnp.dot(o, w, preferred_element_type=F32)
            if half == 0:
                part[0] = t
                return
            x = R[pl.ds(pl.multiple_of(seg * L + off, 32), nrows), n * 128:(n + 1) * 128].astype(F32)
            t = t + part[0]
            PN[PD:PD + 8, :] = t[nrows - 8:nrows]
            PG[512:520, :] = t[nrows - 8:nrows]
            T[n, pl.ds(pl.multiple_of(seg * L + off, 32), nrows), :] = (x + _rb2(t)).astype(BF16)

        return [_bind(rnd, n, half) for n in range(8) for half in range(2)]

    def attn(seg, g, buf, mem, last=False):
        Kb, Qm, PQ, PK, VT, SB, RD = buf
        Kb, PQ, PK = Kb.bitcast(U32), PQ.bitcast(U32), PK.bitcast(U32)
        zz = ZS[0]
        pg0 = 0 if buf is bufs[0] else 256
        ml = {}
        m8_ = {}
        acc = {}
        fin = {}

        def bfly(e, rows):
            lane = jax.lax.broadcasted_iota(jnp.int32, (rows, 128), 1)
            s0 = (lane & 32) != 0
            s1 = (lane & 64) != 0

            def sel(m, x, y):
                if x is None and y is None:
                    return None
                z = jnp.zeros_like(x if y is None else y)
                return jnp.where(m, z if x is None else x, z if y is None else y)

            a = [[sel(s1, e[2 + j], e[j]), sel(s1, e[j], e[2 + j])] for j in range(2)]
            return [sel(s0, a[1][0], a[0][0]), sel(s0, a[0][0], a[1][1]),
                    sel(s0, a[1][1], a[0][1]), sel(s0, a[0][1], a[1][0])]

        def put_max(qb, m8):
            m = jnp.broadcast_to(jnp.max(m8, axis=0, keepdims=True), (8, 512))
            m = [m[:, 128 * h:128 * (h + 1)] for h in range(4)]
            for i, v in enumerate(m + bfly(m, 8)):
                if qb > 0 or i >= 4:
                    PG[pg0 + 64 * qb + 8 * i:pg0 + 64 * qb + 8 * i + 8, :] = v

        def get_max(i):
            for qb, h in [(dg.index(i), 4 + j) for j in range(4)] if i in dg else [t[:2] for t in tiles(i)]:
                if (i, h) not in ml:
                    ml[(i, h)] = PG[pl.ds(pl.multiple_of(zz * (i + 1) + pg0 + 64 * qb + 8 * h, 8), 8), :]

        def diag(qa):
            lm = [jnp.concatenate([LM[i]] * 2, axis=0) for i in range(4)]
            for qb, rev in ((qa, False), (qa + 1, True)):
                m8 = [None] * 4
                for j in range(3, -1, -1):
                    w = jnp.concatenate([Qm[qb, 16 * h:16 * h + 16, :] & lm[(j + h) % 4] for h in range(4)], axis=0)
                    rs = range(j, -1, -1) if rev else range(j + 1)
                    kq = jnp.concatenate([Kb[64 * qb + 16 * r:64 * qb + 16 * r + 16, :] for r in rs], axis=0)
                    d = jnp.dot(pltpu.bitcast(kq, BF16), pltpu.bitcast(w, BF16), preferred_element_type=F32)
                    for i, r in enumerate(rs):
                        v = d[32 * i:32 * i + 32] + CM[...] if r == j else d[32 * i:32 * i + 32]
                        SB[qb][j, 128 * qb + 32 * r:128 * qb + 32 * r + 32, :] = v
                        mx = jnp.max(v.reshape(4, 8, 128), axis=0)
                        m8[j] = mx if m8[j] is None else jnp.maximum(m8[j], mx)
                m8_[qb] = jnp.concatenate(bfly(m8, 8), axis=1)
            if qa == 0:
                put_max(0, m8_[0])

        def qk(qb):
            z16 = jnp.zeros((16, 128), U32)
            w = jnp.concatenate([jnp.concatenate([Qm[qb, 16 * h:16 * h + 16, :] if i == h else z16
                                                  for i in range(4)], axis=0) for h in range(4)], axis=1)
            s = jnp.dot(pltpu.bitcast(Kb[0:64 * qb, :], BF16), pltpu.bitcast(w, BF16), preferred_element_type=F32)
            m8 = m8_[qb]
            for c in range(qb):
                blk = s[c * 128:(c + 1) * 128, :]
                for h in range(4):
                    SB[qb][h, c * 128:(c + 1) * 128, :] = blk[:, 128 * h:128 * (h + 1)]
                m8 = jnp.maximum(m8, jnp.max(blk.reshape(16, 8, 512), axis=0))
            put_max(qb, m8)

        def pv(qb, h, c, p, l8):
            o = jnp.dot(pltpu.bitcast(VT[c, 16 * h:16 * h + 16, :], BF16), p, preferred_element_type=F32)
            if (qb, h) in acc:
                o0, l0, n = acc[(qb, h)]
                o = o + o0
                l8 = l0 + l8
            else:
                n = 0
            acc[(qb, h)] = (o, l8, n + 1)
            if n == qb:
                gt = GT[g]
                l = jnp.sum(l8, axis=0, keepdims=True)
                res = o * (gt[4 + h:5 + h, :] * _rcp(l))
                if h > 0:
                    res = pltpu.roll(res, 128 - 32 * h, 1)
                if mem:
                    num = RD[zz + qb, 32 * h:32 * h + 32, :]
                    den = RD[zz + qb, 128:136, :][h:h + 1, :] + 1e-06
                    res = num * (gt[h:h + 1, :] * _rcp(den)) + res
                fin[(qb, h)] = res

        def pv_tile(i, qb, h, c):
            m = jnp.concatenate([ml[(i, h)]] * 16, axis=0)
            p = jnp.exp2(SB[qb][h, pl.ds(pl.multiple_of(zz + c * 128, 128), 128), :] - m)
            l8 = p[120:128]
            for r in range(14, -1, -1):
                l8 = l8 + p[8 * r:8 * r + 8]
            pv(qb, h, c, p.astype(BF16), l8)

        def pv_diag(qb):
            m = [ml[(dg[qb], 4 + j)] for j in range(4)]
            l8 = [None] * 4
            w = {}
            for r in range(3, -1, -1):
                e = [None] * 4
                for j in range(r, 4):
                    mj = jnp.concatenate([m[j]] * 2, axis=0)
                    p = [jnp.exp2(SB[qb][j, pl.ds(zz + 128 * qb + 32 * r + i, 16, stride=2), :] - mj)
                         for i in range(2)]
                    for v in (p[1][8:16], p[1][0:8], p[0][8:16], p[0][0:8]):
                        l8[j] = v if l8[j] is None else l8[j] + v
                    e[j] = pltpu.pack_elementwise(p, packed_dtype=BF16)
                w[r] = bfly(e, 16)
            l8 = bfly(l8, 8)
            for h in range(4):
                pv(qb, h, qb, pltpu.bitcast(jnp.concatenate([w[r][h] for r in range(4)], axis=0), BF16), l8[h])

        def put(qb):
            ot = jnp.concatenate([fin[(qb, i)] for i in range(4)], axis=0).astype(BF16)
            if last:
                ot = pltpu.bitcast(ot.T, U32)
                OL[qb][...] = ot
                PG[pl.ds(pl.multiple_of(520 + zz, 8), 8), :] = pltpu.bitcast(ot[56:64], F32)
                return
            o2 = pl.multiple_of((seg % 2) * (L // 2) + 64 * qb, 64)
            OBu[g, pl.ds(o2, 64), :] = pltpu.bitcast(ot.T, U32)

        dg = (0, 1, 3, 6)

        def tiles(i):
            i = (2, 4, 5, 7, 8, 9).index(i)
            return [(qb, h, c) for qb in range(4) for h in range(4) for c in range(qb)][4 * i:4 * i + 4]

        def grp(i):
            get_max(i)
            if i in dg:
                pv_diag(dg.index(i))
                return
            for t in tiles(i):
                pv_tile(i, *t)

        def rd():
            r = jax.lax.dot_general(MST[g].astype(BF16), pltpu.bitcast(PQ[...], BF16), NT, preferred_element_type=F32)
            for c in range(4):
                RD[c] = r[0:136, c * 128:(c + 1) * 128]

        def upd():
            vall = pltpu.bitcast(jnp.concatenate([VT[c] for c in range(4)], axis=1), BF16)
            u = jnp.dot(vall, pltpu.bitcast(PK[...], BF16), preferred_element_type=F32)
            rr = jax.lax.broadcasted_iota(jnp.int32, (144, 128), 0)
            cc = jax.lax.broadcasted_iota(jnp.int32, (144, 128), 1) // DH
            keep = jnp.where(rr < 128, rr // DH, rr - 128) == cc
            u = jnp.where(keep, u, 0.0)
            MST[g] = MST[g + zz] + u if mem else u

        def act(tok):
            if tok[0] == "Q":
                qk(int(tok[1]))
            elif tok[0] == "D":
                diag(int(tok[1]))
            elif tok[0] == "G":
                grp(int(tok[1]))
            elif tok[0] == "g":
                get_max(int(tok[1]))
            elif tok[0] == "S":
                put(int(tok[1]))
            elif tok == "R":
                rd()
            else:
                assert tok == "U"
                upd()

        return act

    def run(sched, steps, queues):
        queues = {k: list(v) for k, v in queues.items()}
        si = 0
        for tok in sched.split():
            if tok == "|":
                si += 1
            elif tok == "z":
                pin_load()
            elif tok == "Z":
                queues["O"].pop(0)(pin=True)
            elif tok in queues:
                queues[tok].pop(0)()
            elif tok[-1] == "+":
                steps[si + 1](tok[:-1])
            else:
                steps[si](tok)
        assert all(not v for v in queues.values()), {k: len(v) for k, v in queues.items()}

    def ffn_patch(layer):
        hi = RT[0:8, :]
        lo = RT[8:16, :]
        RT[...] = jnp.full((16, 128), IMIN, I32)
        for sh in (4, 2, 1):
            h2 = pltpu.roll(hi, sh, 0)
            lo = jnp.maximum(jnp.minimum(hi, h2), jnp.maximum(lo, pltpu.roll(lo, sh, 0)))
            hi = jnp.maximum(hi, h2)
        i1 = jnp.clip(S - 1 - (hi[0, 0] & (S - 1)), 0, S - 1)
        i2 = jnp.clip(S - 1 - (lo[0, 0] & (S - 1)), 0, S - 1)
        b1 = pl.multiple_of((i1 // 16) * 16, 16)
        b2 = pl.multiple_of((i2 // 16) * 16, 16)
        i16 = jax.lax.broadcasted_iota(jnp.int32, (16, 1), 0)
        s1 = i16 + b1 == i1
        s2 = i16 + b2 == i2

        def pick(i):
            u = jnp.concatenate([jnp.broadcast_to(Tu[k, pl.ds(i // 2, 1), :], (8, 128)) for k in range(8)], axis=1)
            sh = (16 - 16 * (i % 2)).astype(U32)
            return pltpu.bitcast((u << sh) & jnp.uint32(0xFFFF0000), F32)

        x1 = jnp.concatenate([pick(i1), pick(i2)], axis=0)
        yb = _ln_f32(x1).astype(BF16)
        kv = jnp.concatenate([hi, lo], axis=0) & -65536
        rsel = pltpu.bitcast(jnp.where(kv < 0, (-kv) | IMIN, kv), F32)[:, 0:1]

        def dot512(x, ref, r, c):
            return jnp.dot(x, ref[512 * r:512 * (r + 1), 128 * c:128 * (c + 1)], preferred_element_type=F32)

        def gate_up(c):
            hs = []
            for n in range(4 * c, 4 * c + 4):
                gt, up = [_rb(dot512(yb[:, :512], w, 0, n) + dot512(yb[:, 512:], w, 1, n)) for w in (WG, WU)]
                hs.append(_rb(gt * _rb(jax.nn.sigmoid(gt))) * up)
            return jnp.concatenate(hs, axis=1).astype(BF16)

        hm = gate_up(0)
        yv = None
        for c in range(NFC):
            nxt = gate_up(c + 1) if c + 1 < NFC else None
            dn = jnp.concatenate([dot512(hm, WD, c, n) for n in range(8)], axis=1)
            yv = dn if yv is None else yv + dn
            hm = nxt

        def patch_r():
            x2 = _rb(x1 + _rb(yb.astype(F32) + _rb(_rb(yv) * _rb(jax.nn.sigmoid(rsel)))))
            for b, sel, lo in ((b1, s1, 0), (b2, s2, 8)):
                new = jnp.concatenate([x2[lo:lo + 8], x2[lo:lo + 8]], axis=0)
                R[pl.ds(b, 16), :] = jnp.where(sel, new, R[pl.ds(b, 16), :].astype(F32)).astype(BF16)
            return x2

        def patch_xn():
            xn = _rb(_ln_f32(patch_r()))
            for b, sel, lo in ((b1, s1, 0), (b2, s2, 8)):
                new = jnp.concatenate([xn[lo:lo + 8], xn[lo:lo + 8]], axis=0)
                for k in range(8):
                    XN[k, pl.ds(b, 16), :] = jnp.where(sel, new[:, k * 128:(k + 1) * 128],
                                                       XN[k, pl.ds(b, 16), :].astype(F32)).astype(BF16)

        @pl.when(layer == 0)
        def _():
            hit = [(i1 // 128 == c) | (i2 // 128 == c) for c in range(4)]
            ca = jnp.where(hit[0], jnp.where(hit[1], 2, 1), 0)
            cb = jnp.where(hit[3], jnp.where(hit[2], 1, 2), 3)
            cc = jnp.where(ca == 0, jnp.where(cb == 1, 2, 1), 0)
            cd = jnp.clip(6 - ca - cb - cc, 0, 3)
            run("P P P P P P P P P P P P x P P m m P P m m P P m m P P m m P P P P", [],
                {"P": proj_rounds(0, 0, bufs[0], (ca, cb, cc, cd)), "x": [patch_xn],
                 "m": ln_units(L, 128, False, 2)[:8]})

        @pl.when(layer == 1)
        def _():
            for s in range(11):
                out_copy(0, 128, s).wait()
            out_copy(0, 640, 11).wait()
            patch_r()
            c1 = out_copy(b1, 16, 0)
            c1.start()

            @pl.when(b2 != b1)
            def _():
                c2 = out_copy(b2, 16, 1)
                c2.start()
                c2.wait()

            c1.wait()

    p0 = proj_rounds(0, 0, bufs[0])
    x_copy(0, 128, 0).wait()
    for f in ln_units(0, 128, False, 2):
        f()
    for c in range(4):
        if c == 0:
            for j in range(3):
                w_copy(0, j).wait()
        if c < 3:
            x_copy(128 * (c + 1), 128, c + 1).wait()
            run("f f f f P P f f f f P P P P f f f f", [],
                {"P": p0[6 * c:6 * c + 6], "f": ln_units(128 * (c + 1), 128, False, 2)})
        else:
            x_copy(0, 128, 4).wait()
            run("m m m m P P m m P P m m P P", [], {"P": p0[18:24], "m": ln_units(L, 128, False, 2)[:8]})

    def layer_body(layer, carry):
        def a_body(gp, carry2):
            g0 = 2 * gp
            g2 = (g0 + 2) % NG

            @pl.when(layer == 0)
            def _():
                @pl.when(gp < 3)
                def _():
                    for j in range(3):
                        w_copy(g0 + 3, j).start()

                @pl.when(gp < 2)
                def _():
                    for j in range(3):
                        w_copy(g0 + 4, j).start()

                @pl.when(gp < 2)
                def _():
                    x_copy(pl.multiple_of(768 + 128 * gp, 128), 128, 6 + gp).start()

                @pl.when(gp == 1)
                def _():
                    for n in range(8):
                        wo_copy(n).start()

                @pl.when(gp >= 2)
                def _():
                    x_copy(pl.multiple_of(gp * L, L), L, 6 + gp).start()

                for j in range(3):
                    w_copy(g0 + 1, j).wait()

                @pl.when(gp < 3)
                def _():
                    for j in range(3):
                        w_copy(g2, j).wait()
                    x_copy(0, 128, 5 + gp).wait()

                @pl.when(gp == 3)
                def _():
                    x_copy(0, L, 8).wait()

            run(SCHED_A, [attn(0, g0, bufs[0], False), attn(0, g0 + 1, bufs[1], False)],
                {"P": proj_rounds(0, g0 + 1, bufs[1]) + proj_rounds(gp // 3, g2, bufs[0]),
                 "n": ln_units(L + gp * 128, 128, False, 2)[8:],
                 "m": ln_units(L + 128 + gp * 128, 128, False, 2)[:8]})
            return carry2

        jax.lax.fori_loop(0, 4, a_body, 0)

        @pl.when(layer == 0)
        def _():
            for c in ffn_copies:
                c.start()
            for n in range(8):
                wo_copy(n).wait()
            x_copy(0, L, 9).wait()

        def b_body(it, carry2):
            seg = 1 + it // 4
            gp = it % 4
            g0 = 2 * gp
            g2 = (g0 + 2) % NG
            prow = (seg - 1) * L + gp * 128
            run(SCHED_B, [attn(seg, g0, bufs[0], True), attn(seg, g0 + 1, bufs[1], True)],
                {"P": proj_rounds(seg, g0 + 1, bufs[1]) + proj_rounds(seg + gp // 3, g2, bufs[0]),
                 "O": out_rounds(seg - 1, gp * 128, 128),
                 "n": ln_units((1024 + it * 128) % S, 128, False, 2)[8:],
                 "m": ln_units((1152 + it * 128) % S, 128, False, 2)[:8],
                 "t": ln_units(prow, 128, True, 0)})

            @pl.when(layer == 1)
            def _():
                out_copy(pl.multiple_of(prow, 128), 128, it).start()

            return carry2

        jax.lax.fori_loop(0, 11, b_body, 0)

        pieces = ((0, 128), (128, 128), (256, 64), (320, 64), (384, 64), (448, 32), (480, 32))
        run(SCHED_T, [attn(3, 6, bufs[0], True), attn(3, 7, bufs[1], True, True)],
            {"P": proj_rounds(3, 7, bufs[1]),
             "O": out_rounds(2, 384, 128) + [f for off, n in pieces for f in out_rounds(3, off, n, True)],
             "n": ln_units(384, 128, False, 2)[8:],
             "t": ln_units(2 * L + 384, 128, True, 0, 1)
             + [f for i, (off, n) in enumerate(pieces)
                for f in ln_units(3 * L + off, n, True, 4 + 2 * (i % 2), 2)]})

        @pl.when(layer == 0)
        def _():
            for c in ffn_copies:
                c.wait()

        @pl.when(layer == 1)
        def _():
            out_copy(S - 640, 640, 11).start()

        ffn_patch(layer)
        return carry

    jax.lax.fori_loop(0, 2, layer_body, 0)


@jax.jit
def pallas_interleave_layers__memory_aug_infini_attn__moe_arch_mod__prompt_kernel(
    A_x: jax.Array,
    A_wq: jax.Array,
    A_wk: jax.Array,
    A_wv: jax.Array,
    A_wo: jax.Array,
    A_beta: jax.Array,
    B_x: jax.Array,
    B_w_r: jax.Array,
    B_w_gate: jax.Array,
    B_w_up: jax.Array,
    B_w_down: jax.Array,
):
    hbm = pl.BlockSpec(memory_space=pl.ANY)
    vmem = pl.BlockSpec(memory_space=pltpu.VMEM)
    qkv_set = [
        pltpu.VMEM((L, 128), BF16),
        pltpu.VMEM((4, 64, 128), U32),
        pltpu.VMEM((L, 128), BF16),
        pltpu.VMEM((L, 128), BF16),
        pltpu.VMEM((4, 72, 128), U32),
        pltpu.VMEM((4, 128, 128), F32),
        pltpu.VMEM((4, 256, 128), F32),
        pltpu.VMEM((4, 384, 128), F32),
        pltpu.VMEM((4, 512, 128), F32),
        pltpu.VMEM((4, 136, 128), F32),
    ]
    scratch = [
        pltpu.VMEM((S + 16, D), BF16),
        pltpu.VMEM((8, S + 16, 128), BF16),
        pltpu.VMEM((8, S, 128), BF16),
        pltpu.VMEM((NG, 3, D, 128), BF16),
        pltpu.VMEM((8, D, 128), BF16),
        pltpu.VMEM((D, FF), BF16),
        pltpu.VMEM((D, FF), BF16),
        pltpu.VMEM((FF, D), BF16),
        pltpu.VMEM((NG, 2 * L, 128), BF16),
        pltpu.VMEM((NG, 144, 128), F32),
        pltpu.VMEM((NG, 8, 128), F32),
        pltpu.VMEM((8, D), F32),
        pltpu.VMEM((32, 128), F32),
        pltpu.VMEM((4, 8, 128), U32),
        pltpu.VMEM((PD + 16, 128), F32),
        pltpu.VMEM((536, 128), F32),
        pltpu.VMEM((16, 128), I32),
    ] + qkv_set + qkv_set + [pltpu.VMEM((64, 128), U32)] * 4 + [
        pltpu.VMEM((1024, 128), F32),
        pltpu.SMEM((1,), jnp.int32),
        pltpu.SemaphoreType.DMA((10,)),
        pltpu.SemaphoreType.DMA((NG, 3)),
        pltpu.SemaphoreType.DMA((11,)),
        pltpu.SemaphoreType.DMA((12,)),
    ]
    return pl.pallas_call(
        _kernel,
        out_shape=jax.ShapeDtypeStruct((1, S, D), BF16),
        in_specs=[hbm, hbm, hbm, hbm, hbm, vmem, vmem, hbm, hbm, hbm],
        out_specs=hbm,
        scratch_shapes=scratch,
        compiler_params=pltpu.CompilerParams(vmem_limit_bytes=100 * 1024 * 1024),
    )(A_x, A_wq, A_wk, A_wv, A_wo, A_beta, B_w_r, B_w_gate, B_w_up, B_w_down)
```

```python
import jax
import jax.numpy as jnp
import jax.experimental.pallas as pl
import jax.experimental.pallas.tpu as pltpu

F32 = jnp.float32
BF16 = jnp.bfloat16
U32 = jnp.uint32
I32 = jnp.int32
IMIN = -2147483648

S = 2048
D = 1024
H = 32
DH = 32
NSEG = 4
L = S // NSEG
NG = 8
FF = 3584
FCH = 512
NFC = FF // FCH
LOG2E = 1.4426950408889634
QSCALE = (DH ** -0.5) * LOG2E
NEG = -1000000000.0 * LOG2E
EPS_LN = 1.0013580322265625e-05
BIG = 3.0e38
NT = (((1,), (1,)), ((), ()))
PZ = 1024
PD = 1032

SCHED_A = ("D0 g0 n Q1 g1 n D2 n Q2 n G0 S0 P P G1 g2 m P P G2 g3 S1 m P P G3 g4 Q3 m P P G4 g5 m P P G5 g6 S2 m "
           "P P G6 g7 m P P G7 g8 m P P G8 g9 m P P G9 S3 P P D0+ P P Q1+ g0+ P P U | G0 g1 S0 P P D2 G1 g2 P P "
           "Q2 G2 g3 S1 P P G3 g4 P P G4 g5 Q3 P P G5 g6 S2 P P G6 g7 P P G7 g8 P P G8 g9 P P G9 S3 P P P P P P "
           "U ")
SCHED_B = ("O O n O O n m O O n m O O n m O O m m O O m D0 O O g0 m Q1 R O O g1 m G0 S0 P P D2 G1 g2 t t P P Q2 "
           "G2 g3 S1 t t P P G3 g4 t P P G4 g5 Q3 t P P G5 g6 S2 t P P G6 g7 t P P G7 g8 P P G8 g9 P P G9 S3 t P "
           "P D0+ t P P Q1+ g0+ P P U | R G0 g1 S0 P P D2 G1 g2 P P Q2 G2 g3 S1 P P G3 g4 P P G4 g5 Q3 P P G5 g6 "
           "S2 P P G6 g7 P P G7 g8 P P G8 g9 P P G9 S3 t P P t P P P P U ")
SCHED_T = ("O O n O O n O O n D0 Q1 g0 R O O n G0 g1 S0 D2 G1 g2 P P Q2 G2 g3 S1 P P G3 g4 P P G4 g5 Q3 P P G5 "
           "g6 S2 P P G6 g7 P P G7 g8 P P G8 g9 P P G9 S3 P P D0+ P P Q1+ g0+ P P P P | R O O G0 g1 O O S0 D2 G1 "
           "g2 O O Q2 G2 g3 O O S1 G3 g4 O O G4 g5 Q3 t t O O G5 g6 t t t O O S2 G6 g7 t O O G7 g8 t O O G8 g9 t "
           "O O G9 t O O S3 t z O O t t z O O t z Z O t z Z O t z Z O t z Z O t z Z O t z Z O t z Z O t z Z O t "
           "z O O t z Z O t z O O z Z O t z Z O t z Z O z Z O t z Z O t z Z O z Z O t z Z O t z Z O t z Z O z Z "
           "O t z Z O z Z O t z Z O t z Z O t z Z O z Z O t z Z O z Z O t z Z O z Z O t z Z O Z O t z O O Z O O "
           "O t z Z O Z O t z O O t z Z O O O t O O Z O O O t Z O Z O t t t ")


def _rb(t):
    return t.astype(BF16).astype(F32)


def _rb2(t):
    n = t.shape[0] // 2
    p = pltpu.pack_elementwise([t[:n], t[n:]], packed_dtype=BF16)
    return jnp.concatenate([pltpu.unpack_elementwise(p, index=i, packed_dtype=BF16, unpacked_dtype=F32)
                            for i in range(2)], axis=0)


def _rcp(d):
    d = jnp.minimum(d, BIG)
    r = pl.reciprocal(d, approx=True)
    return r * (2.0 - d * r)


def _rinv(var):
    v = _rb(_rb(var) + EPS_LN)
    vc = jnp.minimum(v, BIG)
    return jnp.minimum(_rcp(_rb(vc * jax.lax.rsqrt(vc))), 1e30 * pl.reciprocal(v, approx=True))


def _ln_f32(x):
    mu = jnp.sum(x, axis=1, keepdims=True) * (1.0 / D)
    xc = x - mu
    var = jnp.sum(xc * xc, axis=1, keepdims=True) * (1.0 / D)
    return (x - _rb(mu)) * _rinv(var)


def _phi(t):
    return jnp.maximum(t, 0.0) + jnp.exp(jnp.minimum(t, 0.0))


def _bind(f, *a):
    return lambda **kw: f(*a, **kw)


def _kernel(x_hbm, wq_hbm, wk_hbm, wv_hbm, wo_hbm, beta_ref, wr_ref, wg_hbm, wu_hbm, wd_hbm,
            out_hbm,
            R, T, XN, W, WO, WG, WU, WD, OB, MST, GT, WR, CM, LM, PN, PG, RT,
            K0, Q0, PQ0, PK0, VT0, SA0, SB0, SC0, SD0, RD0, K1, Q1, PQ1, PK1, VT1, SA1, SB1, SC1, SD1, RD1,
            OL0, OL1, OL2, OL3, PS, ZS, sx, sw, sm, so):
    bufs = ((K0, Q0, PQ0, PK0, VT0, (SA0, SB0, SC0, SD0), RD0), (K1, Q1, PQ1, PK1, VT1, (SA1, SB1, SC1, SD1), RD1))
    OL = (OL0, OL1, OL2, OL3)
    ZS[0] = 0
    XNu = XN.bitcast(U32)
    Wu = W.bitcast(U32)
    WOu = WO.bitcast(U32)
    OBu = OB.bitcast(U32)
    Tu = T.bitcast(U32)

    def x_copy(row0, n, s):
        return pltpu.make_async_copy(x_hbm.at[0, pl.ds(row0, n), :], R.at[pl.ds(row0, n), :], sx.at[s])

    def w_copy(g, j):
        src = (wq_hbm, wk_hbm, wv_hbm)[j]
        return pltpu.make_async_copy(src.at[:, pl.ds(pl.multiple_of(g * 128, 128), 128)], W.at[g, j], sw.at[g, j])

    def w_all(g, start):
        for j in range(3):
            w_copy(g, j).start() if start else w_copy(g, j).wait()

    def wo_copy(n):
        return pltpu.make_async_copy(wo_hbm.at[:, pl.ds(n * 128, 128)], WO.at[n], sm.at[n])

    ffn_copies = (pltpu.make_async_copy(wg_hbm, WG, sm.at[8]),
                  pltpu.make_async_copy(wu_hbm, WU, sm.at[9]),
                  pltpu.make_async_copy(wd_hbm, WD, sm.at[10]))

    def out_copy(row0, n, s):
        return pltpu.make_async_copy(R.at[pl.ds(row0, n), :], out_hbm.at[0, pl.ds(row0, n), :], so.at[s])

    x_copy(0, 128, 0).start()
    w_all(0, True)
    x_copy(128, 128, 1).start()

    gsig = jax.nn.sigmoid(beta_ref[...].astype(F32).reshape(1, H))
    eye = (jax.lax.broadcasted_iota(jnp.int32, (H, H), 0)
           == jax.lax.broadcasted_iota(jnp.int32, (H, H), 1))
    gcol = jnp.sum(jnp.where(eye, jnp.broadcast_to(gsig, (H, H)), 0.0), axis=1, keepdims=True)
    gfull = jnp.broadcast_to(gcol, (H, 128))
    for g in range(NG):
        GT[g, 0:4, :] = gfull[4 * g:4 * g + 4, :]
        GT[g, 4:8, :] = 1.0 - gfull[4 * g:4 * g + 4, :]
    WR[...] = jnp.broadcast_to(wr_ref[...].astype(F32).reshape(1, D), (8, D))
    kk = jax.lax.broadcasted_iota(jnp.int32, (32, 128), 0)
    qq = jax.lax.broadcasted_iota(jnp.int32, (32, 128), 1) % 32
    CM[...] = jnp.where(qq < kk, NEG, 0.0).astype(F32)
    for c in range(4):
        LM[c] = jnp.where(jax.lax.broadcasted_iota(jnp.int32, (8, 128), 1) // DH == c,
                          jnp.uint32(0xFFFFFFFF), jnp.uint32(0))
        VT0[c, 64:72, :] = pltpu.bitcast(jnp.ones((16, 128), BF16), U32)
        VT1[c, 64:72, :] = pltpu.bitcast(jnp.ones((16, 128), BF16), U32)
    RT[...] = jnp.full((16, 128), IMIN, I32)
    PN[PZ:PZ + 8, :] = jnp.zeros((8, 128), F32)
    PG[528:536, :] = jnp.zeros((8, 128), F32)
    R[S:S + 16, 0:128] = jnp.zeros((16, 128), BF16)
    T[0, S:S + 16, :] = jnp.zeros((16, 128), BF16)

    def ln_units(row0, nrows, router, slab, late=0, free=False):
        zz = ZS[0]
        st = PS if late else PN

        def srow(r, v, m):
            return r if free else pl.multiple_of(r + zz * v, m)

        def ld(i, k, v):
            if router:
                r2 = pl.multiple_of(row0 // 2 + 16 * i + zz * v, 16)
                return pltpu.bitcast(Tu[k, pl.ds(r2, 16), :], BF16).astype(F32)
            r1 = pl.multiple_of(row0 + 32 * i + zz * v, 32)
            return R[pl.ds(r1, 32), k * 128:(k + 1) * 128].astype(F32)

        def st_put(i, j, val):
            st[pl.ds(srow((slab + j) * 128 + 32 * i, 1, 32), 32), :] = jnp.broadcast_to(val, (32, 128))

        def done(val):
            if not free:
                PG[pl.ds(pl.multiple_of(520 + zz, 8), 8), :] = val[-8:]

        def st_get(i, j, v):
            return st[pl.ds(srow((slab + j) * 128 + 32 * i, v, 32), 32), :]

        def mean(*ii):
            z = PN[pl.ds(srow(PZ, 1, 8), 8), :]
            accs = []
            for i in ii:
                acc = jnp.concatenate([z, z, z, z], axis=0)
                for k in range(8):
                    acc = acc + ld(i, k, 1)
                accs.append(acc)
            for i, acc in zip(ii, accs):
                done(acc)
                st_put(i, 0, jnp.sum(acc, axis=1, keepdims=True) * (1.0 / D))

        def var(*ii):
            mus = [st_get(i, 0, 2) for i in ii]
            for i, mu in zip(ii, mus):
                acc = None
                for k in range(8):
                    xc = ld(i, k, 2) - mu
                    acc = xc * xc if acc is None else acc + xc * xc
                done(acc)
                st_put(i, 1, _rinv(jnp.sum(acc, axis=1, keepdims=True) * (1.0 / D)))

        def norm(i):
            mu = _rb2(st_get(i, 0, 3))
            ri = st_get(i, 1, 3)
            acc = None
            for k in range(8):
                x = ld(i, k, 3)
                y = (x - mu) * ri
                if k == 7 and not late and not free:
                    PN[pl.ds(pl.multiple_of(PD + 8 + zz, 8), 8), :] = y[24:32]
                    done(y)
                if not router:
                    XN[k, pl.ds(pl.multiple_of(row0 + 32 * i, 32), 32), :] = y.astype(BF16)
                    continue
                y = _rb2(y)
                wr = WR[:, k * 128:(k + 1) * 128]
                yw = y * jnp.concatenate([wr, wr, wr, wr], axis=0)
                acc = yw if acc is None else acc + yw
                R[pl.ds(pl.multiple_of(row0 + 32 * i, 32), 32), k * 128:(k + 1) * 128] = (x + y).astype(BF16)
            if router:
                r = jnp.broadcast_to(_rb(jnp.sum(acc, axis=1, keepdims=True)), (32, 128))
                b = pltpu.bitcast(r, I32)
                sg = b >> 31
                tok = jax.lax.broadcasted_iota(I32, (32, 128), 0) + (row0 + 32 * i - (S - 1))
                key = ((b & 0x7FFF0000) ^ sg) - (sg + tok)
                hi = RT[0:8, :]
                lo = RT[8:16, :]
                for j in range(4):
                    kj = key[8 * j:8 * j + 8]
                    lo = jnp.maximum(lo, jnp.minimum(hi, kj))
                    hi = jnp.maximum(hi, kj)
                RT[0:8, :] = hi
                RT[8:16, :] = lo
                if late:
                    done(pltpu.bitcast(lo, F32))

        n = nrows // 32
        if late > 1 and n > 1:
            return ([_bind(f, i, i + 1) for f in (mean, var) for i in range(0, n, 2)]
                    + [_bind(norm, i) for i in range(n)])
        return [_bind(f, i) for f in (mean, var, norm) for i in range(n)]

    def proj_rounds(seg, g, buf, order=(0, 1, 2, 3)):
        Kb, Qm, PQ, PK, VT, SB, RD = buf
        zz = ZS[0]
        part = {}

        def rnd(c, j, half):
            r2 = pl.multiple_of(seg * (L // 2) + c * 64 + zz * j, 64)
            xn = jnp.concatenate([pltpu.bitcast(XNu[k, pl.ds(r2, 64), :], BF16)
                                  for k in range(4 * half, 4 * half + 4)], axis=1)
            w = pltpu.bitcast(Wu[g, j, pl.ds(pl.multiple_of(256 * half + zz * c, 256), 256), :], BF16)
            t = jnp.dot(xn, w, preferred_element_type=F32)
            if half == 0:
                part[0] = t
                return
            t = t + part[0]
            PN[PD:PD + 8, :] = t[120:128]
            PG[512:520, :] = t[120:128]
            rows = pl.ds(c * 128 if isinstance(c, int) else pl.multiple_of(c * 128, 128), 128)
            if j == 0:
                qt = pltpu.bitcast((t * QSCALE).astype(BF16).T, U32)
                for h in range(4):
                    qh = qt[16 * h:16 * h + 16]
                    Qm[c, 16 * h:16 * h + 16, :] = pltpu.roll(qh, 32 * h, 1) if h else qh
                PQ[rows, :] = _phi(t).astype(BF16)
            elif j == 1:
                Kb[rows, :] = t.astype(BF16)
                PK[rows, :] = _phi(t).astype(BF16)
            else:
                VT[c, 0:64, :] = pltpu.bitcast(t.astype(BF16).T, U32)

        return [_bind(rnd, c, j, half) for c in order for j in range(3) for half in range(2)]

    pins = [None]

    def pin_load():
        pins.append(pltpu.bitcast(PG[pl.ds(pl.multiple_of(528 + ZS[0], 8), 8), :], U32)
                    | pltpu.bitcast(R[pl.ds(pl.multiple_of(S + ZS[0], 16), 16), 0:128], U32)
                    | Tu[0, pl.ds(pl.multiple_of(S // 2 + ZS[0], 8), 8), :])

    def out_rounds(seg, off, nrows, last=False):
        zz = ZS[0]
        part = {}
        n2 = nrows // 2

        def rnd(n, half, pin=False):
            o2 = pl.multiple_of(((seg % 2) * L + off) // 2 + zz * (n + 1), 16)
            o = [OBu[k, pl.ds(o2, n2), :] for k in range(4 * half, 4 * half + 4 - (last and half))]
            if last and half:
                o.append(OL[off // 128][pl.ds(pl.multiple_of((off % 128) // 2 + zz * (n + 1), 16), n2), :])
            if pin:
                pins[0:2] = pins[1:2]
            if last and pins[0] is not None:
                o = [jnp.concatenate([v[0:8] | pins[0], v[8:]], axis=0) for v in o]
            o = jnp.concatenate([pltpu.bitcast(v, BF16) for v in o], axis=1)
            w = pltpu.bitcast(WOu[n, pl.ds(pl.multiple_of(256 * half + zz * (seg * L + off), 256), 256), :], BF16)
            t = jnp.dot(o, w, preferred_element_type=F32)
            if half == 0:
                part[0] = t
                return
            x = R[pl.ds(pl.multiple_of(seg * L + off, 32), nrows), n * 128:(n + 1) * 128].astype(F32)
            t = t + part[0]
            PN[PD:PD + 8, :] = t[nrows - 8:nrows]
            PG[512:520, :] = t[nrows - 8:nrows]
            T[n, pl.ds(pl.multiple_of(seg * L + off, 32), nrows), :] = (x + _rb2(t)).astype(BF16)

        return [_bind(rnd, n, half) for n in range(8) for half in range(2)]

    def attn(seg, g, buf, mem, last=False):
        Kb, Qm, PQ, PK, VT, SB, RD = buf
        Kb, PQ, PK = Kb.bitcast(U32), PQ.bitcast(U32), PK.bitcast(U32)
        zz = ZS[0]
        pg0 = 0 if buf is bufs[0] else 256
        ml = {}
        m8_ = {}
        acc = {}
        fin = {}

        def bfly(e, rows):
            lane = jax.lax.broadcasted_iota(jnp.int32, (rows, 128), 1)
            s0 = (lane & 32) != 0
            s1 = (lane & 64) != 0

            def sel(m, x, y):
                if x is None and y is None:
                    return None
                z = jnp.zeros_like(x if y is None else y)
                return jnp.where(m, z if x is None else x, z if y is None else y)

            a = [[sel(s1, e[2 + j], e[j]), sel(s1, e[j], e[2 + j])] for j in range(2)]
            return [sel(s0, a[1][0], a[0][0]), sel(s0, a[0][0], a[1][1]),
                    sel(s0, a[1][1], a[0][1]), sel(s0, a[0][1], a[1][0])]

        def put_max(qb, m8):
            m = jnp.broadcast_to(jnp.max(m8, axis=0, keepdims=True), (8, 512))
            m = [m[:, 128 * h:128 * (h + 1)] for h in range(4)]
            for i, v in enumerate(m + bfly(m, 8)):
                if qb > 0 or i >= 4:
                    PG[pg0 + 64 * qb + 8 * i:pg0 + 64 * qb + 8 * i + 8, :] = v

        def get_max(i):
            for qb, h in [(dg.index(i), 4 + j) for j in range(4)] if i in dg else [t[:2] for t in tiles(i)]:
                if (i, h) not in ml:
                    ml[(i, h)] = PG[pl.ds(pl.multiple_of(zz * (i + 1) + pg0 + 64 * qb + 8 * h, 8), 8), :]

        def diag(qa):
            lm = [jnp.concatenate([LM[i]] * 2, axis=0) for i in range(4)]
            for qb, rev in ((qa, False), (qa + 1, True)):
                m8 = [None] * 4
                for j in range(3, -1, -1):
                    w = jnp.concatenate([Qm[qb, 16 * h:16 * h + 16, :] & lm[(j + h) % 4] for h in range(4)], axis=0)
                    rs = range(j, -1, -1) if rev else range(j + 1)
                    kq = jnp.concatenate([Kb[64 * qb + 16 * r:64 * qb + 16 * r + 16, :] for r in rs], axis=0)
                    d = jnp.dot(pltpu.bitcast(kq, BF16), pltpu.bitcast(w, BF16), preferred_element_type=F32)
                    for i, r in enumerate(rs):
                        v = d[32 * i:32 * i + 32] + CM[...] if r == j else d[32 * i:32 * i + 32]
                        SB[qb][j, 128 * qb + 32 * r:128 * qb + 32 * r + 32, :] = v
                        mx = jnp.max(v.reshape(4, 8, 128), axis=0)
                        m8[j] = mx if m8[j] is None else jnp.maximum(m8[j], mx)
                m8_[qb] = jnp.concatenate(bfly(m8, 8), axis=1)
            if qa == 0:
                put_max(0, m8_[0])

        def qk(qb):
            z16 = jnp.zeros((16, 128), U32)
            w = jnp.concatenate([jnp.concatenate([Qm[qb, 16 * h:16 * h + 16, :] if i == h else z16
                                                  for i in range(4)], axis=0) for h in range(4)], axis=1)
            s = jnp.dot(pltpu.bitcast(Kb[0:64 * qb, :], BF16), pltpu.bitcast(w, BF16), preferred_element_type=F32)
            m8 = m8_[qb]
            for c in range(qb):
                blk = s[c * 128:(c + 1) * 128, :]
                for h in range(4):
                    SB[qb][h, c * 128:(c + 1) * 128, :] = blk[:, 128 * h:128 * (h + 1)]
                m8 = jnp.maximum(m8, jnp.max(blk.reshape(16, 8, 512), axis=0))
            put_max(qb, m8)

        def pv(qb, h, c, p, l8):
            o = jnp.dot(pltpu.bitcast(VT[c, 16 * h:16 * h + 16, :], BF16), p, preferred_element_type=F32)
            if (qb, h) in acc:
                o0, l0, n = acc[(qb, h)]
                o = o + o0
                l8 = l0 + l8
            else:
                n = 0
            acc[(qb, h)] = (o, l8, n + 1)
            if n == qb:
                gt = GT[g]
                l = jnp.sum(l8, axis=0, keepdims=True)
                res = o * (gt[4 + h:5 + h, :] * _rcp(l))
                if h > 0:
                    res = pltpu.roll(res, 128 - 32 * h, 1)
                if mem:
                    num = RD[zz + qb, 32 * h:32 * h + 32, :]
                    den = RD[zz + qb, 128:136, :][h:h + 1, :] + 1e-06
                    res = num * (gt[h:h + 1, :] * _rcp(den)) + res
                fin[(qb, h)] = res

        def pv_tile(i, qb, h, c):
            m = jnp.concatenate([ml[(i, h)]] * 16, axis=0)
            p = jnp.exp2(SB[qb][h, pl.ds(pl.multiple_of(zz + c * 128, 128), 128), :] - m)
            l8 = p[120:128]
            for r in range(14, -1, -1):
                l8 = l8 + p[8 * r:8 * r + 8]
            pv(qb, h, c, p.astype(BF16), l8)

        def pv_diag(qb):
            m = [ml[(dg[qb], 4 + j)] for j in range(4)]
            l8 = [None] * 4
            w = {}
            for r in range(3, -1, -1):
                e = [None] * 4
                for j in range(r, 4):
                    mj = jnp.concatenate([m[j]] * 2, axis=0)
                    p = [jnp.exp2(SB[qb][j, pl.ds(zz + 128 * qb + 32 * r + i, 16, stride=2), :] - mj)
                         for i in range(2)]
                    for v in (p[1][8:16], p[1][0:8], p[0][8:16], p[0][0:8]):
                        l8[j] = v if l8[j] is None else l8[j] + v
                    e[j] = pltpu.pack_elementwise(p, packed_dtype=BF16)
                w[r] = bfly(e, 16)
            l8 = bfly(l8, 8)
            for h in range(4):
                pv(qb, h, qb, pltpu.bitcast(jnp.concatenate([w[r][h] for r in range(4)], axis=0), BF16), l8[h])

        def put(qb):
            ot = jnp.concatenate([fin[(qb, i)] for i in range(4)], axis=0).astype(BF16)
            if last:
                ot = pltpu.bitcast(ot.T, U32)
                OL[qb][...] = ot
                PG[pl.ds(pl.multiple_of(520 + zz, 8), 8), :] = pltpu.bitcast(ot[56:64], F32)
                return
            o2 = pl.multiple_of((seg % 2) * (L // 2) + 64 * qb, 64)
            OBu[g, pl.ds(o2, 64), :] = pltpu.bitcast(ot.T, U32)

        dg = (0, 1, 3, 6)

        def tiles(i):
            i = (2, 4, 5, 7, 8, 9).index(i)
            return [(qb, h, c) for qb in range(4) for h in range(4) for c in range(qb)][4 * i:4 * i + 4]

        def grp(i):
            get_max(i)
            if i in dg:
                pv_diag(dg.index(i))
                return
            for t in tiles(i):
                pv_tile(i, *t)

        def rd():
            r = jax.lax.dot_general(MST[g].astype(BF16), pltpu.bitcast(PQ[...], BF16), NT, preferred_element_type=F32)
            for c in range(4):
                RD[c] = r[0:136, c * 128:(c + 1) * 128]

        def upd():
            vall = pltpu.bitcast(jnp.concatenate([VT[c] for c in range(4)], axis=1), BF16)
            u = jnp.dot(vall, pltpu.bitcast(PK[...], BF16), preferred_element_type=F32)
            rr = jax.lax.broadcasted_iota(jnp.int32, (144, 128), 0)
            cc = jax.lax.broadcasted_iota(jnp.int32, (144, 128), 1) // DH
            keep = jnp.where(rr < 128, rr // DH, rr - 128) == cc
            u = jnp.where(keep, u, 0.0)
            MST[g] = MST[g + zz] + u if mem else u

        def act(tok):
            if tok[0] == "Q":
                qk(int(tok[1]))
            elif tok[0] == "D":
                diag(int(tok[1]))
            elif tok[0] == "G":
                grp(int(tok[1]))
            elif tok[0] == "g":
                get_max(int(tok[1]))
            elif tok[0] == "S":
                put(int(tok[1]))
            elif tok == "R":
                rd()
            else:
                assert tok == "U"
                upd()

        return act

    def run(sched, steps, queues):
        queues = {k: list(v) for k, v in queues.items()}
        si = 0
        for tok in sched.split():
            if tok == "|":
                si += 1
            elif tok == "z":
                pin_load()
            elif tok == "Z":
                queues["O"].pop(0)(pin=True)
            elif tok in queues:
                queues[tok].pop(0)()
            elif tok[-1] == "+":
                steps[si + 1](tok[:-1])
            else:
                steps[si](tok)
        assert all(not v for v in queues.values()), {k: len(v) for k, v in queues.items()}

    def ffn_patch(layer):
        hi = RT[0:8, :]
        lo = RT[8:16, :]
        RT[...] = jnp.full((16, 128), IMIN, I32)
        for sh in (4, 2, 1):
            h2 = pltpu.roll(hi, sh, 0)
            lo = jnp.maximum(jnp.minimum(hi, h2), jnp.maximum(lo, pltpu.roll(lo, sh, 0)))
            hi = jnp.maximum(hi, h2)
        i1 = jnp.clip(S - 1 - (hi[0, 0] & (S - 1)), 0, S - 1)
        i2 = jnp.clip(S - 1 - (lo[0, 0] & (S - 1)), 0, S - 1)
        b1 = pl.multiple_of((i1 // 16) * 16, 16)
        b2 = pl.multiple_of((i2 // 16) * 16, 16)
        i16 = jax.lax.broadcasted_iota(jnp.int32, (16, 1), 0)
        s1 = i16 + b1 == i1
        s2 = i16 + b2 == i2

        def pick(i):
            u = jnp.concatenate([jnp.broadcast_to(Tu[k, pl.ds(i // 2, 1), :], (8, 128)) for k in range(8)], axis=1)
            sh = (16 - 16 * (i % 2)).astype(U32)
            return pltpu.bitcast((u << sh) & jnp.uint32(0xFFFF0000), F32)

        x1 = jnp.concatenate([pick(i1), pick(i2)], axis=0)
        yb = _ln_f32(x1).astype(BF16)
        kv = jnp.concatenate([hi, lo], axis=0) & -65536
        rsel = pltpu.bitcast(jnp.where(kv < 0, (-kv) | IMIN, kv), F32)[:, 0:1]

        def dot512(x, ref, r, c):
            return jnp.dot(x, ref[512 * r:512 * (r + 1), 128 * c:128 * (c + 1)], preferred_element_type=F32)

        def gate_up(c):
            hs = []
            for n in range(4 * c, 4 * c + 4):
                gt, up = [_rb(dot512(yb[:, :512], w, 0, n) + dot512(yb[:, 512:], w, 1, n)) for w in (WG, WU)]
                hs.append(_rb(gt * _rb(jax.nn.sigmoid(gt))) * up)
            return jnp.concatenate(hs, axis=1).astype(BF16)

        hm = gate_up(0)
        yv = None
        for c in range(NFC):
            nxt = gate_up(c + 1) if c + 1 < NFC else None
            dn = jnp.concatenate([dot512(hm, WD, c, n) for n in range(8)], axis=1)
            yv = dn if yv is None else yv + dn
            hm = nxt

        def patch_r():
            x2 = _rb(x1 + _rb(yb.astype(F32) + _rb(_rb(yv) * _rb(jax.nn.sigmoid(rsel)))))
            for b, sel, lo in ((b1, s1, 0), (b2, s2, 8)):
                new = jnp.concatenate([x2[lo:lo + 8], x2[lo:lo + 8]], axis=0)
                R[pl.ds(b, 16), :] = jnp.where(sel, new, R[pl.ds(b, 16), :].astype(F32)).astype(BF16)
            return x2

        def patch_xn():
            xn = _rb(_ln_f32(patch_r()))
            for b, sel, lo in ((b1, s1, 0), (b2, s2, 8)):
                new = jnp.concatenate([xn[lo:lo + 8], xn[lo:lo + 8]], axis=0)
                for k in range(8):
                    XN[k, pl.ds(b, 16), :] = jnp.where(sel, new[:, k * 128:(k + 1) * 128],
                                                       XN[k, pl.ds(b, 16), :].astype(F32)).astype(BF16)

        @pl.when(layer == 0)
        def _():
            hit = [(i1 // 128 == c) | (i2 // 128 == c) for c in range(4)]
            ca = jnp.where(hit[0], jnp.where(hit[1], 2, 1), 0)
            cb = jnp.where(hit[3], jnp.where(hit[2], 1, 2), 3)
            cc = jnp.where(ca == 0, jnp.where(cb == 1, 2, 1), 0)
            cd = jnp.clip(6 - ca - cb - cc, 0, 3)
            run("P P P P P P P P P P P P x P P m m P P m m P P m m P P m m P P P P", [],
                {"P": proj_rounds(0, 0, bufs[0], (ca, cb, cc, cd)), "x": [patch_xn],
                 "m": ln_units(L, 128, False, 2)[:8]})

        @pl.when(layer == 1)
        def _():
            for s in range(11):
                out_copy(0, 128, s).wait()
            out_copy(0, 640, 11).wait()
            patch_r()
            c1 = out_copy(b1, 16, 0)
            c1.start()

            @pl.when(b2 != b1)
            def _():
                c2 = out_copy(b2, 16, 1)
                c2.start()
                c2.wait()

            c1.wait()

    def a_run(gp, wait=None):
        g0 = 2 * gp
        run(SCHED_A.replace("|", "w |") if wait else SCHED_A,
            [attn(0, g0, bufs[0], False), attn(0, g0 + 1, bufs[1], False)],
            {"P": proj_rounds(0, g0 + 1, bufs[1]) + proj_rounds(gp // 3, (g0 + 2) % NG, bufs[0]),
             "n": ln_units(L + gp * 128, 128, False, 2)[8:],
             "m": ln_units(L + 128 + gp * 128, 128, False, 2)[:8], "w": [wait] if wait else []})

    def a0_wait():
        for j in range(3):
            w_copy(2, j).wait()
        for j in range(3):
            w_copy(4, j).start()
        x_copy(768, 128, 6).start()

    p0 = proj_rounds(0, 0, bufs[0])
    x_copy(0, 128, 0).wait()
    x_copy(256, 128, 2).start()
    for f in ln_units(0, 128, False, 2, 0, True):
        f()
    w_all(0, False)
    x_copy(384, 128, 3).start()
    x_copy(512, 128, 4).start()
    w_all(1, True)
    for c in range(4):
        x_copy(0, 128, c + 1).wait()
        if c == 2:
            x_copy(640, 128, 5).start()
            w_all(2, True)
        u = ln_units(128 * (c + 1), 128, False, 2, 0, True)
        for f in u[:8] + p0[6 * c:6 * c + 4] + (u[8:] if c < 3 else []) + p0[6 * c + 4:6 * c + 6]:
            f()
    w_all(3, True)
    w_all(1, False)
    x_copy(0, 128, 5).wait()
    a_run(0, a0_wait)

    def layer_body(layer, carry):
        def a_body(gp, carry2):
            g0 = 2 * gp
            g2 = (g0 + 2) % NG

            @pl.when(layer == 0)
            def _():
                @pl.when(gp < 3)
                def _():
                    for j in range(3):
                        w_copy(g0 + 3, j).start()

                @pl.when(gp == 1)
                def _():
                    for j in range(3):
                        w_copy(6, j).start()
                    x_copy(896, 128, 7).start()
                    for n in range(8):
                        wo_copy(n).start()

                @pl.when(gp >= 2)
                def _():
                    x_copy(pl.multiple_of(gp * L, L), L, 6 + gp).start()

                for j in range(3):
                    w_copy(g0 + 1, j).wait()

                @pl.when(gp < 3)
                def _():
                    for j in range(3):
                        w_copy(g2, j).wait()
                    x_copy(0, 128, 5 + gp).wait()

                @pl.when(gp == 3)
                def _():
                    x_copy(0, L, 8).wait()

            a_run(gp)
            return carry2

        jax.lax.fori_loop(1 - layer, 4, a_body, 0)

        @pl.when(layer == 0)
        def _():
            for c in ffn_copies:
                c.start()
            for n in range(8):
                wo_copy(n).wait()
            x_copy(0, L, 9).wait()

        def b_body(it, carry2):
            seg = 1 + it // 4
            gp = it % 4
            g0 = 2 * gp
            g2 = (g0 + 2) % NG
            prow = (seg - 1) * L + gp * 128
            run(SCHED_B, [attn(seg, g0, bufs[0], True), attn(seg, g0 + 1, bufs[1], True)],
                {"P": proj_rounds(seg, g0 + 1, bufs[1]) + proj_rounds(seg + gp // 3, g2, bufs[0]),
                 "O": out_rounds(seg - 1, gp * 128, 128),
                 "n": ln_units((1024 + it * 128) % S, 128, False, 2)[8:],
                 "m": ln_units((1152 + it * 128) % S, 128, False, 2)[:8],
                 "t": ln_units(prow, 128, True, 0)})

            @pl.when(layer == 1)
            def _():
                out_copy(pl.multiple_of(prow, 128), 128, it).start()

            return carry2

        jax.lax.fori_loop(0, 11, b_body, 0)

        pieces = ((0, 128), (128, 128), (256, 64), (320, 64), (384, 64), (448, 32), (480, 32))
        run(SCHED_T, [attn(3, 6, bufs[0], True), attn(3, 7, bufs[1], True, True)],
            {"P": proj_rounds(3, 7, bufs[1]),
             "O": out_rounds(2, 384, 128) + [f for off, n in pieces for f in out_rounds(3, off, n, True)],
             "n": ln_units(384, 128, False, 2)[8:],
             "t": ln_units(2 * L + 384, 128, True, 0, 1)
             + [f for i, (off, n) in enumerate(pieces)
                for f in ln_units(3 * L + off, n, True, 4 + 2 * (i % 2), 2)]})

        @pl.when(layer == 0)
        def _():
            for c in ffn_copies:
                c.wait()

        @pl.when(layer == 1)
        def _():
            out_copy(S - 640, 640, 11).start()

        ffn_patch(layer)
        return carry

    jax.lax.fori_loop(0, 2, layer_body, 0)


@jax.jit
def pallas_interleave_layers__memory_aug_infini_attn__moe_arch_mod__prompt_kernel(
    A_x: jax.Array,
    A_wq: jax.Array,
    A_wk: jax.Array,
    A_wv: jax.Array,
    A_wo: jax.Array,
    A_beta: jax.Array,
    B_x: jax.Array,
    B_w_r: jax.Array,
    B_w_gate: jax.Array,
    B_w_up: jax.Array,
    B_w_down: jax.Array,
):
    hbm = pl.BlockSpec(memory_space=pl.ANY)
    vmem = pl.BlockSpec(memory_space=pltpu.VMEM)
    qkv_set = [
        pltpu.VMEM((L, 128), BF16),
        pltpu.VMEM((4, 64, 128), U32),
        pltpu.VMEM((L, 128), BF16),
        pltpu.VMEM((L, 128), BF16),
        pltpu.VMEM((4, 72, 128), U32),
        pltpu.VMEM((4, 128, 128), F32),
        pltpu.VMEM((4, 256, 128), F32),
        pltpu.VMEM((4, 384, 128), F32),
        pltpu.VMEM((4, 512, 128), F32),
        pltpu.VMEM((4, 136, 128), F32),
    ]
    scratch = [
        pltpu.VMEM((S + 16, D), BF16),
        pltpu.VMEM((8, S + 16, 128), BF16),
        pltpu.VMEM((8, S, 128), BF16),
        pltpu.VMEM((NG, 3, D, 128), BF16),
        pltpu.VMEM((8, D, 128), BF16),
        pltpu.VMEM((D, FF), BF16),
        pltpu.VMEM((D, FF), BF16),
        pltpu.VMEM((FF, D), BF16),
        pltpu.VMEM((NG, 2 * L, 128), BF16),
        pltpu.VMEM((NG, 144, 128), F32),
        pltpu.VMEM((NG, 8, 128), F32),
        pltpu.VMEM((8, D), F32),
        pltpu.VMEM((32, 128), F32),
        pltpu.VMEM((4, 8, 128), U32),
        pltpu.VMEM((PD + 16, 128), F32),
        pltpu.VMEM((536, 128), F32),
        pltpu.VMEM((16, 128), I32),
    ] + qkv_set + qkv_set + [pltpu.VMEM((64, 128), U32)] * 4 + [
        pltpu.VMEM((1024, 128), F32),
        pltpu.SMEM((1,), jnp.int32),
        pltpu.SemaphoreType.DMA((10,)),
        pltpu.SemaphoreType.DMA((NG, 3)),
        pltpu.SemaphoreType.DMA((11,)),
        pltpu.SemaphoreType.DMA((12,)),
    ]
    return pl.pallas_call(
        _kernel,
        out_shape=jax.ShapeDtypeStruct((1, S, D), BF16),
        in_specs=[hbm, hbm, hbm, hbm, hbm, vmem, vmem, hbm, hbm, hbm],
        out_specs=hbm,
        scratch_shapes=scratch,
        compiler_params=pltpu.CompilerParams(vmem_limit_bytes=100 * 1024 * 1024),
    )(A_x, A_wq, A_wk, A_wv, A_wo, A_beta, B_w_r, B_w_gate, B_w_up, B_w_down)
```

```python
import jax
import jax.numpy as jnp
import jax.experimental.pallas as pl
import jax.experimental.pallas.tpu as pltpu

F32 = jnp.float32
BF16 = jnp.bfloat16
U32 = jnp.uint32
I32 = jnp.int32
IMIN = -2147483648

S = 2048
D = 1024
H = 32
DH = 32
NSEG = 4
L = S // NSEG
NG = 8
FF = 3584
FCH = 512
NFC = FF // FCH
LOG2E = 1.4426950408889634
QSCALE = (DH ** -0.5) * LOG2E
NEG = -1000000000.0 * LOG2E
EPS_LN = 1.0013580322265625e-05
BIG = 3.0e38
NT = (((1,), (1,)), ((), ()))
PZ = 1024
PD = 1032

SCHED_A = ("D0 g0 n Q1 g1 n D2 n Q2 n G0 S0 P P G1 g2 m P P G2 g3 S1 m P P G3 g4 Q3 m P P G4 g5 m P P G5 g6 S2 m "
           "P P G6 g7 m P P G7 g8 m P P G8 g9 m P P G9 S3 P P D0+ P P Q1+ g0+ P P U | G0 g1 S0 P P D2 G1 g2 P P "
           "Q2 G2 g3 S1 P P G3 g4 P P G4 g5 Q3 P P G5 g6 S2 P P G6 g7 P P G7 g8 P P G8 g9 P P G9 S3 P P P P P P "
           "U ")
SCHED_B = ("O O n O O n m O O n m O O n m O O m m O O m D0 O O g0 m Q1 R O O g1 m G0 S0 P P D2 G1 g2 t t P P Q2 "
           "G2 g3 S1 t t P P G3 g4 t P P G4 g5 Q3 t P P G5 g6 S2 t P P G6 g7 t P P G7 g8 P P G8 g9 P P G9 S3 t P "
           "P D0+ t P P Q1+ g0+ P P U | R G0 g1 S0 P P D2 G1 g2 P P Q2 G2 g3 S1 P P G3 g4 P P G4 g5 Q3 P P G5 g6 "
           "S2 P P G6 g7 P P G7 g8 P P G8 g9 P P G9 S3 t P P t P P P P U ")
SCHED_T = ("O O n O O n O O n D0 Q1 g0 R O O n G0 g1 S0 D2 G1 g2 P P Q2 G2 g3 S1 P P G3 g4 P P G4 g5 Q3 P P G5 "
           "g6 S2 P P G6 g7 P P G7 g8 P P G8 g9 P P G9 S3 P P D0+ P P Q1+ g0+ P P P P | R O O G0 g1 O O S0 D2 G1 "
           "g2 O O Q2 G2 g3 O O S1 G3 g4 O O G4 g5 Q3 t t O O G5 g6 t t t O O S2 G6 g7 t O O G7 g8 t O O G8 g9 t "
           "O O G9 t O O S3 t z O O t t z O O t z Z O t z Z O t z Z O t z Z O t z Z O t z Z O t z Z O t z Z O t "
           "z O O t z Z O t z O O z Z O t z Z O t z Z O z Z O t z Z O t z Z O z Z O t z Z O t z Z O t z Z O z Z "
           "O t z Z O z Z O t z Z O t z Z O t z Z O z Z O t z Z O z Z O t z Z O z Z O t z Z O Z O t z O O Z O O "
           "O t z Z O Z O t z O O t z Z O O O t O O Z O O O t Z O Z O t t t ")


def _rb(t):
    return t.astype(BF16).astype(F32)


def _rb2(t):
    n = t.shape[0] // 2
    p = pltpu.pack_elementwise([t[:n], t[n:]], packed_dtype=BF16)
    return jnp.concatenate([pltpu.unpack_elementwise(p, index=i, packed_dtype=BF16, unpacked_dtype=F32)
                            for i in range(2)], axis=0)


def _rcp(d):
    d = jnp.minimum(d, BIG)
    r = pl.reciprocal(d, approx=True)
    return r * (2.0 - d * r)


def _rinv(var):
    v = _rb(_rb(var) + EPS_LN)
    vc = jnp.minimum(v, BIG)
    return jnp.minimum(_rcp(_rb(vc * jax.lax.rsqrt(vc))), 1e30 * pl.reciprocal(v, approx=True))


def _ln_f32(x):
    mu = jnp.sum(x, axis=1, keepdims=True) * (1.0 / D)
    xc = x - mu
    var = jnp.sum(xc * xc, axis=1, keepdims=True) * (1.0 / D)
    return (x - _rb(mu)) * _rinv(var)


def _phi(t):
    return jnp.maximum(t, 0.0) + jnp.exp(jnp.minimum(t, 0.0))


def _bind(f, *a):
    return lambda **kw: f(*a, **kw)


def _kernel(x_hbm, wq_hbm, wk_hbm, wv_hbm, wo_hbm, beta_ref, wr_ref, wg_hbm, wu_hbm, wd_hbm,
            out_hbm,
            R, T, XN, W, WO, WG, WU, WD, OB, MST, GT, WR, CM, LM, PN, PG, RT,
            K0, Q0, PQ0, PK0, VT0, SA0, SB0, SC0, SD0, RD0, K1, Q1, PQ1, PK1, VT1, SA1, SB1, SC1, SD1, RD1,
            OL0, OL1, OL2, OL3, PS, ZS, sx, sw, sm, so):
    bufs = ((K0, Q0, PQ0, PK0, VT0, (SA0, SB0, SC0, SD0), RD0), (K1, Q1, PQ1, PK1, VT1, (SA1, SB1, SC1, SD1), RD1))
    OL = (OL0, OL1, OL2, OL3)
    ZS[0] = 0
    XNu = XN.bitcast(U32)
    Wu = W.bitcast(U32)
    WOu = WO.bitcast(U32)
    OBu = OB.bitcast(U32)
    Tu = T.bitcast(U32)

    def x_copy(row0, n, s):
        return pltpu.make_async_copy(x_hbm.at[0, pl.ds(row0, n), :], R.at[pl.ds(row0, n), :], sx.at[s])

    def w_copy(g, j):
        src = (wq_hbm, wk_hbm, wv_hbm)[j]
        return pltpu.make_async_copy(src.at[:, pl.ds(pl.multiple_of(g * 128, 128), 128)], W.at[g, j], sw.at[g, j])

    def wo_copy(n):
        return pltpu.make_async_copy(wo_hbm.at[:, pl.ds(n * 128, 128)], WO.at[n], sm.at[n])

    ffn_copies = (pltpu.make_async_copy(wg_hbm, WG, sm.at[8]),
                  pltpu.make_async_copy(wu_hbm, WU, sm.at[9]),
                  pltpu.make_async_copy(wd_hbm, WD, sm.at[10]))

    def out_copy(row0, n, s):
        return pltpu.make_async_copy(R.at[pl.ds(row0, n), :], out_hbm.at[0, pl.ds(row0, n), :], so.at[s])

    x_copy(0, 128, 0).start()
    w_copy(0, 0).start()
    x_copy(128, 128, 1).start()
    w_copy(0, 1).start()
    w_copy(0, 2).start()
    x_copy(256, 128, 2).start()
    x_copy(384, 128, 3).start()
    for g in (1, 2):
        for j in range(3):
            w_copy(g, j).start()
    x_copy(512, 128, 4).start()
    x_copy(640, 128, 5).start()

    gsig = jax.nn.sigmoid(beta_ref[...].astype(F32).reshape(1, H))
    eye = (jax.lax.broadcasted_iota(jnp.int32, (H, H), 0)
           == jax.lax.broadcasted_iota(jnp.int32, (H, H), 1))
    gcol = jnp.sum(jnp.where(eye, jnp.broadcast_to(gsig, (H, H)), 0.0), axis=1, keepdims=True)
    gfull = jnp.broadcast_to(gcol, (H, 128))
    for g in range(NG):
        GT[g, 0:4, :] = gfull[4 * g:4 * g + 4, :]
        GT[g, 4:8, :] = 1.0 - gfull[4 * g:4 * g + 4, :]
    WR[...] = jnp.broadcast_to(wr_ref[...].astype(F32).reshape(1, D), (8, D))
    kk = jax.lax.broadcasted_iota(jnp.int32, (32, 128), 0)
    qq = jax.lax.broadcasted_iota(jnp.int32, (32, 128), 1) % 32
    CM[...] = jnp.where(qq < kk, NEG, 0.0).astype(F32)
    for c in range(4):
        LM[c] = jnp.where(jax.lax.broadcasted_iota(jnp.int32, (8, 128), 1) // DH == c,
                          jnp.uint32(0xFFFFFFFF), jnp.uint32(0))
        VT0[c, 64:72, :] = pltpu.bitcast(jnp.ones((16, 128), BF16), U32)
        VT1[c, 64:72, :] = pltpu.bitcast(jnp.ones((16, 128), BF16), U32)
    RT[...] = jnp.full((16, 128), IMIN, I32)
    PN[PZ:PZ + 8, :] = jnp.zeros((8, 128), F32)
    PG[528:536, :] = jnp.zeros((8, 128), F32)
    R[S:S + 16, 0:128] = jnp.zeros((16, 128), BF16)
    T[0, S:S + 16, :] = jnp.zeros((16, 128), BF16)

    def ln_units(row0, nrows, router, slab, late=0):
        zz = ZS[0]
        st = PS if late else PN

        def ld(i, k, v):
            if router:
                r2 = pl.multiple_of(row0 // 2 + 16 * i + zz * v, 16)
                return pltpu.bitcast(Tu[k, pl.ds(r2, 16), :], BF16).astype(F32)
            r1 = pl.multiple_of(row0 + 32 * i + zz * v, 32)
            return R[pl.ds(r1, 32), k * 128:(k + 1) * 128].astype(F32)

        def st_put(i, j, val):
            r = pl.multiple_of((slab + j) * 128 + 32 * i + zz, 32)
            st[pl.ds(r, 32), :] = jnp.broadcast_to(val, (32, 128))

        def done(val):
            PG[pl.ds(pl.multiple_of(520 + zz, 8), 8), :] = val[-8:]

        def st_get(i, j, v):
            return st[pl.ds(pl.multiple_of((slab + j) * 128 + 32 * i + zz * v, 32), 32), :]

        def mean(*ii):
            z = PN[pl.ds(pl.multiple_of(PZ + zz, 8), 8), :]
            accs = []
            for i in ii:
                acc = jnp.concatenate([z, z, z, z], axis=0)
                for k in range(8):
                    acc = acc + ld(i, k, 1)
                accs.append(acc)
            for i, acc in zip(ii, accs):
                done(acc)
                st_put(i, 0, jnp.sum(acc, axis=1, keepdims=True) * (1.0 / D))

        def var(*ii):
            mus = [st_get(i, 0, 2) for i in ii]
            for i, mu in zip(ii, mus):
                acc = None
                for k in range(8):
                    xc = ld(i, k, 2) - mu
                    acc = xc * xc if acc is None else acc + xc * xc
                done(acc)
                st_put(i, 1, _rinv(jnp.sum(acc, axis=1, keepdims=True) * (1.0 / D)))

        def norm(i):
            mu = _rb2(st_get(i, 0, 3))
            ri = st_get(i, 1, 3)
            acc = None
            for k in range(8):
                x = ld(i, k, 3)
                y = (x - mu) * ri
                if k == 7 and not late:
                    PN[pl.ds(pl.multiple_of(PD + 8 + zz, 8), 8), :] = y[24:32]
                    done(y)
                if not router:
                    XN[k, pl.ds(pl.multiple_of(row0 + 32 * i, 32), 32), :] = y.astype(BF16)
                    continue
                y = _rb2(y)
                wr = WR[:, k * 128:(k + 1) * 128]
                yw = y * jnp.concatenate([wr, wr, wr, wr], axis=0)
                acc = yw if acc is None else acc + yw
                R[pl.ds(pl.multiple_of(row0 + 32 * i, 32), 32), k * 128:(k + 1) * 128] = (x + y).astype(BF16)
            if router:
                r = jnp.broadcast_to(_rb(jnp.sum(acc, axis=1, keepdims=True)), (32, 128))
                b = pltpu.bitcast(r, I32)
                sg = b >> 31
                tok = jax.lax.broadcasted_iota(I32, (32, 128), 0) + (row0 + 32 * i - (S - 1))
                key = ((b & 0x7FFF0000) ^ sg) - (sg + tok)
                hi = RT[0:8, :]
                lo = RT[8:16, :]
                for j in range(4):
                    kj = key[8 * j:8 * j + 8]
                    lo = jnp.maximum(lo, jnp.minimum(hi, kj))
                    hi = jnp.maximum(hi, kj)
                RT[0:8, :] = hi
                RT[8:16, :] = lo
                if late:
                    done(pltpu.bitcast(lo, F32))

        n = nrows // 32
        if late > 1 and n > 1:
            return ([_bind(f, i, i + 1) for f in (mean, var) for i in range(0, n, 2)]
                    + [_bind(norm, i) for i in range(n)])
        return [_bind(f, i) for f in (mean, var, norm) for i in range(n)]

    def proj_rounds(seg, g, buf, order=(0, 1, 2, 3)):
        Kb, Qm, PQ, PK, VT, SB, RD = buf
        zz = ZS[0]
        part = {}

        def rnd(c, j, half):
            r2 = pl.multiple_of(seg * (L // 2) + c * 64 + zz * j, 64)
            xn = jnp.concatenate([pltpu.bitcast(XNu[k, pl.ds(r2, 64), :], BF16)
                                  for k in range(4 * half, 4 * half + 4)], axis=1)
            w = pltpu.bitcast(Wu[g, j, pl.ds(pl.multiple_of(256 * half + zz * c, 256), 256), :], BF16)
            t = jnp.dot(xn, w, preferred_element_type=F32)
            if half == 0:
                part[0] = t
                return
            t = t + part[0]
            PN[PD:PD + 8, :] = t[120:128]
            PG[512:520, :] = t[120:128]
            rows = pl.ds(c * 128 if isinstance(c, int) else pl.multiple_of(c * 128, 128), 128)
            if j == 0:
                qt = pltpu.bitcast((t * QSCALE).astype(BF16).T, U32)
                for h in range(4):
                    qh = qt[16 * h:16 * h + 16]
                    Qm[c, 16 * h:16 * h + 16, :] = pltpu.roll(qh, 32 * h, 1) if h else qh
                PQ[rows, :] = _phi(t).astype(BF16)
            elif j == 1:
                Kb[rows, :] = t.astype(BF16)
                PK[rows, :] = _phi(t).astype(BF16)
            else:
                VT[c, 0:64, :] = pltpu.bitcast(t.astype(BF16).T, U32)

        return [_bind(rnd, c, j, half) for c in order for j in range(3) for half in range(2)]

    pins = [None]

    def pin_load():
        pins.append(pltpu.bitcast(PG[pl.ds(pl.multiple_of(528 + ZS[0], 8), 8), :], U32)
                    | pltpu.bitcast(R[pl.ds(pl.multiple_of(S + ZS[0], 16), 16), 0:128], U32)
                    | Tu[0, pl.ds(pl.multiple_of(S // 2 + ZS[0], 8), 8), :])

    def out_rounds(seg, off, nrows, last=False):
        zz = ZS[0]
        part = {}
        n2 = nrows // 2

        def rnd(n, half, pin=False):
            o2 = pl.multiple_of(((seg % 2) * L + off) // 2 + zz * (n + 1), 16)
            o = [OBu[k, pl.ds(o2, n2), :] for k in range(4 * half, 4 * half + 4 - (last and half))]
            if last and half:
                o.append(OL[off // 128][pl.ds(pl.multiple_of((off % 128) // 2 + zz * (n + 1), 16), n2), :])
            if pin:
                pins[0:2] = pins[1:2]
            if last and pins[0] is not None:
                o = [jnp.concatenate([v[0:8] | pins[0], v[8:]], axis=0) for v in o]
            o = jnp.concatenate([pltpu.bitcast(v, BF16) for v in o], axis=1)
            w = pltpu.bitcast(WOu[n, pl.ds(pl.multiple_of(256 * half + zz * (seg * L + off), 256), 256), :], BF16)
            t = jnp.dot(o, w, preferred_element_type=F32)
            if half == 0:
                part[0] = t
                return
            x = R[pl.ds(pl.multiple_of(seg * L + off, 32), nrows), n * 128:(n + 1) * 128].astype(F32)
            t = t + part[0]
            PN[PD:PD + 8, :] = t[nrows - 8:nrows]
            PG[512:520, :] = t[nrows - 8:nrows]
            T[n, pl.ds(pl.multiple_of(seg * L + off, 32), nrows), :] = (x + _rb2(t)).astype(BF16)

        return [_bind(rnd, n, half) for n in range(8) for half in range(2)]

    def attn(seg, g, buf, mem, last=False):
        Kb, Qm, PQ, PK, VT, SB, RD = buf
        Kb, PQ, PK = Kb.bitcast(U32), PQ.bitcast(U32), PK.bitcast(U32)
        zz = ZS[0]
        pg0 = 0 if buf is bufs[0] else 256
        ml = {}
        m8_ = {}
        acc = {}
        fin = {}

        def bfly(e, rows):
            lane = jax.lax.broadcasted_iota(jnp.int32, (rows, 128), 1)
            s0 = (lane & 32) != 0
            s1 = (lane & 64) != 0

            def sel(m, x, y):
                if x is None and y is None:
                    return None
                z = jnp.zeros_like(x if y is None else y)
                return jnp.where(m, z if x is None else x, z if y is None else y)

            a = [[sel(s1, e[2 + j], e[j]), sel(s1, e[j], e[2 + j])] for j in range(2)]
            return [sel(s0, a[1][0], a[0][0]), sel(s0, a[0][0], a[1][1]),
                    sel(s0, a[1][1], a[0][1]), sel(s0, a[0][1], a[1][0])]

        def put_max(qb, m8):
            m = jnp.broadcast_to(jnp.max(m8, axis=0, keepdims=True), (8, 512))
            m = [m[:, 128 * h:128 * (h + 1)] for h in range(4)]
            for i, v in enumerate(m + bfly(m, 8)):
                if qb > 0 or i >= 4:
                    PG[pg0 + 64 * qb + 8 * i:pg0 + 64 * qb + 8 * i + 8, :] = v

        def get_max(i):
            for qb, h in [(dg.index(i), 4 + j) for j in range(4)] if i in dg else [t[:2] for t in tiles(i)]:
                if (i, h) not in ml:
                    ml[(i, h)] = PG[pl.ds(pl.multiple_of(zz * (i + 1) + pg0 + 64 * qb + 8 * h, 8), 8), :]

        def diag(qa):
            lm = [jnp.concatenate([LM[i]] * 2, axis=0) for i in range(4)]
            for qb, rev in ((qa, False), (qa + 1, True)):
                m8 = [None] * 4
                for j in range(3, -1, -1):
                    w = jnp.concatenate([Qm[qb, 16 * h:16 * h + 16, :] & lm[(j + h) % 4] for h in range(4)], axis=0)
                    rs = range(j, -1, -1) if rev else range(j + 1)
                    kq = jnp.concatenate([Kb[64 * qb + 16 * r:64 * qb + 16 * r + 16, :] for r in rs], axis=0)
                    d = jnp.dot(pltpu.bitcast(kq, BF16), pltpu.bitcast(w, BF16), preferred_element_type=F32)
                    for i, r in enumerate(rs):
                        v = d[32 * i:32 * i + 32] + CM[...] if r == j else d[32 * i:32 * i + 32]
                        SB[qb][j, 128 * qb + 32 * r:128 * qb + 32 * r + 32, :] = v
                        mx = jnp.max(v.reshape(4, 8, 128), axis=0)
                        m8[j] = mx if m8[j] is None else jnp.maximum(m8[j], mx)
                m8_[qb] = jnp.concatenate(bfly(m8, 8), axis=1)
            if qa == 0:
                put_max(0, m8_[0])

        def qk(qb):
            z16 = jnp.zeros((16, 128), U32)
            w = jnp.concatenate([jnp.concatenate([Qm[qb, 16 * h:16 * h + 16, :] if i == h else z16
                                                  for i in range(4)], axis=0) for h in range(4)], axis=1)
            s = jnp.dot(pltpu.bitcast(Kb[0:64 * qb, :], BF16), pltpu.bitcast(w, BF16), preferred_element_type=F32)
            m8 = m8_[qb]
            for c in range(qb):
                blk = s[c * 128:(c + 1) * 128, :]
                for h in range(4):
                    SB[qb][h, c * 128:(c + 1) * 128, :] = blk[:, 128 * h:128 * (h + 1)]
                m8 = jnp.maximum(m8, jnp.max(blk.reshape(16, 8, 512), axis=0))
            put_max(qb, m8)

        def pv(qb, h, c, p, l8):
            o = jnp.dot(pltpu.bitcast(VT[c, 16 * h:16 * h + 16, :], BF16), p, preferred_element_type=F32)
            if (qb, h) in acc:
                o0, l0, n = acc[(qb, h)]
                o = o + o0
                l8 = l0 + l8
            else:
                n = 0
            acc[(qb, h)] = (o, l8, n + 1)
            if n == qb:
                gt = GT[g]
                l = jnp.sum(l8, axis=0, keepdims=True)
                res = o * (gt[4 + h:5 + h, :] * _rcp(l))
                if h > 0:
                    res = pltpu.roll(res, 128 - 32 * h, 1)
                if mem:
                    num = RD[zz + qb, 32 * h:32 * h + 32, :]
                    den = RD[zz + qb, 128:136, :][h:h + 1, :] + 1e-06
                    res = num * (gt[h:h + 1, :] * _rcp(den)) + res
                fin[(qb, h)] = res

        def pv_tile(i, qb, h, c):
            m = jnp.concatenate([ml[(i, h)]] * 16, axis=0)
            p = jnp.exp2(SB[qb][h, pl.ds(pl.multiple_of(zz + c * 128, 128), 128), :] - m)
            l8 = p[120:128]
            for r in range(14, -1, -1):
                l8 = l8 + p[8 * r:8 * r + 8]
            pv(qb, h, c, p.astype(BF16), l8)

        def pv_diag(qb):
            m = [ml[(dg[qb], 4 + j)] for j in range(4)]
            l8 = [None] * 4
            w = {}
            for r in range(3, -1, -1):
                e = [None] * 4
                for j in range(r, 4):
                    mj = jnp.concatenate([m[j]] * 2, axis=0)
                    p = [jnp.exp2(SB[qb][j, pl.ds(zz + 128 * qb + 32 * r + i, 16, stride=2), :] - mj)
                         for i in range(2)]
                    for v in (p[1][8:16], p[1][0:8], p[0][8:16], p[0][0:8]):
                        l8[j] = v if l8[j] is None else l8[j] + v
                    e[j] = pltpu.pack_elementwise(p, packed_dtype=BF16)
                w[r] = bfly(e, 16)
            l8 = bfly(l8, 8)
            for h in range(4):
                pv(qb, h, qb, pltpu.bitcast(jnp.concatenate([w[r][h] for r in range(4)], axis=0), BF16), l8[h])

        def put(qb):
            ot = jnp.concatenate([fin[(qb, i)] for i in range(4)], axis=0).astype(BF16)
            if last:
                ot = pltpu.bitcast(ot.T, U32)
                OL[qb][...] = ot
                PG[pl.ds(pl.multiple_of(520 + zz, 8), 8), :] = pltpu.bitcast(ot[56:64], F32)
                return
            o2 = pl.multiple_of((seg % 2) * (L // 2) + 64 * qb, 64)
            OBu[g, pl.ds(o2, 64), :] = pltpu.bitcast(ot.T, U32)

        dg = (0, 1, 3, 6)

        def tiles(i):
            i = (2, 4, 5, 7, 8, 9).index(i)
            return [(qb, h, c) for qb in range(4) for h in range(4) for c in range(qb)][4 * i:4 * i + 4]

        def grp(i):
            get_max(i)
            if i in dg:
                pv_diag(dg.index(i))
                return
            for t in tiles(i):
                pv_tile(i, *t)

        def rd():
            r = jax.lax.dot_general(MST[g].astype(BF16), pltpu.bitcast(PQ[...], BF16), NT, preferred_element_type=F32)
            for c in range(4):
                RD[c] = r[0:136, c * 128:(c + 1) * 128]

        def upd():
            vall = pltpu.bitcast(jnp.concatenate([VT[c] for c in range(4)], axis=1), BF16)
            u = jnp.dot(vall, pltpu.bitcast(PK[...], BF16), preferred_element_type=F32)
            rr = jax.lax.broadcasted_iota(jnp.int32, (144, 128), 0)
            cc = jax.lax.broadcasted_iota(jnp.int32, (144, 128), 1) // DH
            keep = jnp.where(rr < 128, rr // DH, rr - 128) == cc
            u = jnp.where(keep, u, 0.0)
            MST[g] = MST[g + zz] + u if mem else u

        def act(tok):
            if tok[0] == "Q":
                qk(int(tok[1]))
            elif tok[0] == "D":
                diag(int(tok[1]))
            elif tok[0] == "G":
                grp(int(tok[1]))
            elif tok[0] == "g":
                get_max(int(tok[1]))
            elif tok[0] == "S":
                put(int(tok[1]))
            elif tok == "R":
                rd()
            else:
                assert tok == "U"
                upd()

        return act

    def run(sched, steps, queues):
        queues = {k: list(v) for k, v in queues.items()}
        si = 0
        for tok in sched.split():
            if tok == "|":
                si += 1
            elif tok == "z":
                pin_load()
            elif tok == "Z":
                queues["O"].pop(0)(pin=True)
            elif tok in queues:
                queues[tok].pop(0)()
            elif tok[-1] == "+":
                steps[si + 1](tok[:-1])
            else:
                steps[si](tok)
        assert all(not v for v in queues.values()), {k: len(v) for k, v in queues.items()}

    def ffn_patch(layer):
        hi = RT[0:8, :]
        lo = RT[8:16, :]
        RT[...] = jnp.full((16, 128), IMIN, I32)
        for sh in (4, 2, 1):
            h2 = pltpu.roll(hi, sh, 0)
            lo = jnp.maximum(jnp.minimum(hi, h2), jnp.maximum(lo, pltpu.roll(lo, sh, 0)))
            hi = jnp.maximum(hi, h2)
        i1 = jnp.clip(S - 1 - (hi[0, 0] & (S - 1)), 0, S - 1)
        i2 = jnp.clip(S - 1 - (lo[0, 0] & (S - 1)), 0, S - 1)
        b1 = pl.multiple_of((i1 // 16) * 16, 16)
        b2 = pl.multiple_of((i2 // 16) * 16, 16)
        i16 = jax.lax.broadcasted_iota(jnp.int32, (16, 1), 0)
        s1 = i16 + b1 == i1
        s2 = i16 + b2 == i2

        def pick(i):
            u = jnp.concatenate([jnp.broadcast_to(Tu[k, pl.ds(i // 2, 1), :], (8, 128)) for k in range(8)], axis=1)
            sh = (16 - 16 * (i % 2)).astype(U32)
            return pltpu.bitcast((u << sh) & jnp.uint32(0xFFFF0000), F32)

        x1 = jnp.concatenate([pick(i1), pick(i2)], axis=0)
        yb = _ln_f32(x1).astype(BF16)
        kv = jnp.concatenate([hi, lo], axis=0) & -65536
        rsel = pltpu.bitcast(jnp.where(kv < 0, (-kv) | IMIN, kv), F32)[:, 0:1]

        def dot512(x, ref, r, c):
            return jnp.dot(x, ref[512 * r:512 * (r + 1), 128 * c:128 * (c + 1)], preferred_element_type=F32)

        def gate_up(c):
            hs = []
            for n in range(4 * c, 4 * c + 4):
                gt, up = [_rb(dot512(yb[:, :512], w, 0, n) + dot512(yb[:, 512:], w, 1, n)) for w in (WG, WU)]
                hs.append(_rb(gt * _rb(jax.nn.sigmoid(gt))) * up)
            return jnp.concatenate(hs, axis=1).astype(BF16)

        hm = gate_up(0)
        yv = None
        for c in range(NFC):
            nxt = gate_up(c + 1) if c + 1 < NFC else None
            dn = jnp.concatenate([dot512(hm, WD, c, n) for n in range(8)], axis=1)
            yv = dn if yv is None else yv + dn
            hm = nxt

        def patch_r():
            x2 = _rb(x1 + _rb(yb.astype(F32) + _rb(_rb(yv) * _rb(jax.nn.sigmoid(rsel)))))
            for b, sel, lo in ((b1, s1, 0), (b2, s2, 8)):
                new = jnp.concatenate([x2[lo:lo + 8], x2[lo:lo + 8]], axis=0)
                R[pl.ds(b, 16), :] = jnp.where(sel, new, R[pl.ds(b, 16), :].astype(F32)).astype(BF16)
            return x2

        def patch_xn():
            xn = _rb(_ln_f32(patch_r()))
            for b, sel, lo in ((b1, s1, 0), (b2, s2, 8)):
                new = jnp.concatenate([xn[lo:lo + 8], xn[lo:lo + 8]], axis=0)
                for k in range(8):
                    XN[k, pl.ds(b, 16), :] = jnp.where(sel, new[:, k * 128:(k + 1) * 128],
                                                       XN[k, pl.ds(b, 16), :].astype(F32)).astype(BF16)

        @pl.when(layer == 0)
        def _():
            hit = [(i1 // 128 == c) | (i2 // 128 == c) for c in range(4)]
            ca = jnp.where(hit[0], jnp.where(hit[1], 2, 1), 0)
            cb = jnp.where(hit[3], jnp.where(hit[2], 1, 2), 3)
            cc = jnp.where(ca == 0, jnp.where(cb == 1, 2, 1), 0)
            cd = jnp.clip(6 - ca - cb - cc, 0, 3)
            run("P P P P P P P P P P P P x P P m m P P m m P P m m P P m m P P P P", [],
                {"P": proj_rounds(0, 0, bufs[0], (ca, cb, cc, cd)), "x": [patch_xn],
                 "m": ln_units(L, 128, False, 2)[:8]})

        @pl.when(layer == 1)
        def _():
            for s in range(11):
                out_copy(0, 128, s).wait()
            out_copy(0, 640, 11).wait()
            patch_r()
            c1 = out_copy(b1, 16, 0)
            c1.start()

            @pl.when(b2 != b1)
            def _():
                c2 = out_copy(b2, 16, 1)
                c2.start()
                c2.wait()

            c1.wait()

    p0 = proj_rounds(0, 0, bufs[0])
    x_copy(0, 128, 0).wait()
    for f in ln_units(0, 128, False, 2):
        f()
    for c in range(4):
        if c == 0:
            for j in range(3):
                w_copy(0, j).wait()
        if c < 3:
            x_copy(128 * (c + 1), 128, c + 1).wait()
            run("f f f f P P f f f f P P P P f f f f", [],
                {"P": p0[6 * c:6 * c + 6], "f": ln_units(128 * (c + 1), 128, False, 2)})
        else:
            x_copy(0, 128, 4).wait()
            run("m m m m P P m m P P m m P P", [], {"P": p0[18:24], "m": ln_units(L, 128, False, 2)[:8]})

    def layer_body(layer, carry):
        def a_body(gp, carry2):
            g0 = 2 * gp
            g2 = (g0 + 2) % NG

            @pl.when(layer == 0)
            def _():
                @pl.when(gp < 3)
                def _():
                    for j in range(3):
                        w_copy(g0 + 3, j).start()

                @pl.when(gp < 2)
                def _():
                    for j in range(3):
                        w_copy(g0 + 4, j).start()

                @pl.when(gp < 2)
                def _():
                    x_copy(pl.multiple_of(768 + 128 * gp, 128), 128, 6 + gp).start()

                @pl.when(gp == 1)
                def _():
                    for n in range(8):
                        wo_copy(n).start()

                @pl.when(gp >= 2)
                def _():
                    x_copy(pl.multiple_of(gp * L, L), L, 6 + gp).start()

                for j in range(3):
                    w_copy(g0 + 1, j).wait()

                @pl.when(gp < 3)
                def _():
                    for j in range(3):
                        w_copy(g2, j).wait()
                    x_copy(0, 128, 5 + gp).wait()

                @pl.when(gp == 3)
                def _():
                    x_copy(0, L, 8).wait()

            run(SCHED_A, [attn(0, g0, bufs[0], False), attn(0, g0 + 1, bufs[1], False)],
                {"P": proj_rounds(0, g0 + 1, bufs[1]) + proj_rounds(gp // 3, g2, bufs[0]),
                 "n": ln_units(L + gp * 128, 128, False, 2)[8:],
                 "m": ln_units(L + 128 + gp * 128, 128, False, 2)[:8]})
            return carry2

        jax.lax.fori_loop(0, 4, a_body, 0)

        @pl.when(layer == 0)
        def _():
            for c in ffn_copies:
                c.start()
            for n in range(8):
                wo_copy(n).wait()
            x_copy(0, L, 9).wait()

        def b_body(sched, it, carry2):
            seg = 1 + it // 4
            gp = it % 4
            g0 = 2 * gp
            g2 = (g0 + 2) % NG
            prow = (seg - 1) * L + gp * 128
            run(sched, [attn(seg, g0, bufs[0], True), attn(seg, g0 + 1, bufs[1], True)],
                {"P": proj_rounds(seg, g0 + 1, bufs[1]) + proj_rounds(seg + gp // 3, g2, bufs[0]),
                 "O": out_rounds(seg - 1, gp * 128, 128),
                 "n": ln_units((1024 + it * 128) % S, 128, False, 2)[8:],
                 "m": ln_units((1152 + it * 128) % S, 128, False, 2)[:8],
                 "t": ln_units(prow, 128, True, 0)})

            @pl.when(layer == 1)
            def _():
                out_copy(pl.multiple_of(prow, 128), 128, it).start()

            return carry2

        jax.lax.fori_loop(0, 8, lambda it, c: b_body(SCHED_B, it, c), 0)
        jax.lax.fori_loop(8, 11, lambda it, c: b_body(SCHED_B.replace(" U", ""), it, c), 0)

        pieces = ((0, 128), (128, 128), (256, 64), (320, 64), (384, 64), (448, 32), (480, 32))
        run(SCHED_T, [attn(3, 6, bufs[0], True), attn(3, 7, bufs[1], True, True)],
            {"P": proj_rounds(3, 7, bufs[1]),
             "O": out_rounds(2, 384, 128) + [f for off, n in pieces for f in out_rounds(3, off, n, True)],
             "n": ln_units(384, 128, False, 2)[8:],
             "t": ln_units(2 * L + 384, 128, True, 0, 1)
             + [f for i, (off, n) in enumerate(pieces)
                for f in ln_units(3 * L + off, n, True, 4 + 2 * (i % 2), 2)]})

        @pl.when(layer == 0)
        def _():
            for c in ffn_copies:
                c.wait()

        @pl.when(layer == 1)
        def _():
            out_copy(S - 640, 640, 11).start()

        ffn_patch(layer)
        return carry

    jax.lax.fori_loop(0, 2, layer_body, 0)


@jax.jit
def pallas_interleave_layers__memory_aug_infini_attn__moe_arch_mod__prompt_kernel(
    A_x: jax.Array,
    A_wq: jax.Array,
    A_wk: jax.Array,
    A_wv: jax.Array,
    A_wo: jax.Array,
    A_beta: jax.Array,
    B_x: jax.Array,
    B_w_r: jax.Array,
    B_w_gate: jax.Array,
    B_w_up: jax.Array,
    B_w_down: jax.Array,
):
    hbm = pl.BlockSpec(memory_space=pl.ANY)
    vmem = pl.BlockSpec(memory_space=pltpu.VMEM)
    qkv_set = [
        pltpu.VMEM((L, 128), BF16),
        pltpu.VMEM((4, 64, 128), U32),
        pltpu.VMEM((L, 128), BF16),
        pltpu.VMEM((L, 128), BF16),
        pltpu.VMEM((4, 72, 128), U32),
        pltpu.VMEM((4, 128, 128), F32),
        pltpu.VMEM((4, 256, 128), F32),
        pltpu.VMEM((4, 384, 128), F32),
        pltpu.VMEM((4, 512, 128), F32),
        pltpu.VMEM((4, 136, 128), F32),
    ]
    scratch = [
        pltpu.VMEM((S + 16, D), BF16),
        pltpu.VMEM((8, S + 16, 128), BF16),
        pltpu.VMEM((8, S, 128), BF16),
        pltpu.VMEM((NG, 3, D, 128), BF16),
        pltpu.VMEM((8, D, 128), BF16),
        pltpu.VMEM((D, FF), BF16),
        pltpu.VMEM((D, FF), BF16),
        pltpu.VMEM((FF, D), BF16),
        pltpu.VMEM((NG, 2 * L, 128), BF16),
        pltpu.VMEM((NG, 144, 128), F32),
        pltpu.VMEM((NG, 8, 128), F32),
        pltpu.VMEM((8, D), F32),
        pltpu.VMEM((32, 128), F32),
        pltpu.VMEM((4, 8, 128), U32),
        pltpu.VMEM((PD + 16, 128), F32),
        pltpu.VMEM((536, 128), F32),
        pltpu.VMEM((16, 128), I32),
    ] + qkv_set + qkv_set + [pltpu.VMEM((64, 128), U32)] * 4 + [
        pltpu.VMEM((1024, 128), F32),
        pltpu.SMEM((1,), jnp.int32),
        pltpu.SemaphoreType.DMA((10,)),
        pltpu.SemaphoreType.DMA((NG, 3)),
        pltpu.SemaphoreType.DMA((11,)),
        pltpu.SemaphoreType.DMA((12,)),
    ]
    return pl.pallas_call(
        _kernel,
        out_shape=jax.ShapeDtypeStruct((1, S, D), BF16),
        in_specs=[hbm, hbm, hbm, hbm, hbm, vmem, vmem, hbm, hbm, hbm],
        out_specs=hbm,
        scratch_shapes=scratch,
        compiler_params=pltpu.CompilerParams(vmem_limit_bytes=100 * 1024 * 1024),
    )(A_x, A_wq, A_wk, A_wv, A_wo, A_beta, B_w_r, B_w_gate, B_w_up, B_w_down)
```
